```python
import jax
import jax.numpy as jnp

def _softmax(x, axis=-1):
    return jax.nn.softmax(x, axis=axis)

def _gelu(x):
    return jax.nn.gelu(x, approximate=True)

def _silu(x):
    return jax.nn.silu(x)

def _sigmoid(x):
    return jax.nn.sigmoid(x)

def _layernorm(x, axis=-1, eps=1e-05):
    m = jnp.mean(x, axis=axis, keepdims=True)
    v = jnp.var(x, axis=axis, keepdims=True)
    return (x - m) / jnp.sqrt(v + eps)

def _scatter_add(tgt, idx, src, axis=0):
    return tgt.at[idx].add(src)

def _segment_sum(src, seg, n):
    return jax.ops.segment_sum(src, seg, n)

class _Rng:

    def __init__(self, key):
        self._k = key

    def _next(self):
        self._k, sub = jax.random.split(self._k)
        return sub

    def normal(self, shape):
        return jax.random.normal(self._next(), shape, dtype=jnp.bfloat16)

    def randint(self, lo, hi, shape):
        return jax.random.randint(self._next(), shape, lo, hi, dtype=jnp.int32)

    def uniform(self, shape, lo=0.0, hi=1.0):
        return jax.random.uniform(self._next(), shape, jnp.bfloat16, lo, hi)

    def permutation(self, n):
        return jax.random.permutation(self._next(), n)
kernel_name = 'standalone__conformer_family_conformer__speech'

def setup_inputs():
    _rng = _Rng(jax.random.key(int.from_bytes(__import__("os").urandom(4), "little")))
    _w = lambda a: (lambda t: t.astype(jnp.bfloat16) if jnp.issubdtype(t.dtype, jnp.floating) else t)(jnp.asarray(a))
    B, T, D, K = (2, 4000, 512, 15)
    F = 4 * D
    s = D ** (-0.5)
    sf = F ** (-0.5)
    return {'x': _w((lambda *s: _rng.normal(s) * 0.05)(B, T, D)), 'w_ff1_a': _w((lambda *s: _rng.normal(s) * 0.05)(D, F) * s), 'w_ff1_b': _w((lambda *s: _rng.normal(s) * 0.05)(F, D) * sf), 'w_q': _w((lambda *s: _rng.normal(s) * 0.05)(D, D) * s), 'w_k': _w((lambda *s: _rng.normal(s) * 0.05)(D, D) * s), 'w_v': _w((lambda *s: _rng.normal(s) * 0.05)(D, D) * s), 'w_o': _w((lambda *s: _rng.normal(s) * 0.05)(D, D) * s), 'w_pw1': _w((lambda *s: _rng.normal(s) * 0.05)(D, 2 * D) * s), 'dw': _w((lambda *s: _rng.normal(s) * 0.05)(K, D) * K ** (-0.5)), 'w_pw2': _w((lambda *s: _rng.normal(s) * 0.05)(D, D) * s), 'w_ff2_a': _w((lambda *s: _rng.normal(s) * 0.05)(D, F) * s), 'w_ff2_b': _w((lambda *s: _rng.normal(s) * 0.05)(F, D) * sf)}

def reference(x, w_ff1_a, w_ff1_b, w_q, w_k, w_v, w_o, w_pw1, dw, w_pw2, w_ff2_a, w_ff2_b):
    B, T, D = x.shape
    K = dw.shape[0]
    scale = D ** (-0.5)
    h = _layernorm(x, axis=-1)
    h = _silu(h @ w_ff1_a) @ w_ff1_b
    x1 = x + 0.5 * h
    h = _layernorm(x1, axis=-1)
    q = h @ w_q
    k = h @ w_k
    v = h @ w_v
    scores = jnp.einsum('btd,bsd->bts', q, k) * scale
    p = _softmax(scores, axis=-1)
    attn = jnp.einsum('bts,bsd->btd', p, v) @ w_o
    x2 = x1 + attn
    h = _layernorm(x2, axis=-1)
    h = h @ w_pw1
    a = h[..., :D].copy()
    b = h[..., D:].copy()
    h = a * _sigmoid(b)
    pad = K // 2
    hp = jnp.pad(h, ((0, 0), (pad, K - 1 - pad), (0, 0)))
    dc = jnp.zeros_like(h)
    for i in range(K):
        dc = dc + hp[:, i:i + T, :] * dw[i][None, None, :]
    flat = dc.reshape(-1, D)
    mu = flat.mean(0)
    var = ((flat - mu) ** 2).mean(0)
    dc = (dc - mu[None, None, :]) / jnp.sqrt(var[None, None, :] + 1e-05)
    h = _silu(dc) @ w_pw2
    x3 = x2 + h
    h = _layernorm(x3, axis=-1)
    h = _silu(h @ w_ff2_a) @ w_ff2_b
    x4 = x3 + 0.5 * h
    return _layernorm(x4, axis=-1)
```

```python
import functools
import numpy as np
import jax
import jax.numpy as jnp
from jax import lax
import jax.experimental.pallas as pl
import jax.experimental.pallas.tpu as pltpu

BF = jnp.bfloat16
F32 = jnp.float32
U32 = jnp.uint32
EPS = 1e-5
LOG2E = float(np.log2(np.e))
SAFE_BOUND = 60.0


def _div(i, n):
    return i // n if isinstance(i, int) else lax.div(i, jnp.int32(n))


def _ln(x):
    m = jnp.mean(x, axis=-1, keepdims=True)
    xc = x - m
    v = jnp.mean(xc * xc, axis=-1, keepdims=True)
    return xc * lax.rsqrt(v + EPS)


def _silu(a):
    hx = a * 0.5
    return hx * jnp.tanh(hx) + hx


def _pack(v):
    return pltpu.bitcast(v.astype(BF), U32)


def _unpack(v):
    return pltpu.bitcast(v, BF)


def _dot(a, b):
    return jnp.dot(a, b, preferred_element_type=F32)


def _dot_nt(a, b):
    return lax.dot_general(a, b, (((1,), (1,)), ((), ())), preferred_element_type=F32)


def _kernel(x_hbm, wa1_hbm, wb1_hbm, wq_hbm, wk_hbm, wv_hbm, wo_hbm, wp1_hbm, dw_hbm, wp2_hbm,
            wa2_hbm, wb2_hbm, out_hbm,
            xs, x1, hp, qp, g, dc, mbuf,
            wa1, wb1, wa2, wb2, wt0, wt1, mqk, wvo, wp1, wp2, dwb, dwf,
            sbuf, obuf, ubuf, stat_m, stat_v, bn,
            sem_w, sem_x, sem_o,
            *, B, T, D, F, K, TP, MA, TQ, KC):
    N = B * T
    NA = N // MA
    NQ = N // TQ
    QPB = T // TQ
    APB = T // MA
    NC = TP // KC
    GP = T + 8
    pad = K // 2

    w_copies = [
        pltpu.make_async_copy(wq_hbm, wt0, sem_w.at[0]),
        pltpu.make_async_copy(wk_hbm, wt1, sem_w.at[1]),
        pltpu.make_async_copy(wa1_hbm, wa1, sem_w.at[2]),
        pltpu.make_async_copy(wb1_hbm, wb1, sem_w.at[3]),
        pltpu.make_async_copy(dw_hbm, dwb, sem_w.at[4]),
        pltpu.make_async_copy(wp1_hbm, wp1, sem_w.at[5]),
        pltpu.make_async_copy(wp2_hbm, wp2, sem_w.at[6]),
        pltpu.make_async_copy(wa2_hbm, wa2, sem_w.at[7]),
        pltpu.make_async_copy(wb2_hbm, wb2, sem_w.at[8]),
    ]
    wv_copy = pltpu.make_async_copy(wv_hbm, wt0, sem_w.at[9])
    wo_copy = pltpu.make_async_copy(wo_hbm, wt1, sem_w.at[10])

    def x_copy(i):
        r = pl.multiple_of(i * MA, MA) if not isinstance(i, int) else i * MA
        return pltpu.make_async_copy(x_hbm.at[pl.ds(r, MA), :], xs.at[pl.ds(r, MA), :], sem_x.at[i])

    def o_copy(j):
        r = pl.multiple_of(j * MA, MA) if not isinstance(j, int) else j * MA
        return pltpu.make_async_copy(xs.at[pl.ds(r, MA), :], out_hbm.at[pl.ds(r, MA), :], sem_o.at[j])

    w_copies[0].start()
    w_copies[1].start()
    x_copy(0).start()
    w_copies[2].start()
    w_copies[3].start()
    for i in range(1, NA):
        x_copy(i).start()
    for c in w_copies[4:]:
        c.start()

    zero_rows = (TP - T) // 2
    for b in range(B):
        hp[pl.ds(b * (TP // 2) + T // 2, zero_rows), :] = jnp.zeros((zero_rows, D), U32)
    for b in range(B + 1):
        g[:, pl.ds(b * GP, 8), :] = jnp.zeros((D // 128, 8, 128), F32)
    mbuf[...] = jnp.zeros(mbuf.shape, F32)

    w_copies[0].wait()
    w_copies[1].wait()
    mqk[...] = _pack(_dot_nt(wt0[...], wt1[...]) * (LOG2E * float(D) ** -0.5))
    wv_copy.start()
    wo_copy.start()

    def mo(i, n):
        return i * n if isinstance(i, int) else pl.multiple_of(i * n, n)

    def ffa(xn, wa):
        a = _dot(xn, wa[...])
        sbuf[...] = _pack(_silu(a))

    def ffb(wb):
        return _dot(_unpack(sbuf[...]), wb[...])

    def a_first(i):
        x = xs[pl.ds(mo(i, MA), MA), :].astype(F32)
        ffa(_ln(x).astype(BF), wa1)

    def h_row(i):
        if T == TP:
            return mo(i, MA // 2)
        b = _div(i, APB)
        r = b * (TP // 2) + (i - b * APB) * (MA // 2)
        return r if isinstance(r, int) else pl.multiple_of(r, MA // 2)

    def a_second(i):
        y = ffb(wb1)
        x = xs[pl.ds(mo(i, MA), MA), :].astype(F32)
        x1v = x + 0.5 * y
        x1[pl.ds(mo(i, MA), MA), :] = x1v
        h = _pack(_ln(x1v))
        hp[pl.ds(h_row(i), MA // 2), :] = h
        return h

    def a_third(i, h, qmax):
        q = _dot(_unpack(h), _unpack(mqk[...]))
        qp[pl.ds(mo(i, MA // 2), MA // 2), :] = _pack(q)
        n2 = jnp.sum(q * q, axis=-1, keepdims=True)
        return jnp.maximum(qmax, jnp.max(n2.reshape(MA // 8, 8, 1), axis=0))

    x_copy(0).wait()
    w_copies[2].wait()
    a_first(0)
    w_copies[3].wait()
    wv_copy.wait()
    wo_copy.wait()
    wvo[...] = _pack(_dot(wt0[...], wt1[...]))

    def a_body(i, qmax):
        x_copy(i).wait()
        h = a_second(i - 1)
        a_first(i)
        return a_third(i - 1, h, qmax)

    qmax = lax.fori_loop(1, NA, a_body, jnp.zeros((8, 1), F32))
    h = a_second(NA - 1)
    qmax = a_third(NA - 1, h, qmax)
    for c in w_copies[4:]:
        c.wait()
    dwf[...] = dwb[...].astype(F32)

    bound2 = jnp.max(qmax) * (float(D) * 1.05)
    valid_tail = T - (NC - 1) * KC

    @pl.when(jnp.logical_not(bound2 <= SAFE_BOUND * SAFE_BOUND))
    def _():
        RT = 80 if T % 80 == 0 else 16
        def row_body(i, carry):
            b = _div(i * RT, T)
            q = _unpack(qp[pl.ds(pl.multiple_of(i * (RT // 2), RT // 2), RT // 2), :])
            def chunk_body(c, m):
                r = pl.multiple_of(b * (TP // 2) + c * (KC // 2), KC // 2)
                s = _dot_nt(q, _unpack(hp[pl.ds(r, KC // 2), :]))
                col = c * KC + lax.broadcasted_iota(jnp.int32, (RT, KC), 1)
                s = jnp.where(col < T, s, -jnp.inf)
                return jnp.maximum(m, jnp.max(s, axis=-1, keepdims=True))
            m = lax.fori_loop(0, NC, chunk_body, jnp.full((RT, 1), -jnp.inf, F32))
            mbuf[pl.ds(pl.multiple_of(i * RT, RT), RT), :] = jnp.broadcast_to(m, (RT, 128))
            return carry
        lax.fori_loop(0, N // RT, row_body, 0)

    def kv(b, c):
        r = b * (TP // 2) + c * (KC // 2)
        if not isinstance(r, int):
            r = pl.multiple_of(r, KC // 2)
        return _unpack(hp[pl.ds(r, KC // 2), :])

    def g_row(i):
        b = _div(i, QPB)
        r = 8 + b * GP + (i - b * QPB) * TQ
        return r if isinstance(r, int) else pl.multiple_of(r, 8)

    def attn_jobs(i):
        b = _div(i, QPB)
        st = {}

        def s_job(c):
            if 'q' not in st:
                st['q'] = _unpack(qp[pl.ds(mo(i, TQ // 2), TQ // 2), :])
            s = _dot_nt(st['q'], kv(b, c))
            m = mbuf[pl.ds(mo(i, TQ), TQ), :]
            p = jnp.exp2(s - jnp.concatenate([m] * (KC // 128), axis=1))
            if c == NC - 1 and valid_tail < KC:
                full = (valid_tail // 128) * 128
                pieces = [p[:, :full]] if full else []
                for s0 in range(full, KC, 128):
                    nv = valid_tail - s0
                    if nv <= 0:
                        pieces.append(jnp.zeros((TQ, 128), F32))
                    else:
                        lane = lax.broadcasted_iota(jnp.int32, (TQ, 128), 1)
                        pieces.append(jnp.where(lane < nv, p[:, s0:s0 + 128], 0.0))
                p = jnp.concatenate(pieces, axis=1)
            l = jnp.sum(p, axis=-1, keepdims=True)
            st['l'] = l if 'l' not in st else st['l'] + l
            st[('p', c)] = p.astype(BF)

        def pv_job(c):
            o = _dot(st.pop(('p', c)), kv(b, c))
            st['o'] = o if 'o' not in st else st['o'] + o

        def finish():
            obuf[...] = _pack(st['o'] * (1.0 / st['l']))

        return s_job, pv_job, finish

    def post_1(i):
        attn = _dot(_unpack(obuf[...]), _unpack(wvo[...]))
        x2 = x1[pl.ds(mo(i, TQ), TQ), :] + attn
        x1[pl.ds(mo(i, TQ), TQ), :] = x2
        return _ln(x2).astype(BF)

    def post_2(i, hn):
        u = _dot(hn, wp1[...])
        a = u[:, :D]
        bb = u[:, D:]
        ha = a * 0.5
        gv = ha * jnp.tanh(bb * 0.5) + ha
        r = g_row(i)
        for c4 in range(D // 128):
            g[c4, pl.ds(r, TQ), :] = gv[:, c4 * 128:(c4 + 1) * 128]

    def conv(i):
        r = g_row(i)
        for c4 in range(D // 128):
            acc = None
            for j in range(K):
                t = g[c4, pl.ds(r - pad + j, TQ), :] * dwf[pl.ds(j, 1), c4 * 128:(c4 + 1) * 128]
                acc = t if acc is None else acc + t
            dc[pl.ds(mo(i, TQ), TQ), c4 * 128:(c4 + 1) * 128] = acc
            mt = jnp.mean(acc, axis=0, keepdims=True)
            d = acc - mt
            stat_m[pl.ds(mo(i, 8), 8), c4 * 128:(c4 + 1) * 128] = jnp.broadcast_to(mt, (8, 128))
            stat_v[pl.ds(mo(i, 8), 8), c4 * 128:(c4 + 1) * 128] = jnp.sum((d * d).reshape(TQ // 8, 8, 128), axis=0)

    def attention(i, post=None):
        s_job, pv_job, finish = attn_jobs(i)
        if post is not None:
            hn = post_1(post)
        s_job(0)
        if post is not None:
            post_2(post, hn)
        for c in range(1, NC):
            s_job(c)
            pv_job(c - 1)
        pv_job(NC - 1)
        finish()

    attention(0)
    attention(1, post=0)

    def b_body(i, carry):
        conv_after = True
        attention(i, post=i - 1)
        conv(i - 2)
        return carry

    lax.fori_loop(2, NQ, b_body, 0)
    hn = post_1(NQ - 1)
    post_2(NQ - 1, hn)
    conv(NQ - 2)
    conv(NQ - 1)

    means = stat_m[...]
    mu = jnp.mean(means, axis=0, keepdims=True)
    dm = means - mu
    m2 = jnp.sum(stat_v[...], axis=0, keepdims=True) + float(TQ / 8) * jnp.sum(dm * dm, axis=0, keepdims=True)
    bn[pl.ds(0, 1), :] = mu
    bn[pl.ds(1, 1), :] = lax.rsqrt(m2 * (1.0 / N) + EPS)

    def d_pre(j):
        v = (dc[pl.ds(mo(j, MA), MA), :] - bn[pl.ds(0, 1), :]) * bn[pl.ds(1, 1), :]
        ubuf[...] = _pack(_silu(v))

    def d_first(j):
        x3 = x1[pl.ds(mo(j, MA), MA), :] + _dot(_unpack(ubuf[...]), wp2[...])
        x1[pl.ds(mo(j, MA), MA), :] = x3
        return _ln(x3).astype(BF)

    def d_last(j, y):
        x4 = x1[pl.ds(mo(j, MA), MA), :] + 0.5 * y
        xs[pl.ds(mo(j, MA), MA), :] = _ln(x4).astype(BF)
        o_copy(j).start()

    d_pre(0)
    hn = d_first(0)
    ffa(hn, wa2)
    d_pre(1)

    def d_body(j, carry):
        hn = d_first(j)
        y = ffb(wb2)
        d_last(j - 1, y)
        ffa(hn, wa2)
        d_pre(jnp.minimum(j + 1, NA - 1))
        return carry

    lax.fori_loop(1, NA, d_body, 0)
    d_last(NA - 1, ffb(wb2))
    for j in range(NA):
        o_copy(j).wait()


def conformer(x, w_ff1_a, w_ff1_b, w_q, w_k, w_v, w_o, w_pw1, dw, w_pw2, w_ff2_a, w_ff2_b,
              *, MA=400, TQ=400, KC=512, interpret=False, vmem_mb=110):
    B, T, D = x.shape
    F = w_ff1_a.shape[1]
    K = dw.shape[0]
    N = B * T
    TP = -(-T // KC) * KC
    NA = N // MA
    NQ = N // TQ
    kern = functools.partial(_kernel, B=B, T=T, D=D, F=F, K=K, TP=TP, MA=MA, TQ=TQ, KC=KC)
    hbm = pl.BlockSpec(memory_space=pl.ANY)
    V = pltpu.VMEM
    scratch = [
        V((N, D), BF),
        V((N, D), F32),
        V((B * TP // 2, D), U32),
        V((N // 2, D), U32),
        V((D // 128, B * (T + 8) + 8, 128), F32),
        V((N, D), F32),
        V((N, 128), F32),
        V((D, F), BF), V((F, D), BF), V((D, F), BF), V((F, D), BF),
        V((D, D), BF), V((D, D), BF),
        V((D // 2, D), U32), V((D // 2, D), U32),
        V((D, 2 * D), BF), V((D, D), BF),
        V((K, D), BF), V((K, D), F32),
        V((MA // 2, F), U32),
        V((TQ // 2, D), U32),
        V((MA // 2, D), U32),
        V((NQ * 8, D), F32), V((NQ * 8, D), F32), V((8, D), F32),
        pltpu.SemaphoreType.DMA((11,)),
        pltpu.SemaphoreType.DMA((NA,)),
        pltpu.SemaphoreType.DMA((NA,)),
    ]
    out = pl.pallas_call(
        kern,
        out_shape=jax.ShapeDtypeStruct((N, D), x.dtype),
        in_specs=[hbm] * 12,
        out_specs=hbm,
        scratch_shapes=scratch,
        compiler_params=pltpu.CompilerParams(vmem_limit_bytes=vmem_mb * 1024 * 1024),
        interpret=interpret,
    )(x.reshape(N, D), w_ff1_a, w_ff1_b, w_q, w_k, w_v, w_o, w_pw1, dw, w_pw2, w_ff2_a, w_ff2_b)
    return out.reshape(B, T, D)


@jax.jit
def pallas_standalone__conformer_family_conformer__speech_kernel(
    x: jax.Array,
    w_ff1_a: jax.Array,
    w_ff1_b: jax.Array,
    w_q: jax.Array,
    w_k: jax.Array,
    w_v: jax.Array,
    w_o: jax.Array,
    w_pw1: jax.Array,
    dw: jax.Array,
    w_pw2: jax.Array,
    w_ff2_a: jax.Array,
    w_ff2_b: jax.Array,
):
    return conformer(x, w_ff1_a, w_ff1_b, w_q, w_k, w_v, w_o, w_pw1, dw, w_pw2, w_ff2_a, w_ff2_b)
```

```python
import functools
import numpy as np
import jax
import jax.numpy as jnp
from jax import lax
import jax.experimental.pallas as pl
import jax.experimental.pallas.tpu as pltpu

BF = jnp.bfloat16
F32 = jnp.float32
U32 = jnp.uint32
EPS = 1e-5
LOG2E = float(np.log2(np.e))
SAFE_BOUND = 60.0


def _div(i, n):
    return i // n if isinstance(i, int) else lax.div(i, jnp.int32(n))


def _ln(x):
    m = jnp.mean(x, axis=-1, keepdims=True)
    xc = x - m
    v = jnp.mean(xc * xc, axis=-1, keepdims=True)
    return xc * lax.rsqrt(v + EPS)


def _silu(a):
    hx = a * 0.5
    return hx * jnp.tanh(hx) + hx


def _pack(v):
    return pltpu.bitcast(v.astype(BF), U32)


def _unpack(v):
    return pltpu.bitcast(v, BF)


def _dot(a, b):
    return jnp.dot(a, b, preferred_element_type=F32)


def _dot_nt(a, b):
    return lax.dot_general(a, b, (((1,), (1,)), ((), ())), preferred_element_type=F32)


def _kernel(x_hbm, wa1_hbm, wb1_hbm, wq_hbm, wk_hbm, wv_hbm, wo_hbm, wp1_hbm, dw_hbm, wp2_hbm,
            wa2_hbm, wb2_hbm, out_hbm,
            xs, x1, hp, qp, g, dc, mbuf,
            ta1, tb1, ta2, tb2, wa_s, wb_s, wt0, wt1, mqk, wvo, wp1, wp2, dwb, dwf,
            sbuf, obuf, ubuf, stat_c, stat_m, stat_v, bn,
            sem_w, sem_x, sem_o,
            *, B, T, D, F, K, TP, MA, TQ, KC, RG, CVPOS, scopes):
    import contextlib
    def scope(n):
        return jax.named_scope(n) if scopes else contextlib.nullcontext()
    N = B * T
    NA = N // MA
    NQ = N // TQ
    QPB = T // TQ
    APB = T // MA
    NC = TP // KC
    GP = T + 8
    pad = K // 2
    GJ = B * GP + 8

    w_copies = [
        pltpu.make_async_copy(wq_hbm, wt0, sem_w.at[0]),
        pltpu.make_async_copy(wk_hbm, wt1, sem_w.at[1]),
        pltpu.make_async_copy(wa1_hbm, wa_s, sem_w.at[2]),
        pltpu.make_async_copy(wb1_hbm, wb_s, sem_w.at[3]),
        pltpu.make_async_copy(dw_hbm, dwb, sem_w.at[4]),
        pltpu.make_async_copy(wp1_hbm, wp1, sem_w.at[5]),
        pltpu.make_async_copy(wp2_hbm, wp2, sem_w.at[6]),
    ]
    wa2_copy = pltpu.make_async_copy(wa2_hbm, wa_s, sem_w.at[7])
    wb2_copy = pltpu.make_async_copy(wb2_hbm, wb_s, sem_w.at[8])
    wv_copy = pltpu.make_async_copy(wv_hbm, wt0, sem_w.at[9])
    wo_copy = pltpu.make_async_copy(wo_hbm, wt1, sem_w.at[10])

    def x_copy(i):
        r = pl.multiple_of(i * MA, MA) if not isinstance(i, int) else i * MA
        return pltpu.make_async_copy(x_hbm.at[pl.ds(r, MA), :], xs.at[pl.ds(r, MA), :], sem_x.at[i])

    def o_copy(j):
        r = pl.multiple_of(j * MA, MA) if not isinstance(j, int) else j * MA
        return pltpu.make_async_copy(xs.at[pl.ds(r, MA), :], out_hbm.at[pl.ds(r, MA), :], sem_o.at[j])

    w_copies[0].start()
    w_copies[1].start()
    x_copy(0).start()
    w_copies[2].start()
    w_copies[3].start()
    for i in range(1, NA):
        x_copy(i).start()
    for c in w_copies[4:]:
        c.start()

    zero_rows = (TP - T) // 2
    hp[pl.ds(B * T // 2, zero_rows), :] = jnp.zeros((zero_rows, D), U32)
    for b in range(B + 1):
        g[:, pl.ds(b * GP, 8), :] = jnp.zeros((D // 128, 8, 128), F32)
    mbuf[...] = jnp.zeros(mbuf.shape, F32)

    w_copies[0].wait()
    w_copies[1].wait()
    mqk[...] = _pack(_dot_nt(wt0[...], wt1[...]) * (LOG2E * float(D) ** -0.5))
    wv_copy.start()
    wo_copy.start()

    def mo(i, n):
        return i * n if isinstance(i, int) else pl.multiple_of(i * n, n)

    R = MA // 2
    HD, HF = D // 2, F // 2

    def lhs7(a11, a12, a21, a22):
        return [a11 + a22, a21 + a22, a11, a22, a11 + a12, a21 - a11, a12 - a22]

    def rhs7(b11, b12, b21, b22):
        return [b11 + b22, b11, b12 - b22, b21 - b11, b22, b11 + b12, b21 + b22]

    def comb(m):
        return (m[0] + m[3] - m[4] + m[6], m[2] + m[4], m[1] + m[3], m[0] - m[1] + m[2] + m[5])

    def prep_strassen(w_ref, t_ref, kk, nn, scale, cw):
        hk, hn = kk // 2, nn // 2
        for c0 in range(0, hn, cw):
            blk = [w_ref[r0:r0 + hk, cc:cc + cw].astype(F32) * scale
                   for r0 in (0, hk) for cc in (c0, hn + c0)]
            for p, t in enumerate(rhs7(*blk)):
                t_ref[p * hk // 2:(p + 1) * hk // 2, c0:c0 + cw] = _pack(t)

    SL = 256

    def ffa(xn, ta):
        S = [t.astype(BF) for t in lhs7(xn[:R, :HD], xn[:R, HD:], xn[R:, :HD], xn[R:, HD:])]
        for c0 in range(0, HF, SL):
            cs = slice(c0, c0 + SL)
            ms = [_dot(S[p], _unpack(ta[p * HD // 2:(p + 1) * HD // 2, cs])) for p in range(7)]
            act = [hx * jnp.tanh(hx) + hx for hx in comb(ms)]
            for p, t in enumerate(lhs7(*act)):
                sbuf[p * R // 2:(p + 1) * R // 2, cs] = _pack(t)

    def ffb_blocks(tb):
        ms = [_dot(_unpack(sbuf[p * R // 2:(p + 1) * R // 2, :]),
                   _unpack(tb[p * HF // 2:(p + 1) * HF // 2, :])) for p in range(7)]
        return comb(ms)

    def ffb(tb):
        y11, y12, y21, y22 = ffb_blocks(tb)
        return jnp.concatenate([jnp.concatenate([y11, y12], 1), jnp.concatenate([y21, y22], 1)], 0)

    def a_first(i):
        x = xs[pl.ds(mo(i, MA), MA), :].astype(F32)
        ffa(_ln(x), ta1)

    def a_second(i):
        y = ffb(tb1)
        x = xs[pl.ds(mo(i, MA), MA), :].astype(F32)
        x1v = x + y
        x1[pl.ds(mo(i, MA), MA), :] = x1v
        h = _pack(_ln(x1v))
        hp[pl.ds(mo(i, MA // 2), MA // 2), :] = h
        return h

    def a_third(i, h, qmax):
        q = _dot(_unpack(h), _unpack(mqk[...]))
        qp[pl.ds(mo(i, MA // 2), MA // 2), :] = _pack(q)
        n2 = jnp.sum(q * q, axis=-1, keepdims=True)
        return jnp.maximum(qmax, jnp.max(n2.reshape(MA // 8, 8, 1), axis=0))

    w_copies[2].wait()
    prep_strassen(wa_s, ta1, D, F, 0.5, 256)
    wa2_copy.start()
    x_copy(0).wait()
    a_first(0)
    w_copies[3].wait()
    prep_strassen(wb_s, tb1, F, D, 0.5, 128)
    wb2_copy.start()

    def a_body(i, qmax):
        x_copy(i).wait()
        h = a_second(i - 1)
        a_first(i)
        return a_third(i - 1, h, qmax)

    with scope('loopA'):
        qmax = lax.fori_loop(1, NA, a_body, jnp.zeros((8, 1), F32))
    h = a_second(NA - 1)
    qmax = a_third(NA - 1, h, qmax)
    for c in w_copies[4:]:
        c.wait()
    wv_copy.wait()
    wo_copy.wait()
    wvo[...] = _pack(_dot(wt0[...], wt1[...]))
    wa2_copy.wait()
    wb2_copy.wait()
    prep_strassen(wa_s, ta2, D, F, 0.5, 256)
    prep_strassen(wb_s, tb2, F, D, 0.5, 128)
    dwf[...] = dwb[...].astype(F32)

    bound2 = jnp.max(qmax) * (float(D) * 1.05)
    valid_tail = T - (NC - 1) * KC

    @pl.when(jnp.logical_not(bound2 <= SAFE_BOUND * SAFE_BOUND))
    def _():
        RT = 80 if T % 80 == 0 else 16
        def row_body(i, carry):
            b = _div(i * RT, T)
            q = _unpack(qp[pl.ds(pl.multiple_of(i * (RT // 2), RT // 2), RT // 2), :])
            def chunk_body(c, m):
                r = pl.multiple_of(b * (T // 2) + c * (KC // 2), 8)
                s = _dot_nt(q, _unpack(hp[pl.ds(r, KC // 2), :]))
                col = c * KC + lax.broadcasted_iota(jnp.int32, (RT, KC), 1)
                s = jnp.where(col < T, s, -jnp.inf)
                return jnp.maximum(m, jnp.max(s, axis=-1, keepdims=True))
            m = lax.fori_loop(0, NC, chunk_body, jnp.full((RT, 1), -jnp.inf, F32))
            mbuf[pl.ds(pl.multiple_of(i * RT, RT), RT), :] = jnp.broadcast_to(m, (RT, 128))
            return carry
        lax.fori_loop(0, N // RT, row_body, 0)

    def kv(b, c):
        r = b * (T // 2) + c * (KC // 2)
        if not isinstance(r, int):
            r = pl.multiple_of(r, 8)
        return _unpack(hp[pl.ds(r, KC // 2), :])

    def g_row(i):
        b = _div(i, QPB)
        r = 8 + b * GP + (i - b * QPB) * TQ
        return r if isinstance(r, int) else pl.multiple_of(r, 8)

    def attn_jobs(i):
        b = _div(i, QPB)
        st = {}

        def s_job(c):
            if 'q' not in st:
                st['q'] = _unpack(qp[pl.ds(mo(i, TQ // 2), TQ // 2), :])
            s = _dot_nt(st['q'], kv(b, c))
            m = mbuf[pl.ds(mo(i, TQ), TQ), :]
            p = jnp.exp2(s - jnp.concatenate([m] * (KC // 128), axis=1))
            if c == NC - 1 and valid_tail < KC:
                full = (valid_tail // 128) * 128
                pieces = [p[:, :full]] if full else []
                for s0 in range(full, KC, 128):
                    nv = valid_tail - s0
                    if nv <= 0:
                        pieces.append(jnp.zeros((TQ, 128), F32))
                    else:
                        lane = lax.broadcasted_iota(jnp.int32, (TQ, 128), 1)
                        pieces.append(jnp.where(lane < nv, p[:, s0:s0 + 128], 0.0))
                p = jnp.concatenate(pieces, axis=1)
            l = jnp.sum(p, axis=-1, keepdims=True)
            st['l'] = l if 'l' not in st else st['l'] + l
            st[('p', c)] = p.astype(BF)
            st[('pf', c)] = p

        def pin(c, i_dyn, pieces):
            p = st.pop(('pf', c))
            n = len(pieces)
            for t, piece in enumerate(pieces):
                nt = t % (KC // 128)
                j = (t * (TQ // 8)) // n
                jr = GJ + 8 * (i_dyn & 1)
                g[0, pl.ds(pl.multiple_of(jr, 8), 8), :] = p[j * 8:(j + 1) * 8, nt * 128:(nt + 1) * 128]
                piece()
        s_job.pin = pin

        def pv_job(c):
            o = _dot(st.pop(('p', c)), kv(b, c))
            st['o'] = o if 'o' not in st else st['o'] + o

        def finish():
            obuf[...] = _pack(st['o'] * (1.0 / st['l']))

        return s_job, pv_job, finish

    def post_1(i):
        attn = _dot(_unpack(obuf[...]), _unpack(wvo[...]))
        x2 = x1[pl.ds(mo(i, TQ), TQ), :] + attn
        x1[pl.ds(mo(i, TQ), TQ), :] = x2
        return _ln(x2).astype(BF)

    def post_2(i, hn):
        u = _dot(hn, wp1[...])
        a = u[:, :D]
        bb = u[:, D:]
        ha = a * 0.5
        gv = ha * jnp.tanh(bb * 0.5) + ha
        r = g_row(i)
        for c4 in range(D // 128):
            g[c4, pl.ds(r, TQ), :] = gv[:, c4 * 128:(c4 + 1) * 128]

    def tree_sum(xs_):
        xs_ = list(xs_)
        while len(xs_) > 1:
            nxt = [xs_[k] + xs_[k + 1] for k in range(0, len(xs_) - 1, 2)]
            if len(xs_) % 2:
                nxt.append(xs_[-1])
            xs_ = nxt
        return xs_[0]

    def conv_pieces(i):
        r = g_row(i)
        pieces = []
        for c4 in range(D // 128):
            cs = slice(c4 * 128, (c4 + 1) * 128)
            stt = {}
            for k in range(TQ // RG):
                def piece(c4=c4, cs=cs, k=k, stt=stt):
                    if k == 0:
                        stt['w'] = [dwf[pl.ds(j, 1), cs] for j in range(K)]
                    w = stt['w']
                    acc = None
                    for j in range(K):
                        t = g[c4, pl.ds(r + k * RG - pad + j, RG), :] * w[j]
                        acc = t if acc is None else acc + t
                    dc[pl.ds(mo(i, TQ) + k * RG, RG), cs] = acc
                    if k == 0:
                        stt['shift'] = acc[0:1]
                    d = acc - stt['shift']
                    d2 = d * d
                    for u in range(RG // 8):
                        du = d[u * 8:(u + 1) * 8]
                        d2u = d2[u * 8:(u + 1) * 8]
                        stt['s1'] = du if 's1' not in stt else stt['s1'] + du
                        stt['s2'] = d2u if 's2' not in stt else stt['s2'] + d2u
                    if k == TQ // RG - 1:
                        stat_c[pl.ds(mo(i, 8), 8), cs] = jnp.broadcast_to(stt['shift'], (8, 128))
                        stat_m[pl.ds(mo(i, 8), 8), cs] = stt['s1']
                        stat_v[pl.ds(mo(i, 8), 8), cs] = stt['s2']
                pieces.append(piece)
        return pieces

    def conv(i):
        for p_ in conv_pieces(i):
            p_()

    def attention(i, post=None, cv=None):
        s_job, pv_job, finish = attn_jobs(i)
        pieces = conv_pieces(cv) if cv is not None else []
        if post is not None:
            hn = post_1(post)
        s_job(0)
        if post is not None:
            post_2(post, hn)
        if CVPOS == 0:
            for p_ in pieces:
                p_()
        elif CVPOS == 3:
            s_job.pin(0, i, pieces[:len(pieces) // NC])
        for c in range(1, NC):
            s_job(c)
            if CVPOS == 3:
                n = len(pieces)
                s_job.pin(c, i, pieces[c * n // NC:(c + 1) * n // NC])
            pv_job(c - 1)
        if CVPOS == 2:
            for p_ in pieces:
                p_()
        pv_job(NC - 1)
        finish()

    attention(0)
    attention(1, post=0)

    def b_body(i, carry):
        attention(i, post=i - 1, cv=i - 2)
        return carry

    with scope('loopB'):
        lax.fori_loop(2, NQ, b_body, 0)
    hn = post_1(NQ - 1)
    post_2(NQ - 1, hn)
    conv(NQ - 2)
    conv(NQ - 1)

    sh = stat_c[...].reshape(NQ, 8, D)
    s1 = jnp.sum(stat_m[...].reshape(NQ, 8, D), axis=1, keepdims=True)
    s2 = jnp.sum(stat_v[...].reshape(NQ, 8, D), axis=1, keepdims=True)
    tm = sh[:, 0:1, :] + s1 * (1.0 / TQ)
    mu = jnp.mean(tm, axis=0)
    dm = tm - mu
    m2 = jnp.sum(s2 - s1 * s1 * (1.0 / TQ) + float(TQ) * dm * dm, axis=0)
    bn[pl.ds(0, 1), :] = mu
    bn[pl.ds(1, 1), :] = lax.rsqrt(m2 * (1.0 / N) + EPS)

    def d_pre(j):
        v = (dc[pl.ds(mo(j, MA), MA), :] - bn[pl.ds(0, 1), :]) * bn[pl.ds(1, 1), :]
        ubuf[...] = _pack(_silu(v))

    def d_first(j):
        x3 = x1[pl.ds(mo(j, MA), MA), :] + _dot(_unpack(ubuf[...]), wp2[...])
        x1[pl.ds(mo(j, MA), MA), :] = x3
        return _ln(x3)

    def d_last(j, y):
        x4 = x1[pl.ds(mo(j, MA), MA), :] + y
        xs[pl.ds(mo(j, MA), MA), :] = _ln(x4).astype(BF)
        o_copy(j).start()

    d_pre(0)
    hn = d_first(0)
    ffa(hn, ta2)
    d_pre(1)

    def d_body(j, carry):
        hn = d_first(j)
        y = ffb(tb2)
        d_last(j - 1, y)
        ffa(hn, ta2)
        d_pre(jnp.minimum(j + 1, NA - 1))
        return carry

    with scope('loopD'):
        lax.fori_loop(1, NA, d_body, 0)
    d_last(NA - 1, ffb(tb2))
    for j in range(NA):
        o_copy(j).wait()


def conformer(x, w_ff1_a, w_ff1_b, w_q, w_k, w_v, w_o, w_pw1, dw, w_pw2, w_ff2_a, w_ff2_b,
              *, MA=320, TQ=400, KC=512, RG=8, CVPOS=3, scopes=0, interpret=False, vmem_mb=110, lp=0, ev=0):
    B, T, D = x.shape
    F = w_ff1_a.shape[1]
    K = dw.shape[0]
    N = B * T
    TP = -(-T // KC) * KC
    NA = N // MA
    NQ = N // TQ
    kern = functools.partial(_kernel, B=B, T=T, D=D, F=F, K=K, TP=TP, MA=MA, TQ=TQ, KC=KC, RG=RG, CVPOS=CVPOS, scopes=scopes)
    flags = {}
    if lp: flags['XLA_TPU_FORCE_LP_LLO_SCHEDULER'] = True
    if ev: flags['XLA_TPU_EVENLY_DISTRIBUTE_CRITICAL_NODES'] = True
    hbm = pl.BlockSpec(memory_space=pl.ANY)
    V = pltpu.VMEM
    scratch = [
        V((N, D), BF),
        V((N, D), F32),
        V(((B - 1) * T // 2 + TP // 2, D), U32),
        V((N // 2, D), U32),
        V((D // 128, B * (T + 8) + 8 + 16, 128), F32),
        V((N, D), F32),
        V((N, 128), F32),
        V((7 * D // 4, F // 2), U32), V((7 * F // 4, D // 2), U32),
        V((7 * D // 4, F // 2), U32), V((7 * F // 4, D // 2), U32),
        V((D, F), BF), V((F, D), BF),
        V((D, D), BF), V((D, D), BF),
        V((D // 2, D), U32), V((D // 2, D), U32),
        V((D, 2 * D), BF), V((D, D), BF),
        V((K, D), BF), V((K, D), F32),
        V((7 * MA // 4, F // 2), U32),
        V((TQ // 2, D), U32),
        V((MA // 2, D), U32),
        V((NQ * 8, D), F32), V((NQ * 8, D), F32), V((NQ * 8, D), F32), V((8, D), F32),
        pltpu.SemaphoreType.DMA((11,)),
        pltpu.SemaphoreType.DMA((NA,)),
        pltpu.SemaphoreType.DMA((NA,)),
    ]
    out = pl.pallas_call(
        kern,
        out_shape=jax.ShapeDtypeStruct((N, D), x.dtype),
        in_specs=[hbm] * 12,
        out_specs=hbm,
        scratch_shapes=scratch,
        compiler_params=pltpu.CompilerParams(vmem_limit_bytes=vmem_mb * 1024 * 1024, flags=flags),
        interpret=interpret,
    )(x.reshape(N, D), w_ff1_a, w_ff1_b, w_q, w_k, w_v, w_o, w_pw1, dw, w_pw2, w_ff2_a, w_ff2_b)
    return out.reshape(B, T, D)


@jax.jit
def pallas_standalone__conformer_family_conformer__speech_kernel(
    x: jax.Array,
    w_ff1_a: jax.Array,
    w_ff1_b: jax.Array,
    w_q: jax.Array,
    w_k: jax.Array,
    w_v: jax.Array,
    w_o: jax.Array,
    w_pw1: jax.Array,
    dw: jax.Array,
    w_pw2: jax.Array,
    w_ff2_a: jax.Array,
    w_ff2_b: jax.Array,
):
    return conformer(x, w_ff1_a, w_ff1_b, w_q, w_k, w_v, w_o, w_pw1, dw, w_pw2, w_ff2_a, w_ff2_b)
```

```python
import contextlib
import functools

import numpy as np
import jax
import jax.numpy as jnp
from jax import lax
import jax.experimental.pallas as pl
import jax.experimental.pallas.tpu as pltpu

BF = jnp.bfloat16
F32 = jnp.float32
U32 = jnp.uint32
EPS = 1e-5
LOG2E = float(np.log2(np.e))
SAFE_BOUND = 60.0


def _div(i, n):
    return i // n if isinstance(i, int) else lax.div(i, jnp.int32(n))


def _mo(v, n):
    return v if isinstance(v, int) else pl.multiple_of(v, n)


def _ln(x):
    m = jnp.mean(x, axis=-1, keepdims=True)
    xc = x - m
    v = jnp.mean(xc * xc, axis=-1, keepdims=True)
    return xc * lax.rsqrt(v + EPS)


def _pack(v):
    return pltpu.bitcast(v.astype(BF), U32)


def _unpack(v):
    return pltpu.bitcast(v, BF)


def _dot(a, b):
    return jnp.dot(a, b, preferred_element_type=F32)


def _dot_nt(a, b):
    return lax.dot_general(a, b, (((1,), (1,)), ((), ())), preferred_element_type=F32)


def _lhs7(a11, a12, a21, a22):
    return [a11 + a22, a21 + a22, a11, a22, a11 + a12, a21 - a11, a12 - a22]


def _rhs7(b11, b12, b21, b22):
    return [b11 + b22, b11, b12 - b22, b21 - b11, b22, b11 + b12, b21 + b22]


def _comb(m):
    return (m[0] + m[3] - m[4] + m[6], m[2] + m[4], m[1] + m[3], m[0] - m[1] + m[2] + m[5])


def _quads(x):
    r, h = x.shape[0] // 2, x.shape[1] // 2
    return x[:r, :h], x[:r, h:], x[r:, :h], x[r:, h:]


def _join(c11, c12, c21, c22):
    return jnp.concatenate([jnp.concatenate([c11, c12], 1), jnp.concatenate([c21, c22], 1)], 0)


def _kernel(x_hbm, wa1_hbm, wb1_hbm, wq_hbm, wk_hbm, wv_hbm, wo_hbm, wp1_hbm, dw_hbm, wp2_hbm,
            wa2_hbm, wb2_hbm, out_hbm,
            xs, x1, hv, kx, q7, g, dc,
            ta1, tb1, ta2, tb2, wa_s, wb_s, wt0, wt1, wp1_s, wp2_s, tqk, tvo, tp1, tp2, dwb, dwf,
            sbuf, pbuf, obuf, ubuf, stat_c, stat_1, stat_2, bn,
            sem_w, sem_x, sem_o,
            *, B, T, D, F, K, U, KH, KS, UA, UB, UD, CG, CMODE, scopes):
    def scope(n):
        return jax.named_scope(n) if scopes else contextlib.nullcontext()

    N = B * T
    NU = N // U
    UPB = T // U
    R = U // 2
    RP = R // 2
    HD, HF = D // 2, F // 2
    NS = KH // KS
    KV = UPB * R
    KHP = KH // 2
    GP = T + 8
    GJ = B * GP + 8
    pad = K // 2
    NC4 = D // 128

    def wcopy(src, dst, k):
        return pltpu.make_async_copy(src, dst, sem_w.at[k])

    c_wq, c_wk = wcopy(wq_hbm, wt0, 0), wcopy(wk_hbm, wt1, 1)
    c_wa1, c_wb1 = wcopy(wa1_hbm, wa_s, 2), wcopy(wb1_hbm, wb_s, 3)
    c_dw, c_wp1, c_wp2 = wcopy(dw_hbm, dwb, 4), wcopy(wp1_hbm, wp1_s, 5), wcopy(wp2_hbm, wp2_s, 6)
    c_wa2, c_wb2 = wcopy(wa2_hbm, wa_s, 7), wcopy(wb2_hbm, wb_s, 8)
    c_wv, c_wo = wcopy(wv_hbm, wt0, 9), wcopy(wo_hbm, wt1, 10)

    XC = 2 * U
    NX = N // XC

    def x_copy(i):
        r = _mo(i * XC, XC)
        return pltpu.make_async_copy(x_hbm.at[pl.ds(r, XC), :], xs.at[pl.ds(r, XC), :], sem_x.at[i])

    def o_copy(j):
        r = _mo(j * U, U)
        return pltpu.make_async_copy(xs.at[pl.ds(r, U), :], out_hbm.at[pl.ds(r, U), :], sem_o.at[j])

    c_wq.start()
    c_wk.start()
    x_copy(0).start()
    c_wa1.start()
    x_copy(1).start()
    c_wb1.start()
    for i in range(2, NX):
        x_copy(i).start()
    for c in (c_dw, c_wp1, c_wp2):
        c.start()

    for b in range(B):
        for s in range(2):
            r0 = (2 * b + s) * KHP + KV // 2
            hv[pl.ds(r0, KHP - KV // 2), :] = jnp.zeros((KHP - KV // 2, D), U32)
        r0 = b * KHP + KV // 2
        kx[pl.ds(r0, KHP - KV // 2), :] = jnp.zeros((KHP - KV // 2, 5 * HD), U32)
    for b in range(B + 1):
        g[:, pl.ds(b * GP, 8), :] = jnp.zeros((NC4, 8, 128), F32)
    g[:, pl.ds(8 + UB * U, 8), :] = jnp.zeros((NC4, 8, 128), F32)

    def store7(t_ref, blocks, scale=None):
        hk = blocks[0].shape[0]
        for p, t in enumerate(_rhs7(*blocks)):
            t_ref[p * hk // 2:(p + 1) * hk // 2, :] = _pack(t if scale is None else t * scale)

    def prep_weight(w_ref, t_ref, scale, cw):
        kk, nn = w_ref.shape
        hk, hn = kk // 2, nn // 2
        for c0 in range(0, hn, cw):
            blk = [w_ref[r0:r0 + hk, cc:cc + cw].astype(F32) * scale
                   for r0 in (0, hk) for cc in (c0, hn + c0)]
            for p, t in enumerate(_rhs7(*blk)):
                t_ref[p * hk // 2:(p + 1) * hk // 2, c0:c0 + cw] = _pack(t)

    c_wq.wait()
    c_wk.wait()
    store7(tqk, _quads(_dot_nt(wt0[...], wt1[...])), LOG2E * float(D) ** -0.5)
    c_wv.start()
    c_wo.start()

    def mm7(ops, t_ref, cs=slice(None)):
        hk = t_ref.shape[0] // 7
        return [_dot(ops[p], _unpack(t_ref[p * hk:(p + 1) * hk, cs])) for p in range(7)]

    def load7(ref, r0=0):
        return [_unpack(ref[pl.ds(r0 + p * RP, RP), :]) for p in range(7)]

    def store_lhs7(ref, r0, blocks, cs=slice(None)):
        for p, t in enumerate(_lhs7(*blocks)):
            ref[pl.ds(r0 + p * RP, RP), cs] = _pack(t)

    SL = 256
    NSL = HF // SL

    def ffa_prep(xn):
        return [t.astype(BF) for t in _lhs7(*_quads(xn))]

    def ffa_slab(ops, ta, s):
        cs = slice(s * SL, (s + 1) * SL)
        act = [hx * jnp.tanh(hx) + hx for hx in _comb(mm7(ops, ta, cs))]
        store_lhs7(sbuf, 0, act, cs)

    def ffb(tb):
        return _join(*_comb(mm7(load7(sbuf), tb)))

    def a_prep(i):
        return ffa_prep(_ln(xs[pl.ds(_mo(i * U, U), U), :].astype(F32)))

    def a_second(i):
        y = ffb(tb1)
        r = _mo(i * U, U)
        x1v = xs[pl.ds(r, U), :].astype(F32) + y
        x1[pl.ds(r, U), :] = x1v
        h = _ln(x1v)
        b = _div(i, UPB)
        u = i - b * UPB
        rk = _mo(b * KHP + u * RP, 8)
        rv = _mo(2 * b * KHP + u * RP, 8)
        hv[pl.ds(rv, RP), :] = _pack(h[:R])
        hv[pl.ds(rv + KHP, RP), :] = _pack(h[R:])
        h11, h12, h21, h22 = _quads(h)
        for n, t in enumerate((h11 + h22, h21 - h22, h12 - h11, h11 + h21, h12 + h22)):
            kx[pl.ds(rk, RP), n * HD:(n + 1) * HD] = _pack(t)
        return [t.astype(BF) for t in _lhs7(h11, h12, h21, h22)]

    def a_third(i, hops, qmax):
        c = _comb(mm7(hops, tqk))
        store_lhs7(q7, _mo(i * 7 * RP, 8), c)
        n_top = jnp.sum(c[0] * c[0] + c[1] * c[1], axis=-1, keepdims=True)
        n_bot = jnp.sum(c[2] * c[2] + c[3] * c[3], axis=-1, keepdims=True)
        n2 = jnp.maximum(n_top, n_bot)
        return jnp.maximum(qmax, jnp.max(n2.reshape(R // 8, 8, 1), axis=0))

    c_wa1.wait()
    prep_weight(wa_s, ta1, 0.5, 256)
    c_wa2.start()
    x_copy(0).wait()
    ops = a_prep(0)
    for s in range(NSL):
        ffa_slab(ops, ta1, s)
    c_wb1.wait()
    prep_weight(wb_s, tb1, 0.5, 128)
    c_wb2.start()

    def a_step(i, qmax):
        hops = a_second(i - 1)
        ops = a_prep(i)
        ffa_slab(ops, ta1, 0)
        ffa_slab(ops, ta1, 1)
        qmax = a_third(i - 1, hops, qmax)
        for s in range(2, NSL):
            ffa_slab(ops, ta1, s)
        return qmax

    lead = (NU - 1) % UA
    qmax = jnp.zeros((8, 1), F32)
    for i in range(1, 1 + lead):
        if i % 2 == 0:
            x_copy(i // 2).wait()
        qmax = a_step(i, qmax)

    def a_body(k, qmax):
        for t in range(UA):
            i = 1 + lead + k * UA + t
            if (1 + lead + t) % 2 == 0 and UA % 2 == 0:
                x_copy(_div(i, 2)).wait()
            elif UA % 2:
                @pl.when(lax.rem(i, 2) == 0)
                def _():
                    x_copy(_div(i, 2)).wait()
            qmax = a_step(i, qmax)
        return qmax

    with scope('loopA'):
        qmax = lax.fori_loop(0, (NU - 1 - lead) // UA, a_body, qmax)
    hops = a_second(NU - 1)
    qmax = a_third(NU - 1, hops, qmax)
    for c in (c_dw, c_wp1, c_wp2, c_wv, c_wo, c_wa2, c_wb2):
        c.wait()
    dwf[...] = dwb[...].astype(F32)
    store7(tvo, _quads(_dot(wt0[...], wt1[...])))
    prep_weight(wp1_s, tp1, 1.0, 256)
    prep_weight(wp2_s, tp2, 1.0, 256)
    prep_weight(wa_s, ta2, 0.5, 256)
    prep_weight(wb_s, tb2, 0.5, 128)

    dc[:, 0:128] = jnp.zeros((N, 128), F32)

    def k_ops(b, s):
        rk = _mo(b * KHP + s * (KS // 2), 8)
        rv = _mo(2 * b * KHP + s * (KS // 2), 8)
        x = [_unpack(kx[pl.ds(rk, KS // 2), n * HD:(n + 1) * HD]) for n in range(5)]
        return [x[0], _unpack(hv[pl.ds(rv, KS // 2), 0:HD]), x[1], x[2],
                _unpack(hv[pl.ds(rv + KHP, KS // 2), HD:D]), x[3], x[4]]

    def s_blocks(qops, b, s):
        ko = k_ops(b, s)
        return _comb([_dot_nt(qops[p], ko[p]) for p in range(7)])

    bound2 = jnp.max(qmax) * (float(D) * 1.05)

    @pl.when(jnp.logical_not(bound2 <= SAFE_BOUND * SAFE_BOUND))
    def _():
        def unit_body(i, carry):
            b = _div(i, UPB)
            qops = load7(q7, pl.multiple_of(i * 7 * RP, 8))

            def slab_body(s, m):
                c = s_blocks(qops, b, s)
                col = s * KS + lax.broadcasted_iota(jnp.int32, (R, KS), 1)
                c = [jnp.where(col < KV, t, -jnp.inf) for t in c]
                top = jnp.max(jnp.maximum(c[0], c[1]), axis=-1, keepdims=True)
                bot = jnp.max(jnp.maximum(c[2], c[3]), axis=-1, keepdims=True)
                return jnp.maximum(m[0], top), jnp.maximum(m[1], bot)

            ninf = jnp.full((R, 1), -jnp.inf, F32)
            mt, mb = lax.fori_loop(0, NS, slab_body, (ninf, ninf))
            r = pl.multiple_of(i * U, U)
            dc[pl.ds(r, R), 0:128] = jnp.broadcast_to(mt, (R, 128))
            dc[pl.ds(r + R, R), 0:128] = jnp.broadcast_to(mb, (R, 128))
            return carry

        lax.fori_loop(0, NU, unit_body, 0)

    def g_row(i):
        b = _div(i, UPB)
        return _mo(8 + b * GP + (i - b * UPB) * U, 8)

    def s_job(i, slot, pieces, pin_i):
        b = _div(i, UPB)
        r = _mo(i * U, U)
        qops = load7(q7, _mo(i * 7 * RP, 8))
        m = [jnp.concatenate([dc[pl.ds(r + h * R, R), 0:128]] * (KS // 128), axis=1) for h in range(2)]
        l = [None, None]
        np_ = len(pieces)
        for s in range(NS):
            c = s_blocks(qops, b, s)
            pv = []
            for q in range(4):
                p = jnp.exp2(c[q] - m[q // 2])
                lo, hi = s * KS, (s + 1) * KS
                if hi > KV:
                    parts = []
                    for c0 in range(0, KS, 128):
                        nv = KV - (lo + c0)
                        if nv >= 128:
                            parts.append(p[:, c0:c0 + 128])
                        elif nv <= 0:
                            parts.append(jnp.zeros((R, 128), F32))
                        else:
                            lane = lax.broadcasted_iota(jnp.int32, (R, 128), 1)
                            parts.append(jnp.where(lane < nv, p[:, c0:c0 + 128], 0.0))
                    p = jnp.concatenate(parts, axis=1)
                pv.append(p)
                pbuf[slot, (q // 2) * RP:(q // 2 + 1) * RP,
                     (q % 2) * KH + s * KS:(q % 2) * KH + (s + 1) * KS] = _pack(p)
            for h in range(2):
                t = jnp.sum(pv[2 * h] + pv[2 * h + 1], axis=-1, keepdims=True)
                l[h] = t if l[h] is None else l[h] + t
            mine = pieces[s * np_ // NS:(s + 1) * np_ // NS]
            for t, piece in enumerate(mine):
                jr = GJ + 8 * (pin_i & 1)
                q = t % 4
                j = (t * (R // 8)) // len(mine)
                nt = (t // 4) % (KS // 128)
                g[0, pl.ds(pl.multiple_of(jr, 8), 8), :] = pv[q][j * 8:(j + 1) * 8, nt * 128:(nt + 1) * 128]
                piece()
        return l

    def pv_job(i, slot, l):
        b = _div(i, UPB)
        rv = _mo(2 * b * KHP, 8)
        o = _dot(_unpack(pbuf[slot]), _unpack(hv[pl.ds(rv, 2 * KHP), :]))
        o = jnp.concatenate([o[:R] * (1.0 / l[0]), o[R:] * (1.0 / l[1])], axis=0)
        store_lhs7(obuf, slot * 7 * RP, _quads(o))

    def post_1(i, slot):
        attn = _join(*_comb(mm7(load7(obuf, slot * 7 * RP), tvo)))
        r = _mo(i * U, U)
        x2 = x1[pl.ds(r, U), :] + attn
        x1[pl.ds(r, U), :] = x2
        return ffa_prep(_ln(x2))

    def post_2(i, ops):
        a_top, g_top, a_bot, g_bot = _comb(mm7(ops, tp1))
        gr = g_row(i)
        for a, bb, r0 in ((a_top, g_top, 0), (a_bot, g_bot, R)):
            ha = a * 0.5
            gv = ha * jnp.tanh(bb * 0.5) + ha
            for c4 in range(NC4):
                g[c4, pl.ds(gr + r0, R), :] = gv[:, c4 * 128:(c4 + 1) * 128]

    def conv_pieces(i):
        gr = g_row(i)
        r = _mo(i * U, U)
        pieces = []
        G = CG * 8
        for c4 in range(NC4):
            cs = slice(c4 * 128, (c4 + 1) * 128)
            stt = {}

            def out_rows(k0, stt=stt, c4=c4, cs=cs):
                w = stt['w']
                if CMODE == 0:
                    acc = None
                    for j in range(K):
                        t = g[c4, pl.ds(gr + k0 - pad + j, 8), :] * w[j]
                        acc = t if acc is None else acc + t
                    return acc
                st = 2 if CMODE == 1 else 4

                def y(b, k):
                    if (b, k) not in stt:
                        acc = None
                        for j in range(b, K, st):
                            t = g[c4, pl.ds(gr + k - pad + j - b, 8), :] * w[j]
                            acc = t if acc is None else acc + t
                        stt[(b, k)] = acc
                    return stt[(b, k)]

                sub = lax.broadcasted_iota(jnp.int32, (8, 128), 0)
                acc = y(0, k0)
                for b in range(1, st):
                    lo = pltpu.roll(y(b, k0), 8 - b, 0)
                    hi = pltpu.roll(y(b, k0 + 8), 8 - b, 0)
                    acc = acc + jnp.where(sub < 8 - b, lo, hi)
                return acc

            for k in range(U // G):
                def piece(k=k, stt=stt, cs=cs, out_rows=out_rows):
                    if k == 0:
                        stt['w'] = [dwf[pl.ds(j, 1), cs] for j in range(K)]
                    for k0 in range(k * G, (k + 1) * G, 8):
                        acc = out_rows(k0)
                        dc[pl.ds(r + k0, 8), cs] = acc
                        if k0 == 0:
                            stt['c'] = acc[0:1]
                        d = acc - stt['c']
                        stt['s1'] = d if k0 == 0 else stt['s1'] + d
                        stt['s2'] = d * d if k0 == 0 else stt['s2'] + d * d
                    if k == U // G - 1:
                        stat_c[pl.ds(_mo(i * 8, 8), 8), cs] = jnp.broadcast_to(stt['c'], (8, 128))
                        stat_1[pl.ds(_mo(i * 8, 8), 8), cs] = stt['s1']
                        stat_2[pl.ds(_mo(i * 8, 8), 8), cs] = stt['s2']
                pieces.append(piece)
        return pieces

    def conv(i):
        for p_ in conv_pieces(i):
            p_()

    def b_group(k, do_post, do_conv):
        units = [k * UB + t for t in range(UB)]
        if do_post:
            pops = [post_1(u - UB, t) for t, u in enumerate(units)]
        ls = []
        for t, u in enumerate(units):
            pieces = []
            if do_conv:
                cu = u - 2 * UB
                pieces = conv_pieces(max(cu, t) if isinstance(cu, int) else jnp.maximum(cu, t))
            ls.append(s_job(u, t, pieces, k))
            if do_post and t == 0:
                for t2, u2 in enumerate(units):
                    post_2(u2 - UB, pops[t2])
        for t, u in enumerate(units):
            pv_job(u, t, ls[t])

    NG = NU // UB
    b_group(0, False, False)

    def b_body(k, carry):
        b_group(k, True, True)
        return carry

    with scope('loopB'):
        lax.fori_loop(1, NG, b_body, 0)
    last = [(NG - 1) * UB + t for t in range(UB)]
    pops = [post_1(u, t) for t, u in enumerate(last)]
    for t, u in enumerate(last):
        post_2(u, pops[t])
    for u in range((NG - 2) * UB, NU):
        conv(u)

    sh = stat_c[...].reshape(NU, 8, D)
    s1 = jnp.sum(stat_1[...].reshape(NU, 8, D), axis=1, keepdims=True)
    s2 = jnp.sum(stat_2[...].reshape(NU, 8, D), axis=1, keepdims=True)
    tm = sh[:, 0:1, :] + s1 * (1.0 / U)
    mu = jnp.mean(tm, axis=0)
    dm = tm - mu
    m2 = jnp.sum(s2 - s1 * s1 * (1.0 / U) + float(U) * dm * dm, axis=0)
    bn[pl.ds(0, 1), :] = mu
    bn[pl.ds(1, 1), :] = lax.rsqrt(m2 * (1.0 / N) + EPS)

    def d_pre(j, slot):
        v = (dc[pl.ds(_mo(j * U, U), U), :] - bn[pl.ds(0, 1), :]) * bn[pl.ds(1, 1), :]
        hx = v * 0.5
        store_lhs7(ubuf, slot * 7 * RP, _quads(hx * jnp.tanh(hx) + hx))

    def d_first(j, slot):
        r = _mo(j * U, U)
        x3 = x1[pl.ds(r, U), :] + _join(*_comb(mm7(load7(ubuf, slot * 7 * RP), tp2)))
        x1[pl.ds(r, U), :] = x3
        return ffa_prep(_ln(x3))

    def d_last(j, y):
        r = _mo(j * U, U)
        xs[pl.ds(r, U), :] = _ln(x1[pl.ds(r, U), :] + y).astype(BF)
        o_copy(j).start()

    d_pre(0, 0)
    ops = d_first(0, 0)
    for s in range(NSL):
        ffa_slab(ops, ta2, s)
    d_pre(1, 1)

    def d_step(j, slot):
        ops = d_first(j, slot)
        y = ffb(tb2)
        d_last(j - 1, y)
        for s in range(NSL):
            ffa_slab(ops, ta2, s)
        nxt = min(j + 1, NU - 1) if isinstance(j, int) else jnp.minimum(j + 1, NU - 1)
        d_pre(nxt, 1 - slot)

    lead = (NU - 1) % UD
    for j in range(1, 1 + lead):
        d_step(j, j % 2)

    def d_body(k, carry):
        for t in range(UD):
            d_step(1 + lead + k * UD + t, (1 + lead + t) % 2)
        return carry

    assert UD % 2 == 0
    with scope('loopD'):
        lax.fori_loop(0, (NU - 1 - lead) // UD, d_body, 0)
    d_last(NU - 1, ffb(tb2))
    for j in range(NU):
        o_copy(j).wait()


def conformer(x, w_ff1_a, w_ff1_b, w_q, w_k, w_v, w_o, w_pw1, dw, w_pw2, w_ff2_a, w_ff2_b,
              *, U=160, KS=256, UA=2, UB=2, UD=2, CG=1, CMODE=0, interpret=False, vmem_mb=127, scopes=0):
    B, T, D = x.shape
    F = w_ff1_a.shape[1]
    K = dw.shape[0]
    N = B * T
    NU = N // U
    R = U // 2
    RP = R // 2
    KH = -(-(T // 2) // KS) * KS
    kern = functools.partial(_kernel, B=B, T=T, D=D, F=F, K=K, U=U, KH=KH, KS=KS, UA=UA, UB=UB, UD=UD,
                             CG=CG, CMODE=CMODE, scopes=scopes)
    hbm = pl.BlockSpec(memory_space=pl.ANY)
    V = pltpu.VMEM
    HD, HF = D // 2, F // 2
    scratch = [
        V((N, D), BF),
        V((N, D), F32),
        V((B * KH, D), U32),
        V((B * KH // 2, 5 * HD), U32),
        V((NU * 7 * RP, HD), U32),
        V((D // 128, B * (T + 8) + 8 + 16, 128), F32),
        V((N, D), F32),
        V((7 * HD // 2, HF), U32), V((7 * HF // 2, HD), U32),
        V((7 * HD // 2, HF), U32), V((7 * HF // 2, HD), U32),
        V((D, F), BF), V((F, D), BF),
        V((D, D), BF), V((D, D), BF),
        V((D, 2 * D), BF), V((D, D), BF),
        V((7 * HD // 2, HD), U32), V((7 * HD // 2, HD), U32),
        V((7 * HD // 2, D), U32), V((7 * HD // 2, HD), U32),
        V((K, D), BF), V((K, D), F32),
        V((7 * RP, HF), U32),
        V((UB, 2 * RP, 2 * KH), U32),
        V((UB * 7 * RP, HD), U32),
        V((2 * 7 * RP, HD), U32),
        V((NU * 8, D), F32), V((NU * 8, D), F32), V((NU * 8, D), F32), V((8, D), F32),
        pltpu.SemaphoreType.DMA((11,)),
        pltpu.SemaphoreType.DMA((NU // 2,)),
        pltpu.SemaphoreType.DMA((NU,)),
    ]
    out = pl.pallas_call(
        kern,
        out_shape=jax.ShapeDtypeStruct((N, D), x.dtype),
        in_specs=[hbm] * 12,
        out_specs=hbm,
        scratch_shapes=scratch,
        compiler_params=pltpu.CompilerParams(vmem_limit_bytes=vmem_mb * 1024 * 1024),
        interpret=interpret,
    )(x.reshape(N, D), w_ff1_a, w_ff1_b, w_q, w_k, w_v, w_o, w_pw1, dw, w_pw2, w_ff2_a, w_ff2_b)
    return out.reshape(B, T, D)


@jax.jit
def pallas_standalone__conformer_family_conformer__speech_kernel(
    x: jax.Array,
    w_ff1_a: jax.Array,
    w_ff1_b: jax.Array,
    w_q: jax.Array,
    w_k: jax.Array,
    w_v: jax.Array,
    w_o: jax.Array,
    w_pw1: jax.Array,
    dw: jax.Array,
    w_pw2: jax.Array,
    w_ff2_a: jax.Array,
    w_ff2_b: jax.Array,
):
    return conformer(x, w_ff1_a, w_ff1_b, w_q, w_k, w_v, w_o, w_pw1, dw, w_pw2, w_ff2_a, w_ff2_b)
```

```python
import contextlib
import functools

import numpy as np
import jax
import jax.numpy as jnp
from jax import lax
import jax.experimental.pallas as pl
import jax.experimental.pallas.tpu as pltpu

BF = jnp.bfloat16
F32 = jnp.float32
U32 = jnp.uint32
EPS = 1e-5
LOG2E = float(np.log2(np.e))
SAFE_BOUND = 60.0


def _div(i, n):
    return i // n if isinstance(i, int) else lax.div(i, jnp.int32(n))


def _mo(v, n):
    return v if isinstance(v, int) else pl.multiple_of(v, n)


def _ln(x):
    m = jnp.mean(x, axis=-1, keepdims=True)
    xc = x - m
    v = jnp.mean(xc * xc, axis=-1, keepdims=True)
    return xc * lax.rsqrt(v + EPS)


def _pack(v):
    return pltpu.bitcast(v.astype(BF), U32)


def _unpack(v):
    return pltpu.bitcast(v, BF)


def _dot(a, b):
    return jnp.dot(a, b, preferred_element_type=F32)


def _dot_nt(a, b):
    return lax.dot_general(a, b, (((1,), (1,)), ((), ())), preferred_element_type=F32)


def _lhs7(a11, a12, a21, a22):
    return [a11 + a22, a21 + a22, a11, a22, a11 + a12, a21 - a11, a12 - a22]


def _rhs7(b11, b12, b21, b22):
    return [b11 + b22, b11, b12 - b22, b21 - b11, b22, b11 + b12, b21 + b22]


def _comb(m):
    return (m[0] + m[3] - m[4] + m[6], m[2] + m[4], m[1] + m[3], m[0] - m[1] + m[2] + m[5])


def _quads(x):
    r, h = x.shape[0] // 2, x.shape[1] // 2
    return x[:r, :h], x[:r, h:], x[r:, :h], x[r:, h:]


def _join(c11, c12, c21, c22):
    return jnp.concatenate([jnp.concatenate([c11, c12], 1), jnp.concatenate([c21, c22], 1)], 0)


def _kernel(x_hbm, wa1_hbm, wb1_hbm, wq_hbm, wk_hbm, wv_hbm, wo_hbm, wp1_hbm, dw_hbm, wp2_hbm,
            wa2_hbm, wb2_hbm, out_hbm,
            xs, x1, kx, q7, g, dc,
            ta1, tb1, ta2, tb2, wa_s, wb_s, wt0, wt1, wp1_s, wp2_s, tqk, tvo, tp1, tp2, dwb, dwf,
            sbuf, pbuf, obuf, ubuf, stat_c, stat_1, stat_2, bn,
            sem_w, sem_x, sem_o,
            *, B, T, D, F, K, U, KH, KS, UA, UB, UD, CG, CMODE, PINMODE, WR, APOS, KG, scopes):
    def scope(n):
        return jax.named_scope(n) if scopes else contextlib.nullcontext()

    def scope2(n):
        return jax.named_scope(n) if scopes == 2 else contextlib.nullcontext()

    N = B * T
    NU = N // U
    UPB = T // U
    R = U // 2
    RP = R // 2
    M = 2 * U
    UP = U // 2
    NB = N // M
    HD, HF = D // 2, F // 2
    NS = KH // KS
    KV = UPB * R
    KHP = KH // 2
    GP = T + 8
    GJ = B * GP + 8
    pad = K // 2
    NC4 = D // 128

    def wcopy(src, dst, k):
        return pltpu.make_async_copy(src, dst, sem_w.at[k])

    c_wq, c_wk = wcopy(wq_hbm, wt0, 0), wcopy(wk_hbm, wt1, 1)
    def lead(ref):
        return ref.at[pl.ds(0, ref.shape[0] - 32), :]

    c_wa1, c_wb1 = wcopy(wa1_hbm, lead(wa_s), 2), wcopy(wb1_hbm, lead(wb_s), 3)
    c_dw, c_wp1, c_wp2 = wcopy(dw_hbm, dwb, 4), wcopy(wp1_hbm, lead(wp1_s), 5), wcopy(wp2_hbm, lead(wp2_s), 6)
    c_wa2, c_wb2 = wcopy(wa2_hbm, lead(wa_s), 7), wcopy(wb2_hbm, lead(wb_s), 8)
    c_wv, c_wo = wcopy(wv_hbm, wt0, 9), wcopy(wo_hbm, wt1, 10)

    NS_X = 4

    def slot_row(i):
        return (i % NS_X) * M if isinstance(i, int) else pl.multiple_of((i & (NS_X - 1)) * M, M)

    def x_copy(i):
        src = (i if i < NB else 0) if isinstance(i, int) else jnp.where(i < NB, i, 0)
        sem = sem_x.at[i % NS_X if isinstance(i, int) else i & (NS_X - 1)]
        return pltpu.make_async_copy(x_hbm.at[pl.ds(_mo(src * M, M), M), :],
                                     xs.at[pl.ds(slot_row(i), M), :], sem)

    def o_copy(j):
        sem = sem_o.at[j % NS_X if isinstance(j, int) else j & (NS_X - 1)]
        return pltpu.make_async_copy(xs.at[pl.ds(slot_row(j), M), :],
                                     out_hbm.at[pl.ds(_mo(j * M, M), M), :], sem)

    c_wq.start()
    c_wk.start()

    for b in range(B):
        r0 = b * KHP + KV // 2
        kx[pl.ds(r0, KHP - KV // 2), :] = jnp.zeros((KHP - KV // 2, 11 * HD), U32)
    for b in range(B + 1):
        g[:, pl.ds(b * GP, 8), :] = jnp.zeros((NC4, 8, 128), F32)
    g[:, pl.ds(8 + 2 * U, 8), :] = jnp.zeros((NC4, 8, 128), F32)

    def store7(t_ref, blocks, scale=None):
        hk = blocks[0].shape[0]
        for p, t in enumerate(_rhs7(*blocks)):
            t_ref[p * hk // 2:(p + 1) * hk // 2, :] = _pack(t if scale is None else t * scale)

    def prep_weight(w_ref, t_ref, scale, cw):
        kk, nn = w_ref.shape[0] - 32, w_ref.shape[1]
        hk, hn = kk // 2, nn // 2
        for c0 in range(0, hn, cw):
            blk = [w_ref[r0:r0 + hk, cc:cc + cw].astype(F32) * scale
                   for r0 in (0, hk) for cc in (c0, hn + c0)]
            for p, t in enumerate(_rhs7(*blk)):
                t_ref[p * hk // 2:(p + 1) * hk // 2, c0:c0 + cw] = _pack(t)

    def weight_pieces(w_ref, t_ref, scale, rows):
        kk, nn = w_ref.shape[0] - 32, w_ref.shape[1]
        hk, hn = kk // 2, nn // 2

        def piece(r0, c0, n, pinval):
            if pinval is not None:
                pin_to(w_ref, kk + 16 * (n & 1), pinval)
            blk = [w_ref[rr:rr + rows, cc:cc + 128].astype(F32) * scale
                   for rr in (r0, hk + r0) for cc in (c0, hn + c0)]
            for p, t in enumerate(_rhs7(*blk)):
                t_ref[(p * hk + r0) // 2:(p * hk + r0 + rows) // 2, c0:c0 + 128] = _pack(t)

        return [functools.partial(piece, r0, c0, r0 // rows + c0 // 128)
                for c0 in range(0, hn, 128) for r0 in range(0, hk, rows)]

    with scope2('s0a'):
        c_wk.wait()
        c_wq.wait()
    with scope2('s0b'):
        x_copy(0).start()
        c_wa1.start()
        store7(tqk, _quads(_dot_nt(wt0[...], wt1[...])), LOG2E * float(D) ** -0.5)

    def mm7(ops, t_ref, cs=slice(None)):
        hk = t_ref.shape[0] // 7
        return [_dot(ops[p], _unpack(t_ref[p * hk:(p + 1) * hk, cs])) for p in range(7)]

    def load7(ref, r0, hp):
        return [_unpack(ref[pl.ds(r0 + p * hp, hp), :]) for p in range(7)]

    def store_lhs7(ref, r0, blocks, cs=slice(None)):
        hp = blocks[0].shape[0] // 2
        for p, t in enumerate(_lhs7(*blocks)):
            ref[pl.ds(r0 + p * hp, hp), cs] = _pack(t)

    SL = 256
    NSL = HF // SL

    def ffa_prep(xn):
        return [t.astype(BF) for t in _lhs7(*_quads(xn))]

    def ffa_slab(ops, ta, s, pieces=()):
        cs = slice(s * SL, (s + 1) * SL)
        ms = mm7(ops, ta, cs)
        for p in range(7):
            for piece in share(pieces, p, 7):
                piece(ms[p])
        act = [hx * jnp.tanh(hx) + hx for hx in _comb(ms)]
        store_lhs7(sbuf, 0, act, cs)

    def pin_to(ref, row, val):
        n = 16 if ref.dtype == BF else 8
        v = val[0:n, 0:128]
        ref[pl.ds(pl.multiple_of(row, n), n), 0:128] = (
            pltpu.bitcast(v, U32) if ref.dtype == U32 else v.astype(ref.dtype))

    def share(pieces, step, steps):
        return pieces[step * len(pieces) // steps:(step + 1) * len(pieces) // steps]

    KB = 256

    def ffb(tb, pieces=()):
        ms = []
        nk = HF // KB
        for p in range(7):
            acc = None
            for kc in range(nk):
                part = _dot(_unpack(sbuf[p * UP:(p + 1) * UP, kc * KB:(kc + 1) * KB]),
                            _unpack(tb[(p * HF + kc * KB) // 2:(p * HF + (kc + 1) * KB) // 2, :]))
                acc = part if acc is None else acc + part
                for piece in share(pieces, p * nk + kc, 7 * nk):
                    piece(part)
            ms.append(acc)
        return _join(*_comb(ms))

    PR = 16

    def lhs7_pieces(src, r, junk, fn, slot, packed):
        def piece(j, pinval):
            if pinval is not None:
                pin_to(src, junk, pinval)
            if packed:
                top = fn(_unpack(src[pl.ds(r + j * PR // 2, PR // 2), :]).astype(F32))
                bot = fn(_unpack(src[pl.ds(r + (U + j * PR) // 2, PR // 2), :]).astype(F32))
            else:
                top = fn(src[pl.ds(r + j * PR, PR), :].astype(F32))
                bot = fn(src[pl.ds(r + U + j * PR, PR), :].astype(F32))
            for p, t in enumerate(_lhs7(top[:, :HD], top[:, HD:], bot[:, :HD], bot[:, HD:])):
                ubuf[pl.ds(_mo(slot * 7 * UP + p * UP + j * (PR // 2), 8), PR // 2), :] = _pack(t)
        return [functools.partial(piece, j) for j in range(U // PR)]

    def a_prep(i, slot):
        return lhs7_pieces(xs, slot_row(i), NS_X * M + 16 * (slot & 1), _ln, slot, False)

    def a_second(i, pieces=()):
        y = ffb(tb1, pieces)
        r = _mo(i * M, M)
        x1v = xs[pl.ds(slot_row(i), M), :].astype(F32) + y
        x1[pl.ds(r, M), :] = x1v
        h = _ln(x1v)
        for sub in range(2):
            un = 2 * i + sub
            b = _div(un, UPB)
            u = un - b * UPB
            rk = _mo(b * KHP + u * RP, 8)
            h11, h12, h21, h22 = _quads(h[sub * U:(sub + 1) * U])
            blocks = (h11 + h22, h11, h22,
                      h21 - h22, h12 - h11, h11 + h21, h12 + h22,
                      h12 - h22, h21 - h11, h11 + h12, h21 + h22)
            for n, t in enumerate(blocks):
                kx[pl.ds(rk, RP), n * HD:(n + 1) * HD] = _pack(t)
        return [t.astype(BF) for t in _lhs7(*_quads(h))]

    def a_third(i, hops, qmax):
        q = _join(*_comb(mm7(hops, tqk)))
        for sub in range(2):
            store_lhs7(q7, _mo((2 * i + sub) * 7 * RP, 8), _quads(q[sub * U:(sub + 1) * U]))
        n2 = jnp.sum(q * q, axis=-1, keepdims=True)
        return jnp.maximum(qmax, jnp.max(n2.reshape(M // 8, 8, 1), axis=0))

    with scope2('s0c'):
        c_wa1.wait()
    with scope2('s0d'):
        x_copy(1).start()
        c_wb1.start()
        prep_weight(wa_s, ta1, 0.5, 256)
    with scope2('s0e'):
        x_copy(0).wait()
        for piece in a_prep(0, 0):
            piece(None)
        ops = load7(ubuf, 0, UP)
        for s in range(NSL):
            ffa_slab(ops, ta1, s)
        x_copy(1).wait()
        x_copy(2).start()
        for piece in a_prep(1, 1):
            piece(None)
    with scope2('s0f'):
        c_wb1.wait()
    with scope2('s0g'):
        x_copy(3).start()
        for c in (c_wv, c_wo, c_dw, c_wp1, c_wp2, c_wa2):
            c.start()
        prep_weight(wb_s, tb1, 0.5, 128)
        c_wb2.start()

    def a_step(i, slot, qmax):
        ops = load7(ubuf, slot * 7 * UP, UP)
        pcs = a_prep(i + 1, 1 - slot)
        hops = a_second(i - 1, pcs if APOS == 0 else ())
        ffa_slab(ops, ta1, 0)
        ffa_slab(ops, ta1, 1, share(pcs, 0, 3) if APOS == 2 else ())
        qmax = a_third(i - 1, hops, qmax)
        ffa_slab(ops, ta1, 2, share(pcs, 0, 2) if APOS == 1 else share(pcs, 1, 3) if APOS == 2 else ())
        ffa_slab(ops, ta1, 3, share(pcs, 1, 2) if APOS == 1 else share(pcs, 2, 3) if APOS == 2 else ())
        return qmax

    def a_body(k, qmax):
        for t in range(2):
            i = 1 + 2 * k + t
            x_copy(i + 1).wait()
            qmax = a_step(i, (1 + t) % 2, qmax)
            x_copy(i + 3).start()
        return qmax

    assert (NB - 1) % 2 == 0
    qmax = jnp.zeros((8, 1), F32)
    with scope('loopA'):
        qmax = lax.fori_loop(0, (NB - 1) // 2, a_body, qmax)
    with scope2('seg2'):
        x_copy(NB + 1).wait()
        x_copy(NB + 2).wait()
        hops = a_second(NB - 1)
        qmax = a_third(NB - 1, hops, qmax)
        for c in (c_dw, c_wp1, c_wp2, c_wv, c_wo, c_wa2, c_wb2):
            c.wait()
        dwf[...] = dwb[...].astype(F32)
        store7(tvo, _quads(_dot(wt0[...], wt1[...])))

    def g_row(i):
        b = _div(i, UPB)
        return _mo(8 + b * GP + (i - b * UPB) * U, 8)

    for b in range(B):
        g[0, pl.ds(8 + b * GP, T), :] = jnp.zeros((T, 128), F32)

    def kv_ops(b, r0, n, which):
        rk = _mo(b * KHP + r0, 8)
        return [_unpack(kx[pl.ds(rk, n), i * HD:(i + 1) * HD]) for i in which]

    K_OPS = (0, 1, 3, 4, 2, 5, 6)
    V_OPS = (0, 1, 7, 8, 2, 9, 10)

    def s_blocks(qops, b, s):
        ko = kv_ops(b, s * (KS // 2), KS // 2, K_OPS)
        return _comb([_dot_nt(qops[p], ko[p]) for p in range(7)])

    bound2 = jnp.max(qmax) * (float(D) * 1.05)

    @pl.when(jnp.logical_not(bound2 <= SAFE_BOUND * SAFE_BOUND))
    def _():
        def unit_body(i, carry):
            b = _div(i, UPB)
            qops = load7(q7, pl.multiple_of(i * 7 * RP, 8), RP)

            def slab_body(s, m):
                c = s_blocks(qops, b, s)
                col = s * KS + lax.broadcasted_iota(jnp.int32, (R, KS), 1)
                c = [jnp.where(col < KV, t, -jnp.inf) for t in c]
                top = jnp.max(jnp.maximum(c[0], c[1]), axis=-1, keepdims=True)
                bot = jnp.max(jnp.maximum(c[2], c[3]), axis=-1, keepdims=True)
                return jnp.maximum(m[0], top), jnp.maximum(m[1], bot)

            ninf = jnp.full((R, 1), -jnp.inf, F32)
            mt, mb = lax.fori_loop(0, NS, slab_body, (ninf, ninf))
            r = g_row(i)
            g[0, pl.ds(r, R), :] = jnp.broadcast_to(mt, (R, 128))
            g[0, pl.ds(r + R, R), :] = jnp.broadcast_to(mb, (R, 128))
            return carry

        lax.fori_loop(0, NU, unit_body, 0)

    def pin(pin_i, val):
        g[0, pl.ds(pl.multiple_of(GJ + 8 * (pin_i & 1), 8), 8), :] = val

    def s_job(i, slot, pieces, pin_i):
        b = _div(i, UPB)
        r = g_row(i)
        qops = load7(q7, _mo(i * 7 * RP, 8), RP)
        m = [jnp.concatenate([g[0, pl.ds(r + h * R, R), :]] * (KS // 128), axis=1) for h in range(2)]
        l = [None, None]
        np_ = len(pieces)
        for s in range(NS):
            c = s_blocks(qops, b, s)
            pv = []
            for q in range(4):
                p = jnp.exp2(c[q] - m[q // 2])
                lo, hi = s * KS, (s + 1) * KS
                if hi > KV:
                    parts = []
                    for c0 in range(0, KS, 128):
                        nv = KV - (lo + c0)
                        if nv >= 128:
                            parts.append(p[:, c0:c0 + 128])
                        elif nv <= 0:
                            parts.append(jnp.zeros((R, 128), F32))
                        else:
                            lane = lax.broadcasted_iota(jnp.int32, (R, 128), 1)
                            parts.append(jnp.where(lane < nv, p[:, c0:c0 + 128], 0.0))
                    p = jnp.concatenate(parts, axis=1)
                pv.append(p)
                pbuf[slot * 4 + q, :, s * KS:(s + 1) * KS] = p
            for h in range(2):
                t = jnp.sum(pv[2 * h] + pv[2 * h + 1], axis=-1, keepdims=True)
                l[h] = t if l[h] is None else l[h] + t
            if PINMODE == 0:
                mine = pieces[s * np_ // NS:(s + 1) * np_ // NS]
                for t, piece in enumerate(mine):
                    q = t % 4
                    j = (t * (R // 8)) // len(mine)
                    nt = (t // 4) % (KS // 128)
                    pin(pin_i, pv[q][j * 8:(j + 1) * 8, nt * 128:(nt + 1) * 128])
                    piece()
        return l

    def pv_job(i, slot, l, pieces, pin_i):
        b = _div(i, UPB)
        inv = [1.0 / l[0], 1.0 / l[1]]
        NKG = KH // KG
        acc = [None] * 7
        for kg in range(NKG):
            cs = slice(kg * KG, (kg + 1) * KG)
            ops = _lhs7(*[pbuf[slot * 4 + q, :, cs] * inv[q // 2] for q in range(4)])
            vo = kv_ops(b, kg * (KG // 2), KG // 2, V_OPS)
            for p in range(7):
                part = _dot(ops[p].astype(BF), vo[p])
                acc[p] = part if acc[p] is None else acc[p] + part
                mine = share(pieces, kg * 7 + p, NKG * 7)
                for t, piece in enumerate(mine):
                    j = (t * (R // 16)) // len(mine)
                    piece(part[j * 16:(j + 1) * 16, :])
        return _join(*_comb(acc))

    def post_1(k):
        attn = _join(*_comb(mm7(load7(obuf, 0, UP), tvo)))
        r = _mo(k * M, M)
        x2 = x1[pl.ds(r, M), :] + attn
        x1[pl.ds(r, M), :] = x2
        return ffa_prep(_ln(x2))

    def post_2(k, ops):
        a_top, g_top, a_bot, g_bot = _comb(mm7(ops, tp1))
        for a, bb, sub in ((a_top, g_top, 0), (a_bot, g_bot, 1)):
            gr = g_row(2 * k + sub)
            ha = a * 0.5
            gv = ha * jnp.tanh(bb * 0.5) + ha
            for c4 in range(NC4):
                g[c4, pl.ds(gr, U), :] = gv[:, c4 * 128:(c4 + 1) * 128]

    def conv_pieces(i):
        gr = g_row(i)
        r = _mo(i * (U // 2), 8)
        pieces = []
        G = CG * 8
        for c4 in range(NC4):
            cs = slice(c4 * 128, (c4 + 1) * 128)
            stt = {}

            def out_rows(k0, stt=stt, c4=c4, cs=cs):
                w = stt['w']
                if CMODE == 0:
                    acc = None
                    for j in range(K):
                        t = g[c4, pl.ds(gr + k0 - pad + j, 8), :] * w[j]
                        acc = t if acc is None else acc + t
                    return acc
                st = 2 if CMODE == 1 else 4

                def y(b, k):
                    if (b, k) not in stt:
                        acc = None
                        for j in range(b, K, st):
                            t = g[c4, pl.ds(gr + k - pad + j - b, 8), :] * w[j]
                            acc = t if acc is None else acc + t
                        stt[(b, k)] = acc
                    return stt[(b, k)]

                sub = lax.broadcasted_iota(jnp.int32, (8, 128), 0)
                acc = y(0, k0)
                for b in range(1, st):
                    lo = pltpu.roll(y(b, k0), 8 - b, 0)
                    hi = pltpu.roll(y(b, k0 + 8), 8 - b, 0)
                    acc = acc + jnp.where(sub < 8 - b, lo, hi)
                return acc

            for k in range(U // G):
                def piece(pinval, k=k, stt=stt, cs=cs, out_rows=out_rows):
                    if pinval is not None:
                        g[0, pl.ds(pl.multiple_of(GJ + 8 * (i & 1), 8), 8), :] = pinval[0:8, 0:128]
                    if k == 0:
                        stt['w'] = [dwf[pl.ds(j, 1), cs] for j in range(K)]
                    rows = []
                    for k0 in range(k * G, (k + 1) * G, 8):
                        acc = out_rows(k0)
                        rows.append(acc)
                        if k0 == 0:
                            stt['c'] = acc[0:1]
                        d = acc - stt['c']
                        stt['s1'] = d if k0 == 0 else stt['s1'] + d
                        stt['s2'] = d * d if k0 == 0 else stt['s2'] + d * d
                    dc[pl.ds(r + k * (G // 2), G // 2), cs] = _pack(jnp.concatenate(rows, axis=0))
                    if k == U // G - 1:
                        stat_c[pl.ds(_mo(i * 8, 8), 8), cs] = jnp.broadcast_to(stt['c'], (8, 128))
                        stat_1[pl.ds(_mo(i * 8, 8), 8), cs] = stt['s1']
                        stat_2[pl.ds(_mo(i * 8, 8), 8), cs] = stt['s2']
                pieces.append(piece)
        return pieces

    def conv(i):
        for p_ in conv_pieces(i):
            p_(None)

    def b_group(k, do_post, do_conv, fill=None):
        units = [2 * k, 2 * k + 1]
        if do_post:
            pops = post_1(k - 1)
        ls, allp = [], []
        for t, u in enumerate(units):
            pieces = conv_pieces(jnp.maximum(u - 4, t)) if do_conv else fill[t]
            allp.append(pieces)
            ls.append(s_job(u, t, pieces, k))
            if do_post and t == 0:
                post_2(k - 1, pops)
        os_ = [pv_job(u, t, ls[t], allp[t], k) for t, u in enumerate(units)]
        store_lhs7(obuf, 0, (os_[0][:, :HD], os_[0][:, HD:], os_[1][:, :HD], os_[1][:, HD:]))

    with scope2('proB'):
        wp = (weight_pieces(wp1_s, tp1, 1.0, WR) + weight_pieces(wp2_s, tp2, 1.0, WR)
              + weight_pieces(wa_s, ta2, 0.5, WR) + weight_pieces(wb_s, tb2, 0.5, WR))
        b_group(0, False, False, [wp[:len(wp) // 2], wp[len(wp) // 2:]])

    def b_body(k, carry):
        b_group(k, True, True)
        return carry

    with scope('loopB'):
        lax.fori_loop(1, NB, b_body, 0)
    with scope2('tail1'):
        post_2(NB - 1, post_1(NB - 1))
    with scope2('tail2'):
        for u in range(NU - 4, NU):
            conv(u)

    acc = None
    for u in range(NU):
        t = stat_1[u * 8:(u + 1) * 8, :] + float(U // 8) * stat_c[u * 8:(u + 1) * 8, :]
        acc = t if acc is None else acc + t
    mu = jnp.sum(acc, axis=0, keepdims=True) * (1.0 / N)
    acc = None
    for u in range(NU):
        e = mu - stat_c[u * 8:(u + 1) * 8, :]
        t = stat_2[u * 8:(u + 1) * 8, :] + e * (float(U // 8) * e - 2.0 * stat_1[u * 8:(u + 1) * 8, :])
        acc = t if acc is None else acc + t
    bn[pl.ds(0, 1), :] = mu
    bn[pl.ds(1, 1), :] = lax.rsqrt(jnp.sum(acc, axis=0, keepdims=True) * (1.0 / N) + EPS)

    def bn_silu(v):
        hx = (v - bn[pl.ds(0, 1), :]) * (bn[pl.ds(1, 1), :] * 0.5)
        return hx * jnp.tanh(hx) + hx

    def d_pre(j, slot):
        return lhs7_pieces(dc, _mo(j * U, 8), N // 2 + 8 * (slot & 1), bn_silu, slot, True)

    def d_first(j, slot):
        r = _mo(j * M, M)
        x3 = x1[pl.ds(r, M), :] + _join(*_comb(mm7(load7(ubuf, _mo(slot * 7 * UP, 8), UP), tp2)))
        x1[pl.ds(r, M), :] = x3
        return ffa_prep(_ln(x3))

    def d_last(j, y):
        r = _mo(j * M, M)
        xs[pl.ds(slot_row(j), M), :] = _ln(x1[pl.ds(r, M), :] + y).astype(BF)
        o_copy(j).start()

    for j in range(NS_X):
        o_copy(j).start()
    with scope2('proD'):
        for piece in d_pre(0, 0):
            piece(None)
        ops = d_first(0, 0)
        for s in range(NSL):
            ffa_slab(ops, ta2, s)
        for piece in d_pre(1, 1):
            piece(None)

    def d_body(k, carry):
        for t in range(2):
            j = 1 + 2 * k + t
            slot = (1 + t) % 2
            o_copy(j - 1).wait()
            ops = d_first(j, slot)
            y = ffb(tb2, d_pre(jnp.minimum(j + 1, NB - 1), 1 - slot))
            d_last(j - 1, y)
            for s in range(NSL):
                ffa_slab(ops, ta2, s)
        return carry

    with scope('loopD'):
        lax.fori_loop(0, (NB - 1) // 2, d_body, 0)
    with scope2('end'):
        o_copy(NB - 1).wait()
        d_last(NB - 1, ffb(tb2))
        for j in range(NB - NS_X, NB):
            o_copy(j).wait()


def conformer(x, w_ff1_a, w_ff1_b, w_q, w_k, w_v, w_o, w_pw1, dw, w_pw2, w_ff2_a, w_ff2_b,
              *, U=160, KS=256, UA=2, UB=2, UD=2, CG=2, CMODE=2, PINMODE=1, WR=32, APOS=0, KG=512, interpret=False, vmem_mb=122, scopes=0):
    B, T, D = x.shape
    F = w_ff1_a.shape[1]
    K = dw.shape[0]
    N = B * T
    NU = N // U
    R = U // 2
    RP = R // 2
    KH = -(-(T // 2) // KS) * KS
    kern = functools.partial(_kernel, B=B, T=T, D=D, F=F, K=K, U=U, KH=KH, KS=KS, UA=UA, UB=UB, UD=UD,
                             CG=CG, CMODE=CMODE, PINMODE=PINMODE, WR=WR, APOS=APOS, KG=KG, scopes=scopes)
    hbm = pl.BlockSpec(memory_space=pl.ANY)
    V = pltpu.VMEM
    HD, HF = D // 2, F // 2
    scratch = [
        V((8 * U + 32, D), BF),
        V((N, D), F32),
        V((B * KH // 2, 11 * HD), U32),
        V((NU * 7 * RP, HD), U32),
        V((D // 128, B * (T + 8) + 8 + 16, 128), F32),
        V((N // 2 + 16, D), U32),
        V((7 * HD // 2, HF), U32), V((7 * HF // 2, HD), U32),
        V((7 * HD // 2, HF), U32), V((7 * HF // 2, HD), U32),
        V((D + 32, F), BF), V((F + 32, D), BF),
        V((D, D), BF), V((D, D), BF),
        V((D + 32, 2 * D), BF), V((D + 32, D), BF),
        V((7 * HD // 2, HD), U32), V((7 * HD // 2, HD), U32),
        V((7 * HD // 2, D), U32), V((7 * HD // 2, HD), U32),
        V((K, D), BF), V((K, D), F32),
        V((7 * U // 2, HF), U32),
        V((8, R, KH), F32),
        V((7 * U // 2, HD), U32),
        V((2 * 7 * U // 2, HD), U32),
        V((NU * 8, D), F32), V((NU * 8, D), F32), V((NU * 8, D), F32), V((8, D), F32),
        pltpu.SemaphoreType.DMA((11,)),
        pltpu.SemaphoreType.DMA((4,)),
        pltpu.SemaphoreType.DMA((4,)),
    ]
    out = pl.pallas_call(
        kern,
        out_shape=jax.ShapeDtypeStruct((N, D), x.dtype),
        in_specs=[hbm] * 12,
        out_specs=hbm,
        scratch_shapes=scratch,
        compiler_params=pltpu.CompilerParams(vmem_limit_bytes=vmem_mb * 1024 * 1024),
        interpret=interpret,
    )(x.reshape(N, D), w_ff1_a, w_ff1_b, w_q, w_k, w_v, w_o, w_pw1, dw, w_pw2, w_ff2_a, w_ff2_b)
    return out.reshape(B, T, D)


@jax.jit
def pallas_standalone__conformer_family_conformer__speech_kernel(
    x: jax.Array,
    w_ff1_a: jax.Array,
    w_ff1_b: jax.Array,
    w_q: jax.Array,
    w_k: jax.Array,
    w_v: jax.Array,
    w_o: jax.Array,
    w_pw1: jax.Array,
    dw: jax.Array,
    w_pw2: jax.Array,
    w_ff2_a: jax.Array,
    w_ff2_b: jax.Array,
):
    return conformer(x, w_ff1_a, w_ff1_b, w_q, w_k, w_v, w_o, w_pw1, dw, w_pw2, w_ff2_a, w_ff2_b)
```

```python
import contextlib
import functools

import numpy as np
import jax
import jax.numpy as jnp
from jax import lax
import jax.experimental.pallas as pl
import jax.experimental.pallas.tpu as pltpu

BF = jnp.bfloat16
F32 = jnp.float32
U32 = jnp.uint32
EPS = 1e-5
LOG2E = float(np.log2(np.e))
SAFE_BOUND = 60.0


def _div(i, n):
    return i // n if isinstance(i, int) else lax.div(i, jnp.int32(n))


def _mo(v, n):
    return v if isinstance(v, int) else pl.multiple_of(v, n)


def _ln(x):
    m = jnp.mean(x, axis=-1, keepdims=True)
    xc = x - m
    v = jnp.mean(xc * xc, axis=-1, keepdims=True)
    return xc * lax.rsqrt(v + EPS)


def _pack(v):
    return pltpu.bitcast(v.astype(BF), U32)


def _unpack(v):
    return pltpu.bitcast(v, BF)


def _dot(a, b):
    return jnp.dot(a, b, preferred_element_type=F32)


def _dot_nt(a, b):
    return lax.dot_general(a, b, (((1,), (1,)), ((), ())), preferred_element_type=F32)


def _lhs7(a11, a12, a21, a22):
    return [a11 + a22, a21 + a22, a11, a22, a11 + a12, a21 - a11, a12 - a22]


def _rhs7(b11, b12, b21, b22):
    return [b11 + b22, b11, b12 - b22, b21 - b11, b22, b11 + b12, b21 + b22]


def _comb(m):
    return (m[0] + m[3] - m[4] + m[6], m[2] + m[4], m[1] + m[3], m[0] - m[1] + m[2] + m[5])


def _quads(x):
    r, h = x.shape[0] // 2, x.shape[1] // 2
    return x[:r, :h], x[:r, h:], x[r:, :h], x[r:, h:]


def _join(c11, c12, c21, c22):
    return jnp.concatenate([jnp.concatenate([c11, c12], 1), jnp.concatenate([c21, c22], 1)], 0)


def _kernel(x_hbm, wa1_hbm, wb1_hbm, wq_hbm, wk_hbm, wv_hbm, wo_hbm, wp1_hbm, dw_hbm, wp2_hbm,
            wa2_hbm, wb2_hbm, out_hbm,
            xs, x1, kx, k7, g, dc,
            ta1, tb1, ta2, tb2, wa_s, wb_s, wt0, wt1, wp1_s, wp2_s, tqk, tvo, tp1, tp2, dwb, dwf,
            sbuf, pbuf, abuf, obuf, ubuf, stat_c, stat_1, stat_2, bn,
            zero, sem_w, sem_x, sem_o,
            *, B, T, D, F, K, U, KH, KS, UA, UB, UD, CG, CMODE, PINMODE, WR, APOS, KG, PC, CSPLIT, scopes):
    def scope(n):
        return jax.named_scope(n) if scopes else contextlib.nullcontext()

    def scope2(n):
        return jax.named_scope(n) if scopes == 2 else contextlib.nullcontext()

    N = B * T
    NU = N // U
    UPB = T // U
    R = U // 2
    RP = R // 2
    M = 2 * U
    UP = U // 2
    NB = N // M
    HD, HF = D // 2, F // 2
    NS = KH // KS
    KV = UPB * R
    KHP = KH // 2
    GP = T + 8
    GJ = B * GP + 8
    pad = K // 2
    NC4 = D // 128

    def wcopy(src, dst, k):
        return pltpu.make_async_copy(src, dst, sem_w.at[k])

    c_wq, c_wk = wcopy(wq_hbm, wt0, 0), wcopy(wk_hbm, wt1, 1)
    def lead(ref):
        return ref.at[pl.ds(0, ref.shape[0] - 32), :]

    c_wa1, c_wb1 = wcopy(wa1_hbm, lead(wa_s), 2), wcopy(wb1_hbm, lead(wb_s), 3)
    c_dw, c_wp1, c_wp2 = wcopy(dw_hbm, dwb, 4), wcopy(wp1_hbm, lead(wp1_s), 5), wcopy(wp2_hbm, lead(wp2_s), 6)
    c_wa2, c_wb2 = wcopy(wa2_hbm, lead(wa_s), 7), wcopy(wb2_hbm, lead(wb_s), 8)
    c_wv, c_wo = wcopy(wv_hbm, wt0, 9), wcopy(wo_hbm, wt1, 10)

    NS_X = 4

    def slot_row(i):
        return (i % NS_X) * M if isinstance(i, int) else pl.multiple_of((i & (NS_X - 1)) * M, M)

    def x_copy(i):
        src = (i if i < NB else 0) if isinstance(i, int) else jnp.where(i < NB, i, 0)
        sem = sem_x.at[i % NS_X if isinstance(i, int) else i & (NS_X - 1)]
        return pltpu.make_async_copy(x_hbm.at[pl.ds(_mo(src * M, M), M), :],
                                     xs.at[pl.ds(slot_row(i), M), :], sem)

    def o_copy(j):
        sem = sem_o.at[j % NS_X if isinstance(j, int) else j & (NS_X - 1)]
        return pltpu.make_async_copy(xs.at[pl.ds(slot_row(j), M), :],
                                     out_hbm.at[pl.ds(_mo(j * M, M), M), :], sem)

    c_wq.start()
    c_wk.start()

    zero[0] = 0
    for b in range(B):
        r0 = b * KHP + KV // 2
        kx[pl.ds(r0, KHP - KV // 2), :] = jnp.zeros((KHP - KV // 2, 7 * HD), U32)
        k7[pl.ds(r0, KHP - KV // 2), :] = jnp.zeros((KHP - KV // 2, 7 * HD), U32)
    for b in range(B + 1):
        g[:, pl.ds(b * GP, 8), :] = jnp.zeros((NC4, 8, 128), F32)
    g[:, pl.ds(8 + 2 * U, 8), :] = jnp.zeros((NC4, 8, 128), F32)

    def store7(t_ref, blocks, scale=None):
        hk = blocks[0].shape[0]
        for p, t in enumerate(_rhs7(*blocks)):
            t_ref[p * hk // 2:(p + 1) * hk // 2, :] = _pack(t if scale is None else t * scale)

    def prep_weight(w_ref, t_ref, scale, cw):
        kk, nn = w_ref.shape[0] - 32, w_ref.shape[1]
        hk, hn = kk // 2, nn // 2
        for c0 in range(0, hn, cw):
            blk = [w_ref[r0:r0 + hk, cc:cc + cw].astype(F32) * scale
                   for r0 in (0, hk) for cc in (c0, hn + c0)]
            for p, t in enumerate(_rhs7(*blk)):
                t_ref[p * hk // 2:(p + 1) * hk // 2, c0:c0 + cw] = _pack(t)

    def weight_pieces(w_ref, t_ref, scale, rows):
        kk, nn = w_ref.shape[0] - 32, w_ref.shape[1]
        hk, hn = kk // 2, nn // 2

        def piece(r0, c0, n, pinval):
            if pinval is not None:
                pin_to(w_ref, kk + 16 * (n & 1), pinval)
            blk = [w_ref[rr:rr + rows, cc:cc + 128].astype(F32) * scale
                   for rr in (r0, hk + r0) for cc in (c0, hn + c0)]
            for p, t in enumerate(_rhs7(*blk)):
                t_ref[(p * hk + r0) // 2:(p * hk + r0 + rows) // 2, c0:c0 + 128] = _pack(t)

        return [functools.partial(piece, r0, c0, r0 // rows + c0 // 128)
                for c0 in range(0, hn, 128) for r0 in range(0, hk, rows)]

    with scope2('s0a'):
        c_wk.wait()
        c_wq.wait()
    with scope2('s0b'):
        x_copy(0).start()
        c_wa1.start()
        store7(tqk, _quads(_dot_nt(wt1[...], wt0[...])), LOG2E * float(D) ** -0.5)

    def mm7(ops, t_ref, cs=slice(None)):
        hk = t_ref.shape[0] // 7
        return [_dot(ops[p], _unpack(t_ref[p * hk:(p + 1) * hk, cs])) for p in range(7)]

    def load7(ref, r0, hp):
        return [_unpack(ref[pl.ds(r0 + p * hp, hp), :]) for p in range(7)]

    def store_lhs7(ref, r0, blocks, cs=slice(None)):
        hp = blocks[0].shape[0] // 2
        for p, t in enumerate(_lhs7(*blocks)):
            ref[pl.ds(r0 + p * hp, hp), cs] = _pack(t)

    SL = 256
    NSL = HF // SL

    def ffa_prep(xn):
        return [t.astype(BF) for t in _lhs7(*_quads(xn))]

    def ffa_slab(ops, ta, s, pieces=()):
        cs = slice(s * SL, (s + 1) * SL)
        ms = mm7(ops, ta, cs)
        for p in range(7):
            for piece in share(pieces, p, 7):
                piece(ms[p])
        act = [hx * jnp.tanh(hx) + hx for hx in _comb(ms)]
        store_lhs7(sbuf, 0, act, cs)

    def pin_to(ref, row, val):
        n = 16 if ref.dtype == BF else 8
        v = val[0:n, 0:128]
        ref[pl.ds(pl.multiple_of(row, n), n), 0:128] = (
            pltpu.bitcast(v, U32) if ref.dtype == U32 else v.astype(ref.dtype))

    def share(pieces, step, steps):
        return pieces[step * len(pieces) // steps:(step + 1) * len(pieces) // steps]

    def interleave(a, b):
        out, n = [], max(len(a), len(b))
        for t in range(n):
            out += share(a, t, n) + share(b, t, n)
        return out

    KB = 256

    def ffb(tb, pieces=()):
        ms = []
        nk = HF // KB
        for p in range(7):
            acc = None
            for kc in range(nk):
                part = _dot(_unpack(sbuf[p * UP:(p + 1) * UP, kc * KB:(kc + 1) * KB]),
                            _unpack(tb[(p * HF + kc * KB) // 2:(p * HF + (kc + 1) * KB) // 2, :]))
                acc = part if acc is None else acc + part
                for piece in share(pieces, p * nk + kc, 7 * nk):
                    piece(part)
            ms.append(acc)
        return _join(*_comb(ms))

    PR = 16

    def lhs7_pieces(src, r, junk, fn, slot, packed):
        def piece(j, pinval):
            if pinval is not None:
                pin_to(src, junk, pinval)
            if packed:
                top = fn(_unpack(src[pl.ds(r + j * PR // 2, PR // 2), :]).astype(F32))
                bot = fn(_unpack(src[pl.ds(r + (U + j * PR) // 2, PR // 2), :]).astype(F32))
            else:
                top = fn(src[pl.ds(r + j * PR, PR), :].astype(F32))
                bot = fn(src[pl.ds(r + U + j * PR, PR), :].astype(F32))
            for p, t in enumerate(_lhs7(top[:, :HD], top[:, HD:], bot[:, :HD], bot[:, HD:])):
                ubuf[pl.ds(_mo(slot * 7 * UP + p * UP + j * (PR // 2), 8), PR // 2), :] = _pack(t)
        return [functools.partial(piece, j) for j in range(U // PR)]

    def a_prep(i, slot):
        return lhs7_pieces(xs, slot_row(i), NS_X * M + 16 * (slot & 1), _ln, slot, False)

    def a_second(i, pieces=()):
        y = ffb(tb1, pieces)
        r = _mo(i * M, M)
        x1v = xs[pl.ds(slot_row(i), M), :].astype(F32) + y
        x1[pl.ds(r, M), :] = x1v
        h = _ln(x1v)
        for sub in range(2):
            un = 2 * i + sub
            b = _div(un, UPB)
            u = un - b * UPB
            rk = _mo(b * KHP + u * RP, 8)
            h11, h12, h21, h22 = _quads(h[sub * U:(sub + 1) * U])
            blocks = (h11 + h22, h11, h22, h12 - h22, h21 - h11, h11 + h12, h21 + h22)
            for n, t in enumerate(blocks):
                kx[pl.ds(rk, RP), n * HD:(n + 1) * HD] = _pack(t)

    L_OPS = (0, 6, 1, 2, 5, 4, 3)
    V_OPS = (0, 1, 3, 4, 2, 5, 6)

    def unit_row(un):
        b = _div(un, UPB)
        return _mo(b * KHP + (un - b * UPB) * RP, 8)

    def a_third(i, kmax):
        for sub in range(2):
            rk = unit_row(2 * i + sub)
            ops = [_unpack(kx[pl.ds(rk, RP), n * HD:(n + 1) * HD]) for n in L_OPS]
            k11, k12, k21, k22 = _comb(mm7(ops, tqk))
            for n, t in enumerate((k11 + k22, k11, k21 - k22, k12 - k11, k22, k11 + k21, k12 + k22)):
                k7[pl.ds(rk, RP), n * HD:(n + 1) * HD] = _pack(t)
            n2 = jnp.maximum(jnp.sum(k11 * k11 + k12 * k12, axis=-1, keepdims=True),
                             jnp.sum(k21 * k21 + k22 * k22, axis=-1, keepdims=True))
            kmax = jnp.maximum(kmax, jnp.max(n2.reshape(R // 8, 8, 1), axis=0))
        return kmax

    with scope2('s0c'):
        c_wa1.wait()
    with scope2('s0d'):
        x_copy(1).start()
        c_wb1.start()
        prep_weight(wa_s, ta1, 0.5, 256)
    with scope2('s0e'):
        x_copy(0).wait()
        for piece in a_prep(0, 0):
            piece(None)
        ops = load7(ubuf, 0, UP)
        for s in range(NSL):
            ffa_slab(ops, ta1, s)
        x_copy(1).wait()
        x_copy(2).start()
        for piece in a_prep(1, 1):
            piece(None)
    with scope2('s0f'):
        c_wb1.wait()
    with scope2('s0g'):
        x_copy(3).start()
        for c in (c_wv, c_wo, c_dw, c_wp1, c_wp2, c_wa2):
            c.start()
        prep_weight(wb_s, tb1, 0.5, 128)
        c_wb2.start()

    def a_step(i, slot, qmax):
        ops = load7(ubuf, slot * 7 * UP, UP)
        pcs = a_prep(i + 1, 1 - slot)
        a_second(i - 1, pcs if APOS == 0 else ())
        ffa_slab(ops, ta1, 0)
        ffa_slab(ops, ta1, 1, share(pcs, 0, 3) if APOS == 2 else ())
        qmax = a_third(i - 1, qmax)
        ffa_slab(ops, ta1, 2, share(pcs, 0, 2) if APOS == 1 else share(pcs, 1, 3) if APOS == 2 else ())
        ffa_slab(ops, ta1, 3, share(pcs, 1, 2) if APOS == 1 else share(pcs, 2, 3) if APOS == 2 else ())
        return qmax

    def a_body(k, qmax):
        for t in range(2):
            i = 1 + 2 * k + t
            x_copy(i + 1).wait()
            qmax = a_step(i, (1 + t) % 2, qmax)
            x_copy(i + 3).start()
        return qmax

    assert (NB - 1) % 2 == 0
    qmax = jnp.zeros((8, 1), F32)
    with scope('loopA'):
        qmax = lax.fori_loop(0, (NB - 1) // 2, a_body, qmax)
    with scope2('seg2'):
        x_copy(NB + 1).wait()
        x_copy(NB + 2).wait()
        a_second(NB - 1)
        qmax = a_third(NB - 1, qmax)
        for c in (c_dw, c_wp1, c_wp2, c_wv, c_wo, c_wa2, c_wb2):
            c.wait()
        dwf[...] = dwb[...].astype(F32)
        store7(tvo, _quads(_dot(wt0[...], wt1[...])))

    def g_row(i):
        b = _div(i, UPB)
        return _mo(8 + b * GP + (i - b * UPB) * U, 8)

    for b in range(B):
        g[0, pl.ds(8 + b * GP, T), :] = jnp.zeros((T, 128), F32)

    def kv_ops(ref, b, r0, n, which):
        rk = _mo(b * KHP + r0, 8)
        return [_unpack(ref[pl.ds(rk, n), i * HD:(i + 1) * HD]) for i in which]

    def q_ops(un):
        rk = unit_row(un)
        return [_unpack(kx[pl.ds(rk, RP), n * HD:(n + 1) * HD]) for n in L_OPS]

    def s_blocks(qops, b, s):
        ko = kv_ops(k7, b, s * (KS // 2), KS // 2, range(7))
        return _comb([_dot_nt(qops[p], ko[p]) for p in range(7)])

    bound2 = jnp.max(qmax) * (float(D) * 1.05)

    @pl.when(jnp.logical_not(bound2 <= SAFE_BOUND * SAFE_BOUND))
    def _():
        def unit_body(i, carry):
            b = _div(i, UPB)
            qops = q_ops(i)

            def slab_body(s, m):
                c = s_blocks(qops, b, s)
                col = s * KS + lax.broadcasted_iota(jnp.int32, (R, KS), 1)
                c = [jnp.where(col < KV, t, -jnp.inf) for t in c]
                top = jnp.max(jnp.maximum(c[0], c[1]), axis=-1, keepdims=True)
                bot = jnp.max(jnp.maximum(c[2], c[3]), axis=-1, keepdims=True)
                return jnp.maximum(m[0], top), jnp.maximum(m[1], bot)

            ninf = jnp.full((R, 1), -jnp.inf, F32)
            mt, mb = lax.fori_loop(0, NS, slab_body, (ninf, ninf))
            r = g_row(i)
            g[0, pl.ds(r, R), :] = jnp.broadcast_to(mt, (R, 128))
            g[0, pl.ds(r + R, R), :] = jnp.broadcast_to(mb, (R, 128))
            return carry

        lax.fori_loop(0, NU, unit_body, 0)

    def pin(pin_i, val):
        g[0, pl.ds(pl.multiple_of(GJ + 8 * (pin_i & 1), 8), 8), :] = val

    def s_job(i, slot, pieces, pin_i):
        b = _div(i, UPB)
        r = g_row(i)
        qops = q_ops(i)
        m = [jnp.concatenate([g[0, pl.ds(r + h * R, R), :]] * (KS // 128), axis=1) for h in range(2)]
        l = [None, None]
        np_ = len(pieces)
        for s in range(NS):
            c = s_blocks(qops, b, s)
            pv = []
            for q in range(4):
                p = jnp.exp2(c[q] - m[q // 2])
                lo, hi = s * KS, (s + 1) * KS
                if hi > KV:
                    parts = []
                    for c0 in range(0, KS, 128):
                        nv = KV - (lo + c0)
                        if nv >= 128:
                            parts.append(p[:, c0:c0 + 128])
                        elif nv <= 0:
                            parts.append(jnp.zeros((R, 128), F32))
                        else:
                            lane = lax.broadcasted_iota(jnp.int32, (R, 128), 1)
                            parts.append(jnp.where(lane < nv, p[:, c0:c0 + 128], 0.0))
                    p = jnp.concatenate(parts, axis=1)
                pv.append(p)
                pbuf[slot * 4 + q, :, s * KS:(s + 1) * KS] = p
            for h in range(2):
                t = jnp.sum(pv[2 * h] + pv[2 * h + 1], axis=-1, keepdims=True)
                l[h] = t if l[h] is None else l[h] + t
            mine = share(pieces, s, NS)
            for t, piece in enumerate(mine):
                piece(pv[t % 4][(t * (R // 8)) // len(mine) * 8:, :])
        return l

    def pv_prep(slot, l, tick):
        inv = [1.0 / l[0], 1.0 / l[1]]

        def piece(j, c0, pinval):
            if pinval is not None:
                pbuf[8, pl.ds(pl.multiple_of(8 * zero[0], 8), 8), 0:128] = pinval[0:8, 0:128]
            rs, cs = slice(j * 16, (j + 1) * 16), slice(c0, c0 + PC)
            ops = _lhs7(*[pbuf[slot * 4 + q, rs, cs] * inv[q // 2][rs] for q in range(4)])
            for p in range(7):
                r0 = (slot * 7 + p) * RP + j * 8
                abuf[r0:r0 + 8, cs] = _pack(ops[p])
        return [functools.partial(piece, j, c0) for c0 in range(0, KH, PC) for j in range(R // 16)]

    def pv_job(i, slot, pieces):
        b = _div(i, UPB)
        NKG = KH // KG
        acc = [None] * 7
        for p in range(7):
            for kg in range(NKG):
                cs = slice(kg * KG, (kg + 1) * KG)
                vo, = kv_ops(kx, b, kg * (KG // 2), KG // 2, V_OPS[p:p + 1])
                part = _dot(_unpack(abuf[(slot * 7 + p) * RP:(slot * 7 + p + 1) * RP, cs]), vo)
                acc[p] = part if acc[p] is None else acc[p] + part
                mine = share(pieces, p * NKG + kg, NKG * 7)
                for t, piece in enumerate(mine):
                    j = (t * (R // 16)) // len(mine)
                    piece(part[j * 16:(j + 1) * 16, :])
        return _join(*_comb(acc))

    def post_1(k):
        attn = _join(*_comb(mm7(load7(obuf, 0, UP), tvo)))
        r = _mo(k * M, M)
        x2 = x1[pl.ds(r, M), :] + attn
        x1[pl.ds(r, M), :] = x2
        return ffa_prep(_ln(x2))

    def post_2(k, ops):
        a_top, g_top, a_bot, g_bot = _comb(mm7(ops, tp1))
        for a, bb, sub in ((a_top, g_top, 0), (a_bot, g_bot, 1)):
            gr = g_row(2 * k + sub)
            ha = a * 0.5
            gv = ha * jnp.tanh(bb * 0.5) + ha
            for c4 in range(NC4):
                g[c4, pl.ds(gr, U), :] = gv[:, c4 * 128:(c4 + 1) * 128]

    def conv_pieces(i):
        gr = g_row(i)
        r = _mo(i * (U // 2), 8)
        pieces = []
        G = CG * 8
        for c4 in range(NC4):
            cs = slice(c4 * 128, (c4 + 1) * 128)
            stt = {}

            def out_rows(k0, stt=stt, c4=c4, cs=cs):
                w = stt['w']
                if CMODE == 0:
                    acc = None
                    for j in range(K):
                        t = g[c4, pl.ds(gr + k0 - pad + j, 8), :] * w[j]
                        acc = t if acc is None else acc + t
                    return acc
                st = 2 if CMODE == 1 else 4

                def y(b, k):
                    if (b, k) not in stt:
                        acc = None
                        for j in range(b, K, st):
                            t = g[c4, pl.ds(gr + k - pad + j - b, 8), :] * w[j]
                            acc = t if acc is None else acc + t
                        stt[(b, k)] = acc
                    return stt[(b, k)]

                sub = lax.broadcasted_iota(jnp.int32, (8, 128), 0)
                acc = y(0, k0)
                for b in range(1, st):
                    lo = pltpu.roll(y(b, k0), 8 - b, 0)
                    hi = pltpu.roll(y(b, k0 + 8), 8 - b, 0)
                    acc = acc + jnp.where(sub < 8 - b, lo, hi)
                return acc

            for k in range(U // G):
                def piece(pinval, k=k, stt=stt, cs=cs, out_rows=out_rows):
                    if pinval is not None:
                        g[0, pl.ds(pl.multiple_of(GJ + 8 * (i & 1), 8), 8), :] = pinval[0:8, 0:128]
                    if k == 0:
                        stt['w'] = [dwf[pl.ds(j, 1), cs] for j in range(K)]
                    rows = []
                    for k0 in range(k * G, (k + 1) * G, 8):
                        acc = out_rows(k0)
                        rows.append(acc)
                        if k0 == 0:
                            stt['c'] = acc[0:1]
                        d = acc - stt['c']
                        stt['s1'] = d if k0 == 0 else stt['s1'] + d
                        stt['s2'] = d * d if k0 == 0 else stt['s2'] + d * d
                    dc[pl.ds(r + k * (G // 2), G // 2), cs] = _pack(jnp.concatenate(rows, axis=0))
                    if k == U // G - 1:
                        stat_c[pl.ds(_mo(i * 8, 8), 8), cs] = jnp.broadcast_to(stt['c'], (8, 128))
                        stat_1[pl.ds(_mo(i * 8, 8), 8), cs] = stt['s1']
                        stat_2[pl.ds(_mo(i * 8, 8), 8), cs] = stt['s2']
                pieces.append(piece)
        return pieces

    def conv(i):
        for p_ in conv_pieces(i):
            p_(None)

    def b_group(k, do_post, do_conv, fill=None):
        units = [2 * k, 2 * k + 1]
        if do_post:
            pops = post_1(k - 1)
        if do_conv:
            cp = conv_pieces(jnp.maximum(units[0] - 4, 0)) + conv_pieces(jnp.maximum(units[1] - 4, 1))
        else:
            cp = fill
        l0 = s_job(units[0], 0, [], k)
        prep0 = pv_prep(0, l0, k)
        if do_post:
            post_2(k - 1, pops)
        l1 = s_job(units[1], 1, prep0, k)
        prep1 = pv_prep(1, l1, k)
        nc = len(cp) * CSPLIT // 8
        os_ = [pv_job(units[0], 0, interleave(prep1, cp[:nc])), pv_job(units[1], 1, cp[nc:])]
        store_lhs7(obuf, 0, (os_[0][:, :HD], os_[0][:, HD:], os_[1][:, :HD], os_[1][:, HD:]))

    with scope2('proB'):
        wp = (weight_pieces(wp1_s, tp1, 1.0, WR) + weight_pieces(wp2_s, tp2, 1.0, WR)
              + weight_pieces(wa_s, ta2, 0.5, WR) + weight_pieces(wb_s, tb2, 0.5, WR))
        b_group(0, False, False, wp)

    def b_body(k, carry):
        b_group(k, True, True)
        return carry

    with scope('loopB'):
        lax.fori_loop(1, NB, b_body, 0)
    with scope2('tail1'):
        post_2(NB - 1, post_1(NB - 1))
    with scope2('tail2'):
        for u in range(NU - 4, NU):
            conv(u)

    acc = None
    for u in range(NU):
        t = stat_1[u * 8:(u + 1) * 8, :] + float(U // 8) * stat_c[u * 8:(u + 1) * 8, :]
        acc = t if acc is None else acc + t
    mu = jnp.sum(acc, axis=0, keepdims=True) * (1.0 / N)
    acc = None
    for u in range(NU):
        e = mu - stat_c[u * 8:(u + 1) * 8, :]
        t = stat_2[u * 8:(u + 1) * 8, :] + e * (float(U // 8) * e - 2.0 * stat_1[u * 8:(u + 1) * 8, :])
        acc = t if acc is None else acc + t
    bn[pl.ds(0, 1), :] = mu
    bn[pl.ds(1, 1), :] = lax.rsqrt(jnp.sum(acc, axis=0, keepdims=True) * (1.0 / N) + EPS)

    def bn_silu(v):
        hx = (v - bn[pl.ds(0, 1), :]) * (bn[pl.ds(1, 1), :] * 0.5)
        return hx * jnp.tanh(hx) + hx

    def d_pre(j, slot):
        return lhs7_pieces(dc, _mo(j * U, 8), N // 2 + 8 * (slot & 1), bn_silu, slot, True)

    def d_first(j, slot):
        r = _mo(j * M, M)
        x3 = x1[pl.ds(r, M), :] + _join(*_comb(mm7(load7(ubuf, _mo(slot * 7 * UP, 8), UP), tp2)))
        x1[pl.ds(r, M), :] = x3
        return ffa_prep(_ln(x3))

    def d_last(j, y):
        r = _mo(j * M, M)
        xs[pl.ds(slot_row(j), M), :] = _ln(x1[pl.ds(r, M), :] + y).astype(BF)
        o_copy(j).start()

    for j in range(NS_X):
        o_copy(j).start()
    with scope2('proD'):
        for piece in d_pre(0, 0):
            piece(None)
        ops = d_first(0, 0)
        for s in range(NSL):
            ffa_slab(ops, ta2, s)
        for piece in d_pre(1, 1):
            piece(None)

    def d_body(k, carry):
        for t in range(2):
            j = 1 + 2 * k + t
            slot = (1 + t) % 2
            o_copy(j - 1).wait()
            ops = d_first(j, slot)
            y = ffb(tb2, d_pre(jnp.minimum(j + 1, NB - 1), 1 - slot))
            d_last(j - 1, y)
            for s in range(NSL):
                ffa_slab(ops, ta2, s)
        return carry

    with scope('loopD'):
        lax.fori_loop(0, (NB - 1) // 2, d_body, 0)
    with scope2('end'):
        o_copy(NB - 1).wait()
        d_last(NB - 1, ffb(tb2))
        for j in range(NB - NS_X, NB):
            o_copy(j).wait()


def conformer(x, w_ff1_a, w_ff1_b, w_q, w_k, w_v, w_o, w_pw1, dw, w_pw2, w_ff2_a, w_ff2_b,
              *, U=160, KS=256, UA=2, UB=2, UD=2, CG=2, CMODE=2, PINMODE=1, WR=32, APOS=0, KG=256, PC=128, CSPLIT=0, interpret=False, vmem_mb=126, scopes=0):
    B, T, D = x.shape
    F = w_ff1_a.shape[1]
    K = dw.shape[0]
    N = B * T
    NU = N // U
    R = U // 2
    RP = R // 2
    KH = -(-(T // 2) // KS) * KS
    kern = functools.partial(_kernel, B=B, T=T, D=D, F=F, K=K, U=U, KH=KH, KS=KS, UA=UA, UB=UB, UD=UD,
                             CG=CG, CMODE=CMODE, PINMODE=PINMODE, WR=WR, APOS=APOS, KG=KG, PC=PC, CSPLIT=CSPLIT, scopes=scopes)
    hbm = pl.BlockSpec(memory_space=pl.ANY)
    V = pltpu.VMEM
    HD, HF = D // 2, F // 2
    scratch = [
        V((8 * U + 32, D), BF),
        V((N, D), F32),
        V((B * KH // 2, 7 * HD), U32),
        V((B * KH // 2, 7 * HD), U32),
        V((D // 128, B * (T + 8) + 8 + 16, 128), F32),
        V((N // 2 + 16, D), U32),
        V((7 * HD // 2, HF), U32), V((7 * HF // 2, HD), U32),
        V((7 * HD // 2, HF), U32), V((7 * HF // 2, HD), U32),
        V((D + 32, F), BF), V((F + 32, D), BF),
        V((D, D), BF), V((D, D), BF),
        V((D + 32, 2 * D), BF), V((D + 32, D), BF),
        V((7 * HD // 2, HD), U32), V((7 * HD // 2, HD), U32),
        V((7 * HD // 2, D), U32), V((7 * HD // 2, HD), U32),
        V((K, D), BF), V((K, D), F32),
        V((7 * U // 2, HF), U32),
        V((9, R, KH), F32),
        V((2 * 7 * RP, KH), U32),
        V((7 * U // 2, HD), U32),
        V((2 * 7 * U // 2, HD), U32),
        V((NU * 8, D), F32), V((NU * 8, D), F32), V((NU * 8, D), F32), V((8, D), F32),
        pltpu.SMEM((1,), jnp.int32),
        pltpu.SemaphoreType.DMA((11,)),
        pltpu.SemaphoreType.DMA((4,)),
        pltpu.SemaphoreType.DMA((4,)),
    ]
    out = pl.pallas_call(
        kern,
        out_shape=jax.ShapeDtypeStruct((N, D), x.dtype),
        in_specs=[hbm] * 12,
        out_specs=hbm,
        scratch_shapes=scratch,
        compiler_params=pltpu.CompilerParams(vmem_limit_bytes=vmem_mb * 1024 * 1024),
        interpret=interpret,
    )(x.reshape(N, D), w_ff1_a, w_ff1_b, w_q, w_k, w_v, w_o, w_pw1, dw, w_pw2, w_ff2_a, w_ff2_b)
    return out.reshape(B, T, D)


@jax.jit
def pallas_standalone__conformer_family_conformer__speech_kernel(
    x: jax.Array,
    w_ff1_a: jax.Array,
    w_ff1_b: jax.Array,
    w_q: jax.Array,
    w_k: jax.Array,
    w_v: jax.Array,
    w_o: jax.Array,
    w_pw1: jax.Array,
    dw: jax.Array,
    w_pw2: jax.Array,
    w_ff2_a: jax.Array,
    w_ff2_b: jax.Array,
):
    return conformer(x, w_ff1_a, w_ff1_b, w_q, w_k, w_v, w_o, w_pw1, dw, w_pw2, w_ff2_a, w_ff2_b)
```

```python
import contextlib
import functools

import numpy as np
import jax
import jax.numpy as jnp
from jax import lax
import jax.experimental.pallas as pl
import jax.experimental.pallas.tpu as pltpu

BF = jnp.bfloat16
F32 = jnp.float32
U32 = jnp.uint32
EPS = 1e-5
LOG2E = float(np.log2(np.e))
SAFE_BOUND = 60.0


def _div(i, n):
    return i // n if isinstance(i, int) else lax.div(i, jnp.int32(n))


def _mo(v, n):
    return v if isinstance(v, int) else pl.multiple_of(v, n)


def _ln(x):
    m = jnp.mean(x, axis=-1, keepdims=True)
    xc = x - m
    v = jnp.mean(xc * xc, axis=-1, keepdims=True)
    return xc * lax.rsqrt(v + EPS)


def _ln_after(x, token):
    n = x.shape[0]
    t = jnp.concatenate([token] * (n // 8), axis=0)
    s = t
    for c in range(0, x.shape[1], 128):
        s = s + x[:, c:c + 128]
    xc = x - jnp.sum(s, axis=-1, keepdims=True) * (1.0 / x.shape[1])
    v = jnp.mean(xc * xc, axis=-1, keepdims=True)
    return xc * lax.rsqrt(v + EPS)


def _pack(v):
    return pltpu.bitcast(v.astype(BF), U32)


def _unpack(v):
    return pltpu.bitcast(v, BF)


def _dot(a, b):
    return jnp.dot(a, b, preferred_element_type=F32)


def _dot_nt(a, b):
    return lax.dot_general(a, b, (((1,), (1,)), ((), ())), preferred_element_type=F32)


def _lhs7(a11, a12, a21, a22):
    return [a11 + a22, a21 + a22, a11, a22, a11 + a12, a21 - a11, a12 - a22]


def _rhs7(b11, b12, b21, b22):
    return [b11 + b22, b11, b12 - b22, b21 - b11, b22, b11 + b12, b21 + b22]


def _comb(m):
    return (m[0] + m[3] - m[4] + m[6], m[2] + m[4], m[1] + m[3], m[0] - m[1] + m[2] + m[5])


def _quads(x):
    r, h = x.shape[0] // 2, x.shape[1] // 2
    return x[:r, :h], x[:r, h:], x[r:, :h], x[r:, h:]


def _join(c11, c12, c21, c22):
    return jnp.concatenate([jnp.concatenate([c11, c12], 1), jnp.concatenate([c21, c22], 1)], 0)


def _kernel(x_hbm, wa1_hbm, wb1_hbm, wq_hbm, wk_hbm, wv_hbm, wo_hbm, wp1_hbm, dw_hbm, wp2_hbm,
            wa2_hbm, wb2_hbm, out_hbm,
            xs, x1, kx, k7, g, dc,
            ta1, tb1, ta2, tb2, wa_s, wb_s, wt0, wt1, wp1_s, wp2_s, tqk, tvo, tp1, tp2, dwb, dwf,
            sbuf, pbuf, abuf, obuf, ubuf, stat_c, stat_1, stat_2, bn,
            zero, sem_w, sem_x, sem_o,
            *, B, T, D, F, K, U, KH, KS, UA, UB, UD, CG, CMODE, PINMODE, WR, APOS, KG, PC, CSPLIT, PSPLIT, TOK, scopes):
    def scope(n):
        return jax.named_scope(n) if scopes else contextlib.nullcontext()

    def scope2(n):
        return jax.named_scope(n) if scopes == 2 else contextlib.nullcontext()

    N = B * T
    NU = N // U
    UPB = T // U
    R = U // 2
    RP = R // 2
    M = 2 * U
    UP = U // 2
    NB = N // M
    HD, HF = D // 2, F // 2
    NS = KH // KS
    KV = UPB * R
    KHP = KH // 2
    GP = T + 8
    GJ = B * GP + 8
    pad = K // 2
    NC4 = D // 128

    def wcopy(src, dst, k):
        return pltpu.make_async_copy(src, dst, sem_w.at[k])

    c_wq, c_wk = wcopy(wq_hbm, wt0, 0), wcopy(wk_hbm, wt1, 1)
    def lead(ref):
        return ref.at[pl.ds(0, ref.shape[0] - 32), :]

    c_wa1, c_wb1 = wcopy(wa1_hbm, lead(wa_s), 2), wcopy(wb1_hbm, lead(wb_s), 3)
    c_dw, c_wp1, c_wp2 = wcopy(dw_hbm, dwb, 4), wcopy(wp1_hbm, lead(wp1_s), 5), wcopy(wp2_hbm, lead(wp2_s), 6)
    c_wa2, c_wb2 = wcopy(wa2_hbm, lead(wa_s), 7), wcopy(wb2_hbm, lead(wb_s), 8)
    c_wv, c_wo = wcopy(wv_hbm, wt0, 9), wcopy(wo_hbm, wt1, 10)

    NS_X = 8
    OFF = 1 if APOS == 3 else 2

    def slot_row(i):
        return (i % NS_X) * M if isinstance(i, int) else pl.multiple_of((i & (NS_X - 1)) * M, M)

    def x_copy(i):
        src = (i if i < NB else 0) if isinstance(i, int) else jnp.where(i < NB, i, 0)
        sem = sem_x.at[i % NS_X if isinstance(i, int) else i & (NS_X - 1)]
        return pltpu.make_async_copy(x_hbm.at[pl.ds(_mo(src * M, M), M), :],
                                     xs.at[pl.ds(slot_row(i), M), :], sem)

    def o_copy(j):
        dst = (j if j >= 0 else j + NS_X) if isinstance(j, int) else jnp.where(j >= 0, j, j + NS_X)
        sem = sem_o.at[j % NS_X if isinstance(j, int) else j & (NS_X - 1)]
        return pltpu.make_async_copy(xs.at[pl.ds(slot_row(j), M), :],
                                     out_hbm.at[pl.ds(_mo(dst * M, M), M), :], sem)

    c_wq.start()
    c_wk.start()

    zero[0] = 0
    for b in range(B):
        r0 = b * KHP + KV // 2
        kx[pl.ds(r0, KHP - KV // 2), :] = jnp.zeros((KHP - KV // 2, 7 * HD), U32)
        k7[pl.ds(r0, KHP - KV // 2), :] = jnp.zeros((KHP - KV // 2, 7 * HD), U32)
    for b in range(B + 1):
        g[:, pl.ds(b * GP, 8), :] = jnp.zeros((NC4, 8, 128), F32)
    g[:, pl.ds(8 + 2 * U, 8), :] = jnp.zeros((NC4, 8, 128), F32)

    def store7(t_ref, blocks, scale=None):
        hk = blocks[0].shape[0]
        for p, t in enumerate(_rhs7(*blocks)):
            t_ref[p * hk // 2:(p + 1) * hk // 2, :] = _pack(t if scale is None else t * scale)

    def prep_weight(w_ref, t_ref, scale, cw):
        kk, nn = w_ref.shape[0] - 32, w_ref.shape[1]
        hk, hn = kk // 2, nn // 2
        for c0 in range(0, hn, cw):
            blk = [w_ref[r0:r0 + hk, cc:cc + cw].astype(F32) * scale
                   for r0 in (0, hk) for cc in (c0, hn + c0)]
            for p, t in enumerate(_rhs7(*blk)):
                t_ref[p * hk // 2:(p + 1) * hk // 2, c0:c0 + cw] = _pack(t)

    def weight_pieces(w_ref, t_ref, scale, rows):
        kk, nn = w_ref.shape[0] - 32, w_ref.shape[1]
        hk, hn = kk // 2, nn // 2

        def piece(r0, c0, n, pinval):
            if pinval is not None:
                pin_to(w_ref, kk + 16 * (n & 1), pinval)
            blk = [w_ref[rr:rr + rows, cc:cc + 128].astype(F32) * scale
                   for rr in (r0, hk + r0) for cc in (c0, hn + c0)]
            for p, t in enumerate(_rhs7(*blk)):
                t_ref[(p * hk + r0) // 2:(p * hk + r0 + rows) // 2, c0:c0 + 128] = _pack(t)

        return [functools.partial(piece, r0, c0, r0 // rows + c0 // 128)
                for c0 in range(0, hn, 128) for r0 in range(0, hk, rows)]

    with scope2('s0a'):
        c_wk.wait()
        c_wq.wait()
    with scope2('s0b'):
        x_copy(0).start()
        c_wa1.start()
        store7(tqk, _quads(_dot_nt(wt1[...], wt0[...])), LOG2E * float(D) ** -0.5)

    def mm7(ops, t_ref, cs=slice(None)):
        hk = t_ref.shape[0] // 7
        return [_dot(ops[p], _unpack(t_ref[p * hk:(p + 1) * hk, cs])) for p in range(7)]

    def load7(ref, r0, hp):
        return [_unpack(ref[pl.ds(r0 + p * hp, hp), :]) for p in range(7)]

    def store_lhs7(ref, r0, blocks, cs=slice(None)):
        hp = blocks[0].shape[0] // 2
        for p, t in enumerate(_lhs7(*blocks)):
            ref[pl.ds(r0 + p * hp, hp), cs] = _pack(t)

    SL = 256
    NSL = HF // SL

    def ffa_prep(xn):
        return [t.astype(BF) for t in _lhs7(*_quads(xn))]

    def ffa_slab(ops, ta, s, pieces=()):
        cs = slice(s * SL, (s + 1) * SL)
        ms = mm7(ops, ta, cs)
        for p in range(7):
            for piece in share(pieces, p, 7):
                piece(ms[p])
        act = [hx * jnp.tanh(hx) + hx for hx in _comb(ms)]
        store_lhs7(sbuf, 0, act, cs)

    def pin_to(ref, row, val):
        n = 16 if ref.dtype == BF else 8
        v = val[0:n, 0:128]
        ref[pl.ds(pl.multiple_of(row, n), n), 0:128] = (
            pltpu.bitcast(v, U32) if ref.dtype == U32 else v.astype(ref.dtype))

    def share(pieces, step, steps):
        return pieces[step * len(pieces) // steps:(step + 1) * len(pieces) // steps]

    def interleave(a, b):
        out, n = [], max(len(a), len(b))
        for t in range(n):
            out += share(a, t, n) + share(b, t, n)
        return out

    KB = 256

    def ffb(tb, pieces=()):
        ms = []
        nk = HF // KB
        for p in range(7):
            acc = None
            for kc in range(nk):
                part = _dot(_unpack(sbuf[p * UP:(p + 1) * UP, kc * KB:(kc + 1) * KB]),
                            _unpack(tb[(p * HF + kc * KB) // 2:(p * HF + (kc + 1) * KB) // 2, :]))
                acc = part if acc is None else acc + part
                for piece in share(pieces, p * nk + kc, 7 * nk):
                    piece(part)
            ms.append(acc)
        return _join(*_comb(ms))

    tokens = []
    PR = 16

    def lhs7_pieces(src, r, junk, fn, slot, packed):
        def piece(j, pinval):
            if pinval is not None:
                pin_to(src, junk, pinval)
            if packed:
                top = fn(_unpack(src[pl.ds(r + j * PR // 2, PR // 2), :]).astype(F32))
                bot = fn(_unpack(src[pl.ds(r + (U + j * PR) // 2, PR // 2), :]).astype(F32))
            else:
                top = fn(src[pl.ds(r + j * PR, PR), :].astype(F32))
                bot = fn(src[pl.ds(r + U + j * PR, PR), :].astype(F32))
            tokens.append(bot[8:16, 0:128])
            for p, t in enumerate(_lhs7(top[:, :HD], top[:, HD:], bot[:, :HD], bot[:, HD:])):
                ubuf[pl.ds(_mo(slot * 7 * UP + p * UP + j * (PR // 2), 8), PR // 2), :] = _pack(t)
        return [functools.partial(piece, j) for j in range(U // PR)]

    def a_prep(i, slot):
        return lhs7_pieces(xs, slot_row(i), NS_X * M + 16 * (slot & 1), _ln, slot, False)

    def a_second(i, pieces=()):
        y = ffb(tb1, pieces)
        r = _mo(i * M, M)
        x1v = xs[pl.ds(slot_row(i), M), :].astype(F32) + y
        x1[pl.ds(r, M), :] = x1v
        if pieces and TOK:
            tok = jnp.where(jnp.abs(tokens[-1]) > float(D), 1.0, 0.0)
            h = _ln_after(x1v, tok)
        else:
            h = _ln(x1v)
        for sub in range(2):
            un = 2 * i + sub
            b = _div(un, UPB)
            u = un - b * UPB
            rk = _mo(b * KHP + u * RP, 8)
            h11, h12, h21, h22 = _quads(h[sub * U:(sub + 1) * U])
            blocks = (h11 + h22, h11, h22, h12 - h22, h21 - h11, h11 + h12, h21 + h22)
            for n, t in enumerate(blocks):
                kx[pl.ds(rk, RP), n * HD:(n + 1) * HD] = _pack(t)

    L_OPS = (0, 6, 1, 2, 5, 4, 3)
    V_OPS = (0, 1, 3, 4, 2, 5, 6)

    def unit_row(un):
        b = _div(un, UPB)
        return _mo(b * KHP + (un - b * UPB) * RP, 8)

    def a_third(i, kmax):
        for sub in range(2):
            rk = unit_row(2 * i + sub)
            ops = [_unpack(kx[pl.ds(rk, RP), n * HD:(n + 1) * HD]) for n in L_OPS]
            k11, k12, k21, k22 = _comb(mm7(ops, tqk))
            for n, t in enumerate((k11 + k22, k11, k21 - k22, k12 - k11, k22, k11 + k21, k12 + k22)):
                k7[pl.ds(rk, RP), n * HD:(n + 1) * HD] = _pack(t)
            n2 = jnp.maximum(jnp.sum(k11 * k11 + k12 * k12, axis=-1, keepdims=True),
                             jnp.sum(k21 * k21 + k22 * k22, axis=-1, keepdims=True))
            kmax = jnp.maximum(kmax, jnp.max(n2.reshape(R // 8, 8, 1), axis=0))
        return kmax

    with scope2('s0c'):
        c_wa1.wait()
    with scope2('s0d'):
        x_copy(1).start()
        c_wb1.start()
        prep_weight(wa_s, ta1, 0.5, 256)
    with scope2('s0e'):
        x_copy(0).wait()
        for piece in a_prep(0, 0):
            piece(None)
        ops = load7(ubuf, 0, UP)
        for s in range(NSL):
            ffa_slab(ops, ta1, s)
        if OFF == 2:
            x_copy(1).wait()
            for piece in a_prep(1, 1):
                piece(None)
    with scope2('s0f'):
        c_wb1.wait()
    with scope2('s0g'):
        for i in range(2, OFF + 4):
            x_copy(i).start()
        for c in (c_wv, c_wo, c_dw, c_wp1, c_wp2, c_wa2):
            c.start()
        prep_weight(wb_s, tb1, 0.5, 128)
        c_wb2.start()

    def a_step(i, slot, qmax):
        if APOS == 3:
            a_second(i - 1)
            ops = ffa_prep(_ln(xs[pl.ds(slot_row(i), M), :].astype(F32)))
            ffa_slab(ops, ta1, 0)
            ffa_slab(ops, ta1, 1)
            qmax = a_third(i - 1, qmax)
            ffa_slab(ops, ta1, 2)
            ffa_slab(ops, ta1, 3)
            return qmax
        ops = load7(ubuf, _mo(slot * 7 * UP, 8), UP)
        pcs = a_prep(i + 1, 1 - slot)
        a_second(i - 1, pcs if APOS == 0 else ())
        ffa_slab(ops, ta1, 0)
        ffa_slab(ops, ta1, 1, share(pcs, 0, 3) if APOS == 2 else ())
        qmax = a_third(i - 1, qmax)
        ffa_slab(ops, ta1, 2, share(pcs, 0, 2) if APOS == 1 else share(pcs, 1, 3) if APOS == 2 else ())
        ffa_slab(ops, ta1, 3, share(pcs, 1, 2) if APOS == 1 else share(pcs, 2, 3) if APOS == 2 else ())
        return qmax

    def a_body(k, qmax):
        for t in range(UA):
            x_copy(UA * k + OFF + t).wait()
        for t in range(UA):
            x_copy(UA * k + OFF + 4 + t).start()
        for t in range(UA):
            i = 1 + UA * k + t
            qmax = a_step(i, (1 + t) % 2 if UA % 2 == 0 else i & 1, qmax)
        return qmax

    assert (NB - 1) % UA == 0
    qmax = jnp.zeros((8, 1), F32)
    with scope('loopA'):
        qmax = lax.fori_loop(0, (NB - 1) // UA, a_body, qmax)
    with scope2('seg2'):
        for i in range(NB - 1 + OFF, NB + 3 + OFF):
            x_copy(i).wait()
        a_second(NB - 1)
        qmax = a_third(NB - 1, qmax)
        for c in (c_dw, c_wp1, c_wp2, c_wv, c_wo, c_wa2, c_wb2):
            c.wait()
        dwf[...] = dwb[...].astype(F32)
        store7(tvo, _quads(_dot(wt0[...], wt1[...])))

    def g_row(i):
        b = _div(i, UPB)
        return _mo(8 + b * GP + (i - b * UPB) * U, 8)

    for b in range(B):
        g[0, pl.ds(8 + b * GP, T), :] = jnp.zeros((T, 128), F32)

    def kv_ops(ref, b, r0, n, which):
        rk = _mo(b * KHP + r0, 8)
        return [_unpack(ref[pl.ds(rk, n), i * HD:(i + 1) * HD]) for i in which]

    def q_ops(un):
        rk = unit_row(un)
        return [_unpack(kx[pl.ds(rk, RP), n * HD:(n + 1) * HD]) for n in L_OPS]

    def s_blocks(qops, b, s):
        ko = kv_ops(k7, b, s * (KS // 2), KS // 2, range(7))
        return _comb([_dot_nt(qops[p], ko[p]) for p in range(7)])

    bound2 = jnp.max(qmax) * (float(D) * 1.05)

    @pl.when(jnp.logical_not(bound2 <= SAFE_BOUND * SAFE_BOUND))
    def _():
        def unit_body(i, carry):
            b = _div(i, UPB)
            qops = q_ops(i)

            def slab_body(s, m):
                c = s_blocks(qops, b, s)
                col = s * KS + lax.broadcasted_iota(jnp.int32, (R, KS), 1)
                c = [jnp.where(col < KV, t, -jnp.inf) for t in c]
                top = jnp.max(jnp.maximum(c[0], c[1]), axis=-1, keepdims=True)
                bot = jnp.max(jnp.maximum(c[2], c[3]), axis=-1, keepdims=True)
                return jnp.maximum(m[0], top), jnp.maximum(m[1], bot)

            ninf = jnp.full((R, 1), -jnp.inf, F32)
            mt, mb = lax.fori_loop(0, NS, slab_body, (ninf, ninf))
            r = g_row(i)
            g[0, pl.ds(r, R), :] = jnp.broadcast_to(mt, (R, 128))
            g[0, pl.ds(r + R, R), :] = jnp.broadcast_to(mb, (R, 128))
            return carry

        lax.fori_loop(0, NU, unit_body, 0)

    def pin(pin_i, val):
        g[0, pl.ds(pl.multiple_of(GJ + 8 * (pin_i & 1), 8), 8), :] = val

    def s_job(i, slot, pieces, pin_i):
        b = _div(i, UPB)
        r = g_row(i)
        qops = q_ops(i)
        m = [jnp.concatenate([g[0, pl.ds(r + h * R, R), :]] * (KS // 128), axis=1) for h in range(2)]
        l = [None, None]
        np_ = len(pieces)
        for s in range(NS):
            c = s_blocks(qops, b, s)
            pv = []
            for q in range(4):
                p = jnp.exp2(c[q] - m[q // 2])
                lo, hi = s * KS, (s + 1) * KS
                if hi > KV:
                    parts = []
                    for c0 in range(0, KS, 128):
                        nv = KV - (lo + c0)
                        if nv >= 128:
                            parts.append(p[:, c0:c0 + 128])
                        elif nv <= 0:
                            parts.append(jnp.zeros((R, 128), F32))
                        else:
                            lane = lax.broadcasted_iota(jnp.int32, (R, 128), 1)
                            parts.append(jnp.where(lane < nv, p[:, c0:c0 + 128], 0.0))
                    p = jnp.concatenate(parts, axis=1)
                pv.append(p)
                pbuf[slot * 4 + q, :, s * KS:(s + 1) * KS] = p
            for h in range(2):
                t = jnp.sum(pv[2 * h] + pv[2 * h + 1], axis=-1, keepdims=True)
                l[h] = t if l[h] is None else l[h] + t
            mine = share(pieces, s, NS)
            for t, piece in enumerate(mine):
                piece(pv[t % 4][(t * (R // 8)) // len(mine) * 8:, :])
        return l

    def pv_prep(slot, l, tick):
        inv = [1.0 / l[0], 1.0 / l[1]]

        def piece(j, c0, pinval):
            if pinval is not None:
                pbuf[8, pl.ds(pl.multiple_of(8 * zero[0], 8), 8), 0:128] = pinval[0:8, 0:128]
            rs, cs = slice(j * 16, (j + 1) * 16), slice(c0, c0 + PC)
            ops = _lhs7(*[pbuf[slot * 4 + q, rs, cs] * inv[q // 2][rs] for q in range(4)])
            for p in range(7):
                r0 = (slot * 7 + p) * RP + j * 8
                abuf[r0:r0 + 8, cs] = _pack(ops[p])
        return [functools.partial(piece, j, c0) for c0 in range(0, KH, PC) for j in range(R // 16)]

    def pv_job(i, slot, pieces):
        b = _div(i, UPB)
        NKG = KH // KG
        acc = [None] * 7
        for p in range(7):
            for kg in range(NKG):
                cs = slice(kg * KG, (kg + 1) * KG)
                vo, = kv_ops(kx, b, kg * (KG // 2), KG // 2, V_OPS[p:p + 1])
                part = _dot(_unpack(abuf[(slot * 7 + p) * RP:(slot * 7 + p + 1) * RP, cs]), vo)
                acc[p] = part if acc[p] is None else acc[p] + part
                mine = share(pieces, p * NKG + kg, NKG * 7)
                for t, piece in enumerate(mine):
                    j = (t * (R // 16)) // len(mine)
                    piece(part[j * 16:(j + 1) * 16, :])
        return _join(*_comb(acc))

    def post_1(k):
        attn = _join(*_comb(mm7(load7(obuf, 0, UP), tvo)))
        r = _mo(k * M, M)
        x2 = x1[pl.ds(r, M), :] + attn
        x1[pl.ds(r, M), :] = x2
        return ffa_prep(_ln(x2))

    def post_2(k, ops, pieces=()):
        ms = mm7(ops, tp1)
        for p in range(7):
            mine = share(pieces, p, 7)
            for t, piece in enumerate(mine):
                j = (t * (U // 8)) // len(mine)
                c0 = (t % 2) * HD
                piece(ms[p][j * 8:, c0:])
        a_top, g_top, a_bot, g_bot = _comb(ms)
        for a, bb, sub in ((a_top, g_top, 0), (a_bot, g_bot, 1)):
            gr = g_row(2 * k + sub)
            ha = a * 0.5
            gv = ha * jnp.tanh(bb * 0.5) + ha
            for c4 in range(NC4):
                g[c4, pl.ds(gr, U), :] = gv[:, c4 * 128:(c4 + 1) * 128]

    def conv_pieces(i):
        gr = g_row(i)
        r = _mo(i * (U // 2), 8)
        pieces = []
        G = CG * 8
        for c4 in range(NC4):
            cs = slice(c4 * 128, (c4 + 1) * 128)
            stt = {}

            def out_rows(k0, stt=stt, c4=c4, cs=cs):
                w = stt['w']
                if CMODE == 0:
                    acc = None
                    for j in range(K):
                        t = g[c4, pl.ds(gr + k0 - pad + j, 8), :] * w[j]
                        acc = t if acc is None else acc + t
                    return acc
                st = 2 if CMODE == 1 else 4

                def y(b, k):
                    if (b, k) not in stt:
                        acc = None
                        for j in range(b, K, st):
                            t = g[c4, pl.ds(gr + k - pad + j - b, 8), :] * w[j]
                            acc = t if acc is None else acc + t
                        stt[(b, k)] = acc
                    return stt[(b, k)]

                sub = lax.broadcasted_iota(jnp.int32, (8, 128), 0)
                acc = y(0, k0)
                for b in range(1, st):
                    lo = pltpu.roll(y(b, k0), 8 - b, 0)
                    hi = pltpu.roll(y(b, k0 + 8), 8 - b, 0)
                    acc = acc + jnp.where(sub < 8 - b, lo, hi)
                return acc

            for k in range(U // G):
                def piece(pinval, k=k, stt=stt, cs=cs, out_rows=out_rows):
                    if pinval is not None:
                        g[0, pl.ds(pl.multiple_of(GJ + 8 * (i & 1), 8), 8), :] = pinval[0:8, 0:128]
                    if k == 0:
                        stt['w'] = [dwf[pl.ds(j, 1), cs] for j in range(K)]
                    rows = []
                    for k0 in range(k * G, (k + 1) * G, 8):
                        acc = out_rows(k0)
                        rows.append(acc)
                        if k0 == 0:
                            stt['c'] = acc[0:1]
                        d = acc - stt['c']
                        stt['s1'] = d if k0 == 0 else stt['s1'] + d
                        stt['s2'] = d * d if k0 == 0 else stt['s2'] + d * d
                    dc[pl.ds(r + k * (G // 2), G // 2), cs] = _pack(jnp.concatenate(rows, axis=0))
                    if k == U // G - 1:
                        stat_c[pl.ds(_mo(i * 8, 8), 8), cs] = jnp.broadcast_to(stt['c'], (8, 128))
                        stat_1[pl.ds(_mo(i * 8, 8), 8), cs] = stt['s1']
                        stat_2[pl.ds(_mo(i * 8, 8), 8), cs] = stt['s2']
                pieces.append(piece)
        return pieces

    def conv(i):
        for p_ in conv_pieces(i):
            p_(None)

    def b_group(k, do_post, do_conv, fill=None):
        units = [2 * k, 2 * k + 1]
        if do_post:
            pops = post_1(k - 1)
        if do_conv:
            cp = conv_pieces(jnp.maximum(units[0] - 4, 0)) + conv_pieces(jnp.maximum(units[1] - 4, 1))
        else:
            cp = fill
        l0 = s_job(units[0], 0, [], k)
        prep0 = pv_prep(0, l0, k)
        n0 = len(prep0) * PSPLIT // 8 if do_post else 0
        if do_post:
            post_2(k - 1, pops, prep0[:n0])
        l1 = s_job(units[1], 1, prep0[n0:], k)
        prep1 = pv_prep(1, l1, k)
        nc = len(cp) * CSPLIT // 8
        os_ = [pv_job(units[0], 0, interleave(prep1, cp[:nc])), pv_job(units[1], 1, cp[nc:])]
        store_lhs7(obuf, 0, (os_[0][:, :HD], os_[0][:, HD:], os_[1][:, :HD], os_[1][:, HD:]))

    with scope2('proB'):
        wp = (weight_pieces(wp1_s, tp1, 1.0, WR) + weight_pieces(wp2_s, tp2, 1.0, WR)
              + weight_pieces(wa_s, ta2, 0.5, WR) + weight_pieces(wb_s, tb2, 0.5, WR))
        b_group(0, False, False, wp)

    def b_body(k, carry):
        b_group(k, True, True)
        return carry

    with scope('loopB'):
        lax.fori_loop(1, NB, b_body, 0)
    with scope2('tail1'):
        post_2(NB - 1, post_1(NB - 1))
    with scope2('tail2'):
        for u in range(NU - 4, NU):
            conv(u)

    acc = None
    for u in range(NU):
        t = stat_1[u * 8:(u + 1) * 8, :] + float(U // 8) * stat_c[u * 8:(u + 1) * 8, :]
        acc = t if acc is None else acc + t
    mu = jnp.sum(acc, axis=0, keepdims=True) * (1.0 / N)
    acc = None
    for u in range(NU):
        e = mu - stat_c[u * 8:(u + 1) * 8, :]
        t = stat_2[u * 8:(u + 1) * 8, :] + e * (float(U // 8) * e - 2.0 * stat_1[u * 8:(u + 1) * 8, :])
        acc = t if acc is None else acc + t
    bn[pl.ds(0, 1), :] = mu
    bn[pl.ds(1, 1), :] = lax.rsqrt(jnp.sum(acc, axis=0, keepdims=True) * (1.0 / N) + EPS)

    def bn_silu(v):
        hx = (v - bn[pl.ds(0, 1), :]) * (bn[pl.ds(1, 1), :] * 0.5)
        return hx * jnp.tanh(hx) + hx

    def d_pre(j, slot):
        return lhs7_pieces(dc, _mo(j * U, 8), N // 2 + 8 * (slot & 1), bn_silu, slot, True)

    def d_first(j, slot):
        r = _mo(j * M, M)
        x3 = x1[pl.ds(r, M), :] + _join(*_comb(mm7(load7(ubuf, _mo(slot * 7 * UP, 8), UP), tp2)))
        x1[pl.ds(r, M), :] = x3
        return ffa_prep(_ln(x3))

    def d_last(j, y):
        r = _mo(j * M, M)
        xs[pl.ds(slot_row(j), M), :] = _ln(x1[pl.ds(r, M), :] + y).astype(BF)

    for j in range(-NS_X, -UD):
        o_copy(j).start()
    with scope2('proD'):
        for piece in d_pre(0, 0):
            piece(None)
        ops = d_first(0, 0)
        for s in range(NSL):
            ffa_slab(ops, ta2, s)
        for piece in d_pre(1, 1):
            piece(None)

    def d_body(k, carry):
        for t in range(UD):
            o_copy(UD * k + t - NS_X).wait()
        for t in range(UD):
            o_copy(UD * k + t - UD).start()
        for t in range(UD):
            j = 1 + UD * k + t
            slot = (1 + t) % 2 if UD % 2 == 0 else j & 1
            ops = d_first(j, slot)
            y = ffb(tb2, d_pre(jnp.minimum(j + 1, NB - 1), 1 - slot))
            d_last(j - 1, y)
            for s in range(NSL):
                ffa_slab(ops, ta2, s)
        return carry

    assert (NB - 1) % UD == 0
    with scope('loopD'):
        lax.fori_loop(0, (NB - 1) // UD, d_body, 0)
    with scope2('end'):
        o_copy(NB - 1 - NS_X).wait()
        for j in range(NB - 1 - UD, NB - 1):
            o_copy(j).start()
        d_last(NB - 1, ffb(tb2))
        o_copy(NB - 1).start()
        for j in range(NB - NS_X, NB):
            o_copy(j).wait()


def conformer(x, w_ff1_a, w_ff1_b, w_q, w_k, w_v, w_o, w_pw1, dw, w_pw2, w_ff2_a, w_ff2_b,
              *, U=160, KS=256, UA=1, UB=2, UD=1, CG=2, CMODE=2, PINMODE=1, WR=32, APOS=3, KG=256, PC=128, CSPLIT=0, PSPLIT=6, TOK=0, interpret=False, vmem_mb=126, scopes=0):
    B, T, D = x.shape
    F = w_ff1_a.shape[1]
    K = dw.shape[0]
    N = B * T
    NU = N // U
    R = U // 2
    RP = R // 2
    KH = -(-(T // 2) // KS) * KS
    kern = functools.partial(_kernel, B=B, T=T, D=D, F=F, K=K, U=U, KH=KH, KS=KS, UA=UA, UB=UB, UD=UD,
                             CG=CG, CMODE=CMODE, PINMODE=PINMODE, WR=WR, APOS=APOS, KG=KG, PC=PC, CSPLIT=CSPLIT, PSPLIT=PSPLIT, TOK=TOK, scopes=scopes)
    hbm = pl.BlockSpec(memory_space=pl.ANY)
    V = pltpu.VMEM
    HD, HF = D // 2, F // 2
    scratch = [
        V((16 * U + 32, D), BF),
        V((N, D), F32),
        V((B * KH // 2, 7 * HD), U32),
        V((B * KH // 2, 7 * HD), U32),
        V((D // 128, B * (T + 8) + 8 + 16, 128), F32),
        V((N // 2 + 16, D), U32),
        V((7 * HD // 2, HF), U32), V((7 * HF // 2, HD), U32),
        V((7 * HD // 2, HF), U32), V((7 * HF // 2, HD), U32),
        V((D + 32, F), BF), V((F + 32, D), BF),
        V((D, D), BF), V((D, D), BF),
        V((D + 32, 2 * D), BF), V((D + 32, D), BF),
        V((7 * HD // 2, HD), U32), V((7 * HD // 2, HD), U32),
        V((7 * HD // 2, D), U32), V((7 * HD // 2, HD), U32),
        V((K, D), BF), V((K, D), F32),
        V((7 * U // 2, HF), U32),
        V((9, R, KH), F32),
        V((2 * 7 * RP, KH), U32),
        V((7 * U // 2, HD), U32),
        V((2 * 7 * U // 2, HD), U32),
        V((NU * 8, D), F32), V((NU * 8, D), F32), V((NU * 8, D), F32), V((8, D), F32),
        pltpu.SMEM((1,), jnp.int32),
        pltpu.SemaphoreType.DMA((11,)),
        pltpu.SemaphoreType.DMA((8,)),
        pltpu.SemaphoreType.DMA((8,)),
    ]
    out = pl.pallas_call(
        kern,
        out_shape=jax.ShapeDtypeStruct((N, D), x.dtype),
        in_specs=[hbm] * 12,
        out_specs=hbm,
        scratch_shapes=scratch,
        compiler_params=pltpu.CompilerParams(vmem_limit_bytes=vmem_mb * 1024 * 1024),
        interpret=interpret,
    )(x.reshape(N, D), w_ff1_a, w_ff1_b, w_q, w_k, w_v, w_o, w_pw1, dw, w_pw2, w_ff2_a, w_ff2_b)
    return out.reshape(B, T, D)


@jax.jit
def pallas_standalone__conformer_family_conformer__speech_kernel(
    x: jax.Array,
    w_ff1_a: jax.Array,
    w_ff1_b: jax.Array,
    w_q: jax.Array,
    w_k: jax.Array,
    w_v: jax.Array,
    w_o: jax.Array,
    w_pw1: jax.Array,
    dw: jax.Array,
    w_pw2: jax.Array,
    w_ff2_a: jax.Array,
    w_ff2_b: jax.Array,
):
    return conformer(x, w_ff1_a, w_ff1_b, w_q, w_k, w_v, w_o, w_pw1, dw, w_pw2, w_ff2_a, w_ff2_b)
```

```python
import contextlib
import functools

import numpy as np
import jax
import jax.numpy as jnp
from jax import lax
import jax.experimental.pallas as pl
import jax.experimental.pallas.tpu as pltpu

BF = jnp.bfloat16
F32 = jnp.float32
U32 = jnp.uint32
EPS = 1e-5
LOG2E = float(np.log2(np.e))
SAFE_BOUND = 60.0


def _div(i, n):
    return i // n if isinstance(i, int) else lax.div(i, jnp.int32(n))


def _mo(v, n):
    return v if isinstance(v, int) else pl.multiple_of(v, n)


def _ln(x):
    m = jnp.mean(x, axis=-1, keepdims=True)
    xc = x - m
    v = jnp.mean(xc * xc, axis=-1, keepdims=True)
    return xc * lax.rsqrt(v + EPS)


def _ln_after(x, token):
    n = x.shape[0]
    t = jnp.concatenate([token] * (n // 8), axis=0)
    s = t
    for c in range(0, x.shape[1], 128):
        s = s + x[:, c:c + 128]
    xc = x - jnp.sum(s, axis=-1, keepdims=True) * (1.0 / x.shape[1])
    v = jnp.mean(xc * xc, axis=-1, keepdims=True)
    return xc * lax.rsqrt(v + EPS)


def _pack(v):
    return pltpu.bitcast(v.astype(BF), U32)


def _unpack(v):
    return pltpu.bitcast(v, BF)


def _dot(a, b):
    return jnp.dot(a, b, preferred_element_type=F32)


def _dot_nt(a, b):
    return lax.dot_general(a, b, (((1,), (1,)), ((), ())), preferred_element_type=F32)


def _lhs7(a11, a12, a21, a22):
    return [a11 + a22, a21 + a22, a11, a22, a11 + a12, a21 - a11, a12 - a22]


def _rhs7(b11, b12, b21, b22):
    return [b11 + b22, b11, b12 - b22, b21 - b11, b22, b11 + b12, b21 + b22]


def _comb(m):
    return (m[0] + m[3] - m[4] + m[6], m[2] + m[4], m[1] + m[3], m[0] - m[1] + m[2] + m[5])


def _quads(x):
    r, h = x.shape[0] // 2, x.shape[1] // 2
    return x[:r, :h], x[:r, h:], x[r:, :h], x[r:, h:]


def _join(c11, c12, c21, c22):
    return jnp.concatenate([jnp.concatenate([c11, c12], 1), jnp.concatenate([c21, c22], 1)], 0)


def _kernel(x_hbm, wa1_hbm, wb1_hbm, wq_hbm, wk_hbm, wv_hbm, wo_hbm, wp1_hbm, dw_hbm, wp2_hbm,
            wa2_hbm, wb2_hbm, out_hbm,
            xs, x1, kx, k7, g, dc,
            ta1, tb1, ta2, tb2, wa_s, wb_s, wt0, wt1, wp1_s, wp2_s, tqk, tvo, tp1, tp2, dwb, dwf,
            sbuf, pbuf, abuf, obuf, ubuf, stat_c, stat_1, stat_2, bn,
            zero, sem_w, sem_x, sem_o,
            *, B, T, D, F, K, U, KH, KS, UA, UB, UD, CG, CMODE, PINMODE, WR, APOS, KG, PC, CSPLIT, PSPLIT, TOK, scopes):
    def scope(n):
        return jax.named_scope(n) if scopes else contextlib.nullcontext()

    def scope2(n):
        return jax.named_scope(n) if scopes == 2 else contextlib.nullcontext()

    N = B * T
    NU = N // U
    UPB = T // U
    R = U // 2
    RP = R // 2
    M = 2 * U
    UP = U // 2
    NB = N // M
    HD, HF = D // 2, F // 2
    NS = KH // KS
    KV = UPB * R
    KHP = KH // 2
    GP = T + 8
    GJ = B * GP + 8
    pad = K // 2
    NC4 = D // 128

    def wcopy(src, dst, k):
        return pltpu.make_async_copy(src, dst, sem_w.at[k])

    c_wq, c_wk = wcopy(wq_hbm, wt0, 0), wcopy(wk_hbm, wt1, 1)
    def lead(ref):
        return ref.at[pl.ds(0, ref.shape[0] - 32), :]

    c_wb1 = wcopy(wb1_hbm, lead(wb_s), 3)
    c_dw, c_wp1, c_wp2 = wcopy(dw_hbm, dwb, 4), wcopy(wp1_hbm, lead(wp1_s), 5), wcopy(wp2_hbm, lead(wp2_s), 6)
    c_wa2, c_wb2 = wcopy(wa2_hbm, lead(wa_s), 7), wcopy(wb2_hbm, lead(wb_s), 8)

    def wa1_half(q):
        return [wcopy(wa1_hbm.at[:, pl.ds(c0, 512)], wa_s.at[pl.ds(0, D), pl.ds(c0, 512)], 11 + 2 * q + h)
                for h, c0 in enumerate((q * 512, F // 2 + q * 512))]

    c_wv, c_wo = wcopy(wv_hbm, wt0, 9), wcopy(wo_hbm, wt1, 10)

    NS_X = 8
    OFF = 1
    assert APOS == 3

    def slot_row(i):
        return (i % NS_X) * M if isinstance(i, int) else pl.multiple_of((i & (NS_X - 1)) * M, M)

    def x_copy(i):
        src = (i if i < NB else 0) if isinstance(i, int) else jnp.where(i < NB, i, 0)
        sem = sem_x.at[i % NS_X if isinstance(i, int) else i & (NS_X - 1)]
        return pltpu.make_async_copy(x_hbm.at[pl.ds(_mo(src * M, M), M), :],
                                     xs.at[pl.ds(slot_row(i), M), :], sem)

    def o_copy(j):
        dst = (j if j >= 0 else j + NS_X) if isinstance(j, int) else jnp.where(j >= 0, j, j + NS_X)
        sem = sem_o.at[j % NS_X if isinstance(j, int) else j & (NS_X - 1)]
        return pltpu.make_async_copy(xs.at[pl.ds(slot_row(j), M), :],
                                     out_hbm.at[pl.ds(_mo(dst * M, M), M), :], sem)

    x_copy(0).start()
    for c in wa1_half(0):
        c.start()

    zero[0] = 0
    for b in range(B):
        r0 = b * KHP + KV // 2
        kx[pl.ds(r0, KHP - KV // 2), :] = jnp.zeros((KHP - KV // 2, 7 * HD), U32)
        k7[pl.ds(r0, KHP - KV // 2), :] = jnp.zeros((KHP - KV // 2, 7 * HD), U32)
    for b in range(B + 1):
        g[:, pl.ds(b * GP, 8), :] = jnp.zeros((NC4, 8, 128), F32)
    g[:, pl.ds(8 + 2 * U, 8), :] = jnp.zeros((NC4, 8, 128), F32)

    def store7(t_ref, blocks, scale=None):
        hk = blocks[0].shape[0]
        for p, t in enumerate(_rhs7(*blocks)):
            t_ref[p * hk // 2:(p + 1) * hk // 2, :] = _pack(t if scale is None else t * scale)

    def prep_weight(w_ref, t_ref, scale, cw):
        kk, nn = w_ref.shape[0] - 32, w_ref.shape[1]
        hk, hn = kk // 2, nn // 2
        for c0 in range(0, hn, cw):
            blk = [w_ref[r0:r0 + hk, cc:cc + cw].astype(F32) * scale
                   for r0 in (0, hk) for cc in (c0, hn + c0)]
            for p, t in enumerate(_rhs7(*blk)):
                t_ref[p * hk // 2:(p + 1) * hk // 2, c0:c0 + cw] = _pack(t)

    def weight_pieces(w_ref, t_ref, scale, rows):
        kk, nn = w_ref.shape[0] - 32, w_ref.shape[1]
        hk, hn = kk // 2, nn // 2

        def piece(r0, c0, n, pinval):
            if pinval is not None:
                pin_to(w_ref, kk + 16 * (n & 1), pinval)
            blk = [w_ref[rr:rr + rows, cc:cc + 128].astype(F32) * scale
                   for rr in (r0, hk + r0) for cc in (c0, hn + c0)]
            for p, t in enumerate(_rhs7(*blk)):
                t_ref[(p * hk + r0) // 2:(p * hk + r0 + rows) // 2, c0:c0 + 128] = _pack(t)

        return [functools.partial(piece, r0, c0, r0 // rows + c0 // 128)
                for c0 in range(0, hn, 128) for r0 in range(0, hk, rows)]

    def mm7(ops, t_ref, cs=slice(None)):
        hk = t_ref.shape[0] // 7
        return [_dot(ops[p], _unpack(t_ref[p * hk:(p + 1) * hk, cs])) for p in range(7)]

    def load7(ref, r0, hp):
        return [_unpack(ref[pl.ds(r0 + p * hp, hp), :]) for p in range(7)]

    def store_lhs7(ref, r0, blocks, cs=slice(None)):
        hp = blocks[0].shape[0] // 2
        for p, t in enumerate(_lhs7(*blocks)):
            ref[pl.ds(r0 + p * hp, hp), cs] = _pack(t)

    SL = 256
    NSL = HF // SL

    def ffa_prep(xn):
        return [t.astype(BF) for t in _lhs7(*_quads(xn))]

    def ffa_slab(ops, ta, s, pieces=()):
        cs = slice(s * SL, (s + 1) * SL)
        ms = mm7(ops, ta, cs)
        for p in range(7):
            for piece in share(pieces, p, 7):
                piece(ms[p])
        act = [hx * jnp.tanh(hx) + hx for hx in _comb(ms)]
        store_lhs7(sbuf, 0, act, cs)

    def pin_to(ref, row, val):
        n = 16 if ref.dtype == BF else 8
        v = val[0:n, 0:128]
        ref[pl.ds(pl.multiple_of(row, n), n), 0:128] = (
            pltpu.bitcast(v, U32) if ref.dtype == U32 else v.astype(ref.dtype))

    def share(pieces, step, steps):
        return pieces[step * len(pieces) // steps:(step + 1) * len(pieces) // steps]

    def interleave(a, b):
        out, n = [], max(len(a), len(b))
        for t in range(n):
            out += share(a, t, n) + share(b, t, n)
        return out

    KB = 256

    def ffb(tb, pieces=()):
        ms = []
        nk = HF // KB
        for p in range(7):
            acc = None
            for kc in range(nk):
                part = _dot(_unpack(sbuf[p * UP:(p + 1) * UP, kc * KB:(kc + 1) * KB]),
                            _unpack(tb[(p * HF + kc * KB) // 2:(p * HF + (kc + 1) * KB) // 2, :]))
                acc = part if acc is None else acc + part
                for piece in share(pieces, p * nk + kc, 7 * nk):
                    piece(part)
            ms.append(acc)
        return _join(*_comb(ms))

    tokens = []
    PR = 16

    def lhs7_pieces(src, r, junk, fn, slot, packed):
        def piece(j, pinval):
            if pinval is not None:
                pin_to(src, junk, pinval)
            if packed:
                top = fn(_unpack(src[pl.ds(r + j * PR // 2, PR // 2), :]).astype(F32))
                bot = fn(_unpack(src[pl.ds(r + (U + j * PR) // 2, PR // 2), :]).astype(F32))
            else:
                top = fn(src[pl.ds(r + j * PR, PR), :].astype(F32))
                bot = fn(src[pl.ds(r + U + j * PR, PR), :].astype(F32))
            tokens.append(bot[8:16, 0:128])
            for p, t in enumerate(_lhs7(top[:, :HD], top[:, HD:], bot[:, :HD], bot[:, HD:])):
                ubuf[pl.ds(_mo(slot * 7 * UP + p * UP + j * (PR // 2), 8), PR // 2), :] = _pack(t)
        return [functools.partial(piece, j) for j in range(U // PR)]

    def a_prep(i, slot):
        return lhs7_pieces(xs, slot_row(i), NS_X * M + 16 * (slot & 1), _ln, slot, False)

    def a_second(i, pieces=()):
        y = ffb(tb1, pieces)
        r = _mo(i * M, M)
        x1v = xs[pl.ds(slot_row(i), M), :].astype(F32) + y
        x1[pl.ds(r, M), :] = x1v
        if pieces and TOK:
            tok = jnp.where(jnp.abs(tokens[-1]) > float(D), 1.0, 0.0)
            h = _ln_after(x1v, tok)
        else:
            h = _ln(x1v)
        for sub in range(2):
            un = 2 * i + sub
            b = _div(un, UPB)
            u = un - b * UPB
            rk = _mo(b * KHP + u * RP, 8)
            h11, h12, h21, h22 = _quads(h[sub * U:(sub + 1) * U])
            blocks = (h11 + h22, h11, h22, h12 - h22, h21 - h11, h11 + h12, h21 + h22)
            for n, t in enumerate(blocks):
                kx[pl.ds(rk, RP), n * HD:(n + 1) * HD] = _pack(t)

    L_OPS = (0, 6, 1, 2, 5, 4, 3)
    V_OPS = (0, 1, 3, 4, 2, 5, 6)

    def unit_row(un):
        b = _div(un, UPB)
        return _mo(b * KHP + (un - b * UPB) * RP, 8)

    def a_third(i, kmax):
        for sub in range(2):
            rk = unit_row(2 * i + sub)
            ops = [_unpack(kx[pl.ds(rk, RP), n * HD:(n + 1) * HD]) for n in L_OPS]
            k11, k12, k21, k22 = _comb(mm7(ops, tqk))
            for n, t in enumerate((k11 + k22, k11, k21 - k22, k12 - k11, k22, k11 + k21, k12 + k22)):
                k7[pl.ds(rk, RP), n * HD:(n + 1) * HD] = _pack(t)
            n2 = jnp.maximum(jnp.sum(k11 * k11 + k12 * k12, axis=-1, keepdims=True),
                             jnp.sum(k21 * k21 + k22 * k22, axis=-1, keepdims=True))
            kmax = jnp.maximum(kmax, jnp.max(n2.reshape(R // 8, 8, 1), axis=0))
        return kmax

    wp_a1 = weight_pieces(wa_s, ta1, 0.5, WR)
    nh = len(wp_a1) // 2
    with scope2('s0a'):
        x_copy(0).wait()
        for c in wa1_half(0):
            c.wait()
        for c in wa1_half(1):
            c.start()
        for c in (c_wq, c_wk, c_wb1):
            c.start()
        x_copy(1).start()
    with scope2('s0b'):
        ops = ffa_prep(_ln(xs[pl.ds(slot_row(0), M), :].astype(F32)))
        for piece in wp_a1[:nh]:
            piece(None)
        ffa_slab(ops, ta1, 0)
        ffa_slab(ops, ta1, 1)
    with scope2('s0c'):
        for c in wa1_half(1):
            c.wait()
        for piece in wp_a1[nh:]:
            piece(None)
        ffa_slab(ops, ta1, 2)
        ffa_slab(ops, ta1, 3)
    with scope2('s0d'):
        c_wq.wait()
        c_wk.wait()
        store7(tqk, _quads(_dot_nt(wt1[...], wt0[...])), LOG2E * float(D) ** -0.5)
    with scope2('s0e'):
        c_wb1.wait()
        for i in range(2, OFF + 4):
            x_copy(i).start()
        for c in (c_wv, c_wo, c_dw, c_wp1, c_wp2, c_wa2):
            c.start()
    with scope2('s0f'):
        for piece in weight_pieces(wb_s, tb1, 0.5, WR):
            piece(None)
        c_wb2.start()

    def a_step(i, slot, qmax):
        if APOS == 3:
            a_second(i - 1)
            ops = ffa_prep(_ln(xs[pl.ds(slot_row(i), M), :].astype(F32)))
            ffa_slab(ops, ta1, 0)
            ffa_slab(ops, ta1, 1)
            qmax = a_third(i - 1, qmax)
            ffa_slab(ops, ta1, 2)
            ffa_slab(ops, ta1, 3)
            return qmax
        ops = load7(ubuf, _mo(slot * 7 * UP, 8), UP)
        pcs = a_prep(i + 1, 1 - slot)
        a_second(i - 1, pcs if APOS == 0 else ())
        ffa_slab(ops, ta1, 0)
        ffa_slab(ops, ta1, 1, share(pcs, 0, 3) if APOS == 2 else ())
        qmax = a_third(i - 1, qmax)
        ffa_slab(ops, ta1, 2, share(pcs, 0, 2) if APOS == 1 else share(pcs, 1, 3) if APOS == 2 else ())
        ffa_slab(ops, ta1, 3, share(pcs, 1, 2) if APOS == 1 else share(pcs, 2, 3) if APOS == 2 else ())
        return qmax

    def a_body(k, qmax):
        for t in range(UA):
            x_copy(UA * k + OFF + t).wait()
        for t in range(UA):
            x_copy(UA * k + OFF + 4 + t).start()
        for t in range(UA):
            i = 1 + UA * k + t
            qmax = a_step(i, (1 + t) % 2 if UA % 2 == 0 else i & 1, qmax)
        return qmax

    assert (NB - 1) % UA == 0
    qmax = jnp.zeros((8, 1), F32)
    with scope('loopA'):
        qmax = lax.fori_loop(0, (NB - 1) // UA, a_body, qmax)
    with scope2('seg2'):
        for i in range(NB - 1 + OFF, NB + 3 + OFF):
            x_copy(i).wait()
        a_second(NB - 1)
        qmax = a_third(NB - 1, qmax)
        for c in (c_dw, c_wp1, c_wp2, c_wv, c_wo, c_wa2, c_wb2):
            c.wait()
        dwf[...] = dwb[...].astype(F32)
        store7(tvo, _quads(_dot(wt0[...], wt1[...])))

    def g_row(i):
        b = _div(i, UPB)
        return _mo(8 + b * GP + (i - b * UPB) * U, 8)

    for b in range(B):
        g[0, pl.ds(8 + b * GP, T), :] = jnp.zeros((T, 128), F32)

    def kv_ops(ref, b, r0, n, which):
        rk = _mo(b * KHP + r0, 8)
        return [_unpack(ref[pl.ds(rk, n), i * HD:(i + 1) * HD]) for i in which]

    def q_ops(un):
        rk = unit_row(un)
        return [_unpack(kx[pl.ds(rk, RP), n * HD:(n + 1) * HD]) for n in L_OPS]

    def s_blocks(qops, b, s):
        ko = kv_ops(k7, b, s * (KS // 2), KS // 2, range(7))
        return _comb([_dot_nt(qops[p], ko[p]) for p in range(7)])

    bound2 = jnp.max(qmax) * (float(D) * 1.05)

    @pl.when(jnp.logical_not(bound2 <= SAFE_BOUND * SAFE_BOUND))
    def _():
        def unit_body(i, carry):
            b = _div(i, UPB)
            qops = q_ops(i)

            def slab_body(s, m):
                c = s_blocks(qops, b, s)
                col = s * KS + lax.broadcasted_iota(jnp.int32, (R, KS), 1)
                c = [jnp.where(col < KV, t, -jnp.inf) for t in c]
                top = jnp.max(jnp.maximum(c[0], c[1]), axis=-1, keepdims=True)
                bot = jnp.max(jnp.maximum(c[2], c[3]), axis=-1, keepdims=True)
                return jnp.maximum(m[0], top), jnp.maximum(m[1], bot)

            ninf = jnp.full((R, 1), -jnp.inf, F32)
            mt, mb = lax.fori_loop(0, NS, slab_body, (ninf, ninf))
            r = g_row(i)
            g[0, pl.ds(r, R), :] = jnp.broadcast_to(mt, (R, 128))
            g[0, pl.ds(r + R, R), :] = jnp.broadcast_to(mb, (R, 128))
            return carry

        lax.fori_loop(0, NU, unit_body, 0)

    def pin(pin_i, val):
        g[0, pl.ds(pl.multiple_of(GJ + 8 * (pin_i & 1), 8), 8), :] = val

    def s_job(i, slot, pieces, pin_i):
        b = _div(i, UPB)
        r = g_row(i)
        qops = q_ops(i)
        m = [jnp.concatenate([g[0, pl.ds(r + h * R, R), :]] * (KS // 128), axis=1) for h in range(2)]
        l = [None, None]
        np_ = len(pieces)
        for s in range(NS):
            c = s_blocks(qops, b, s)
            pv = []
            for q in range(4):
                p = jnp.exp2(c[q] - m[q // 2])
                lo, hi = s * KS, (s + 1) * KS
                if hi > KV:
                    parts = []
                    for c0 in range(0, KS, 128):
                        nv = KV - (lo + c0)
                        if nv >= 128:
                            parts.append(p[:, c0:c0 + 128])
                        elif nv <= 0:
                            parts.append(jnp.zeros((R, 128), F32))
                        else:
                            lane = lax.broadcasted_iota(jnp.int32, (R, 128), 1)
                            parts.append(jnp.where(lane < nv, p[:, c0:c0 + 128], 0.0))
                    p = jnp.concatenate(parts, axis=1)
                pv.append(p)
                pbuf[slot * 4 + q, :, s * KS:(s + 1) * KS] = p
            for h in range(2):
                t = jnp.sum(pv[2 * h] + pv[2 * h + 1], axis=-1, keepdims=True)
                l[h] = t if l[h] is None else l[h] + t
            mine = share(pieces, s, NS)
            for t, piece in enumerate(mine):
                piece(pv[t % 4][(t * (R // 8)) // len(mine) * 8:, :])
        return l

    def pv_prep(slot, l, tick):
        inv = [1.0 / l[0], 1.0 / l[1]]

        def piece(j, c0, pinval):
            if pinval is not None:
                pbuf[8, pl.ds(pl.multiple_of(8 * zero[0], 8), 8), 0:128] = pinval[0:8, 0:128]
            rs, cs = slice(j * 16, (j + 1) * 16), slice(c0, c0 + PC)
            ops = _lhs7(*[pbuf[slot * 4 + q, rs, cs] * inv[q // 2][rs] for q in range(4)])
            for p in range(7):
                r0 = (slot * 7 + p) * RP + j * 8
                abuf[r0:r0 + 8, cs] = _pack(ops[p])
        return [functools.partial(piece, j, c0) for c0 in range(0, KH, PC) for j in range(R // 16)]

    def pv_job(i, slot, pieces):
        b = _div(i, UPB)
        NKG = KH // KG
        acc = [None] * 7
        for p in range(7):
            for kg in range(NKG):
                cs = slice(kg * KG, (kg + 1) * KG)
                vo, = kv_ops(kx, b, kg * (KG // 2), KG // 2, V_OPS[p:p + 1])
                part = _dot(_unpack(abuf[(slot * 7 + p) * RP:(slot * 7 + p + 1) * RP, cs]), vo)
                acc[p] = part if acc[p] is None else acc[p] + part
                mine = share(pieces, p * NKG + kg, NKG * 7)
                for t, piece in enumerate(mine):
                    j = (t * (R // 16)) // len(mine)
                    piece(part[j * 16:(j + 1) * 16, :])
        return _join(*_comb(acc))

    def post_1(k):
        attn = _join(*_comb(mm7(load7(obuf, 0, UP), tvo)))
        r = _mo(k * M, M)
        x2 = x1[pl.ds(r, M), :] + attn
        x1[pl.ds(r, M), :] = x2
        return ffa_prep(_ln(x2))

    def post_2(k, ops, pieces=()):
        ms = mm7(ops, tp1)
        for p in range(7):
            mine = share(pieces, p, 7)
            for t, piece in enumerate(mine):
                j = (t * (U // 8)) // len(mine)
                c0 = (t % 2) * HD
                piece(ms[p][j * 8:, c0:])
        a_top, g_top, a_bot, g_bot = _comb(ms)
        for a, bb, sub in ((a_top, g_top, 0), (a_bot, g_bot, 1)):
            gr = g_row(2 * k + sub)
            ha = a * 0.5
            gv = ha * jnp.tanh(bb * 0.5) + ha
            for c4 in range(NC4):
                g[c4, pl.ds(gr, U), :] = gv[:, c4 * 128:(c4 + 1) * 128]

    def conv_pieces(i):
        gr = g_row(i)
        r = _mo(i * (U // 2), 8)
        pieces = []
        G = CG * 8
        for c4 in range(NC4):
            cs = slice(c4 * 128, (c4 + 1) * 128)
            stt = {}

            def out_rows(k0, stt=stt, c4=c4, cs=cs):
                w = stt['w']
                if CMODE == 0:
                    acc = None
                    for j in range(K):
                        t = g[c4, pl.ds(gr + k0 - pad + j, 8), :] * w[j]
                        acc = t if acc is None else acc + t
                    return acc
                st = 2 if CMODE == 1 else 4

                def y(b, k):
                    if (b, k) not in stt:
                        acc = None
                        for j in range(b, K, st):
                            t = g[c4, pl.ds(gr + k - pad + j - b, 8), :] * w[j]
                            acc = t if acc is None else acc + t
                        stt[(b, k)] = acc
                    return stt[(b, k)]

                sub = lax.broadcasted_iota(jnp.int32, (8, 128), 0)
                acc = y(0, k0)
                for b in range(1, st):
                    lo = pltpu.roll(y(b, k0), 8 - b, 0)
                    hi = pltpu.roll(y(b, k0 + 8), 8 - b, 0)
                    acc = acc + jnp.where(sub < 8 - b, lo, hi)
                return acc

            for k in range(U // G):
                def piece(pinval, k=k, stt=stt, cs=cs, out_rows=out_rows):
                    if pinval is not None:
                        g[0, pl.ds(pl.multiple_of(GJ + 8 * (i & 1), 8), 8), :] = pinval[0:8, 0:128]
                    if k == 0:
                        stt['w'] = [dwf[pl.ds(j, 1), cs] for j in range(K)]
                    rows = []
                    for k0 in range(k * G, (k + 1) * G, 8):
                        acc = out_rows(k0)
                        rows.append(acc)
                        if k0 == 0:
                            stt['c'] = acc[0:1]
                        d = acc - stt['c']
                        stt['s1'] = d if k0 == 0 else stt['s1'] + d
                        stt['s2'] = d * d if k0 == 0 else stt['s2'] + d * d
                    dc[pl.ds(r + k * (G // 2), G // 2), cs] = _pack(jnp.concatenate(rows, axis=0))
                    if k == U // G - 1:
                        stat_c[pl.ds(_mo(i * 8, 8), 8), cs] = jnp.broadcast_to(stt['c'], (8, 128))
                        stat_1[pl.ds(_mo(i * 8, 8), 8), cs] = stt['s1']
                        stat_2[pl.ds(_mo(i * 8, 8), 8), cs] = stt['s2']
                pieces.append(piece)
        return pieces

    def conv(i):
        for p_ in conv_pieces(i):
            p_(None)

    def b_group(k, do_post, do_conv, fill=None):
        units = [2 * k, 2 * k + 1]
        if do_post:
            pops = post_1(k - 1)
        if do_conv:
            cp = conv_pieces(jnp.maximum(units[0] - 4, 0)) + conv_pieces(jnp.maximum(units[1] - 4, 1))
        else:
            cp = fill
        l0 = s_job(units[0], 0, [], k)
        prep0 = pv_prep(0, l0, k)
        n0 = len(prep0) * PSPLIT // 8 if do_post else 0
        if do_post:
            post_2(k - 1, pops, prep0[:n0])
        l1 = s_job(units[1], 1, prep0[n0:], k)
        prep1 = pv_prep(1, l1, k)
        nc = len(cp) * CSPLIT // 8
        os_ = [pv_job(units[0], 0, interleave(prep1, cp[:nc])), pv_job(units[1], 1, cp[nc:])]
        store_lhs7(obuf, 0, (os_[0][:, :HD], os_[0][:, HD:], os_[1][:, :HD], os_[1][:, HD:]))

    with scope2('proB'):
        wp = (weight_pieces(wp1_s, tp1, 1.0, WR) + weight_pieces(wp2_s, tp2, 1.0, WR)
              + weight_pieces(wa_s, ta2, 0.5, WR) + weight_pieces(wb_s, tb2, 0.5, WR))
        b_group(0, False, False, wp)

    def b_body(k, carry):
        b_group(k, True, True)
        return carry

    with scope('loopB'):
        lax.fori_loop(1, NB, b_body, 0)
    with scope2('tail1'):
        post_2(NB - 1, post_1(NB - 1))
    with scope2('tail2'):
        for u in range(NU - 4, NU):
            conv(u)

    acc = None
    for u in range(NU):
        t = stat_1[u * 8:(u + 1) * 8, :] + float(U // 8) * stat_c[u * 8:(u + 1) * 8, :]
        acc = t if acc is None else acc + t
    mu = jnp.sum(acc, axis=0, keepdims=True) * (1.0 / N)
    acc = None
    for u in range(NU):
        e = mu - stat_c[u * 8:(u + 1) * 8, :]
        t = stat_2[u * 8:(u + 1) * 8, :] + e * (float(U // 8) * e - 2.0 * stat_1[u * 8:(u + 1) * 8, :])
        acc = t if acc is None else acc + t
    bn[pl.ds(0, 1), :] = mu
    bn[pl.ds(1, 1), :] = lax.rsqrt(jnp.sum(acc, axis=0, keepdims=True) * (1.0 / N) + EPS)

    def bn_silu(v):
        hx = (v - bn[pl.ds(0, 1), :]) * (bn[pl.ds(1, 1), :] * 0.5)
        return hx * jnp.tanh(hx) + hx

    def d_pre(j, slot):
        return lhs7_pieces(dc, _mo(j * U, 8), N // 2 + 8 * (slot & 1), bn_silu, slot, True)

    def d_first(j, slot):
        r = _mo(j * M, M)
        x3 = x1[pl.ds(r, M), :] + _join(*_comb(mm7(load7(ubuf, _mo(slot * 7 * UP, 8), UP), tp2)))
        x1[pl.ds(r, M), :] = x3
        return ffa_prep(_ln(x3))

    def d_last(j, y):
        r = _mo(j * M, M)
        xs[pl.ds(slot_row(j), M), :] = _ln(x1[pl.ds(r, M), :] + y).astype(BF)

    for j in range(-NS_X, -UD):
        o_copy(j).start()
    with scope2('proD'):
        for piece in d_pre(0, 0):
            piece(None)
        ops = d_first(0, 0)
        for s in range(NSL):
            ffa_slab(ops, ta2, s)
        for piece in d_pre(1, 1):
            piece(None)

    def d_body(k, carry):
        for t in range(UD):
            o_copy(UD * k + t - NS_X).wait()
        for t in range(UD):
            o_copy(UD * k + t - UD).start()
        for t in range(UD):
            j = 1 + UD * k + t
            slot = (1 + t) % 2 if UD % 2 == 0 else j & 1
            ops = d_first(j, slot)
            y = ffb(tb2, d_pre(jnp.minimum(j + 1, NB - 1), 1 - slot))
            d_last(j - 1, y)
            for s in range(NSL):
                ffa_slab(ops, ta2, s)
        return carry

    assert (NB - 1) % UD == 0
    with scope('loopD'):
        lax.fori_loop(0, (NB - 1) // UD, d_body, 0)
    with scope2('end'):
        o_copy(NB - 1 - NS_X).wait()
        for j in range(NB - 1 - UD, NB - 1):
            o_copy(j).start()
        d_last(NB - 1, ffb(tb2))
        o_copy(NB - 1).start()
        for j in range(NB - NS_X, NB):
            o_copy(j).wait()


def conformer(x, w_ff1_a, w_ff1_b, w_q, w_k, w_v, w_o, w_pw1, dw, w_pw2, w_ff2_a, w_ff2_b,
              *, U=160, KS=256, UA=1, UB=2, UD=1, CG=2, CMODE=2, PINMODE=1, WR=32, APOS=3, KG=256, PC=128, CSPLIT=0, PSPLIT=6, TOK=0, interpret=False, vmem_mb=126, scopes=0):
    B, T, D = x.shape
    F = w_ff1_a.shape[1]
    K = dw.shape[0]
    N = B * T
    NU = N // U
    R = U // 2
    RP = R // 2
    KH = -(-(T // 2) // KS) * KS
    kern = functools.partial(_kernel, B=B, T=T, D=D, F=F, K=K, U=U, KH=KH, KS=KS, UA=UA, UB=UB, UD=UD,
                             CG=CG, CMODE=CMODE, PINMODE=PINMODE, WR=WR, APOS=APOS, KG=KG, PC=PC, CSPLIT=CSPLIT, PSPLIT=PSPLIT, TOK=TOK, scopes=scopes)
    hbm = pl.BlockSpec(memory_space=pl.ANY)
    V = pltpu.VMEM
    HD, HF = D // 2, F // 2
    scratch = [
        V((16 * U + 32, D), BF),
        V((N, D), F32),
        V((B * KH // 2, 7 * HD), U32),
        V((B * KH // 2, 7 * HD), U32),
        V((D // 128, B * (T + 8) + 8 + 16, 128), F32),
        V((N // 2 + 16, D), U32),
        V((7 * HD // 2, HF), U32), V((7 * HF // 2, HD), U32),
        V((7 * HD // 2, HF), U32), V((7 * HF // 2, HD), U32),
        V((D + 32, F), BF), V((F + 32, D), BF),
        V((D, D), BF), V((D, D), BF),
        V((D + 32, 2 * D), BF), V((D + 32, D), BF),
        V((7 * HD // 2, HD), U32), V((7 * HD // 2, HD), U32),
        V((7 * HD // 2, D), U32), V((7 * HD // 2, HD), U32),
        V((K, D), BF), V((K, D), F32),
        V((7 * U // 2, HF), U32),
        V((9, R, KH), F32),
        V((2 * 7 * RP, KH), U32),
        V((7 * U // 2, HD), U32),
        V((2 * 7 * U // 2, HD), U32),
        V((NU * 8, D), F32), V((NU * 8, D), F32), V((NU * 8, D), F32), V((8, D), F32),
        pltpu.SMEM((1,), jnp.int32),
        pltpu.SemaphoreType.DMA((19,)),
        pltpu.SemaphoreType.DMA((8,)),
        pltpu.SemaphoreType.DMA((8,)),
    ]
    out = pl.pallas_call(
        kern,
        out_shape=jax.ShapeDtypeStruct((N, D), x.dtype),
        in_specs=[hbm] * 12,
        out_specs=hbm,
        scratch_shapes=scratch,
        compiler_params=pltpu.CompilerParams(vmem_limit_bytes=vmem_mb * 1024 * 1024),
        interpret=interpret,
    )(x.reshape(N, D), w_ff1_a, w_ff1_b, w_q, w_k, w_v, w_o, w_pw1, dw, w_pw2, w_ff2_a, w_ff2_b)
    return out.reshape(B, T, D)


@jax.jit
def pallas_standalone__conformer_family_conformer__speech_kernel(
    x: jax.Array,
    w_ff1_a: jax.Array,
    w_ff1_b: jax.Array,
    w_q: jax.Array,
    w_k: jax.Array,
    w_v: jax.Array,
    w_o: jax.Array,
    w_pw1: jax.Array,
    dw: jax.Array,
    w_pw2: jax.Array,
    w_ff2_a: jax.Array,
    w_ff2_b: jax.Array,
):
    return conformer(x, w_ff1_a, w_ff1_b, w_q, w_k, w_v, w_o, w_pw1, dw, w_pw2, w_ff2_a, w_ff2_b)
```

```python
import contextlib
import functools

import numpy as np
import jax
import jax.numpy as jnp
from jax import lax
import jax.experimental.pallas as pl
import jax.experimental.pallas.tpu as pltpu

BF = jnp.bfloat16
F32 = jnp.float32
U32 = jnp.uint32
EPS = 1e-5
LOG2E = float(np.log2(np.e))
SAFE_BOUND = 60.0


def _div(i, n):
    return i // n if isinstance(i, int) else lax.div(i, jnp.int32(n))


def _mo(v, n):
    return v if isinstance(v, int) else pl.multiple_of(v, n)


def _ln(x):
    m = jnp.mean(x, axis=-1, keepdims=True)
    xc = x - m
    v = jnp.mean(xc * xc, axis=-1, keepdims=True)
    return xc * lax.rsqrt(v + EPS)


def _ln_after(x, token):
    n = x.shape[0]
    t = jnp.concatenate([token] * (n // 8), axis=0)
    s = t
    for c in range(0, x.shape[1], 128):
        s = s + x[:, c:c + 128]
    xc = x - jnp.sum(s, axis=-1, keepdims=True) * (1.0 / x.shape[1])
    v = jnp.mean(xc * xc, axis=-1, keepdims=True)
    return xc * lax.rsqrt(v + EPS)


def _pack(v):
    return pltpu.bitcast(v.astype(BF), U32)


def _unpack(v):
    return pltpu.bitcast(v, BF)


def _dot(a, b):
    return jnp.dot(a, b, preferred_element_type=F32)


def _dot_nt(a, b):
    return lax.dot_general(a, b, (((1,), (1,)), ((), ())), preferred_element_type=F32)


def _lhs7(a11, a12, a21, a22):
    return [a11 + a22, a21 + a22, a11, a22, a11 + a12, a21 - a11, a12 - a22]


def _rhs7(b11, b12, b21, b22):
    return [b11 + b22, b11, b12 - b22, b21 - b11, b22, b11 + b12, b21 + b22]


def _comb(m):
    return (m[0] + m[3] - m[4] + m[6], m[2] + m[4], m[1] + m[3], m[0] - m[1] + m[2] + m[5])


def _quads(x):
    r, h = x.shape[0] // 2, x.shape[1] // 2
    return x[:r, :h], x[:r, h:], x[r:, :h], x[r:, h:]


def _join(c11, c12, c21, c22):
    return jnp.concatenate([jnp.concatenate([c11, c12], 1), jnp.concatenate([c21, c22], 1)], 0)


def _kernel(x_hbm, wa1_hbm, wb1_hbm, wq_hbm, wk_hbm, wv_hbm, wo_hbm, wp1_hbm, dw_hbm, wp2_hbm,
            wa2_hbm, wb2_hbm, out_hbm,
            xs, x1, kx, k7, g, dc,
            ta1, tb1, ta2, tb2, wa_s, wb_s, wt0, wt1, wp1_s, wp2_s, tqk, tvo, tp1, tp2, dwb, dwf,
            sbuf, pbuf, abuf, obuf, ubuf, stat_c, stat_1, stat_2, bn,
            zero, sem_w, sem_x, sem_o,
            *, B, T, D, F, K, U, KH, KS, UA, UB, UD, CG, CMODE, PINMODE, WR, APOS, KG, PC, CSPLIT, PSPLIT, TOK, scopes):
    def scope(n):
        return jax.named_scope(n) if scopes else contextlib.nullcontext()

    def scope2(n):
        return jax.named_scope(n) if scopes == 2 else contextlib.nullcontext()

    N = B * T
    NU = N // U
    UPB = T // U
    R = U // 2
    RP = R // 2
    M = 2 * U
    UP = U // 2
    NB = N // M
    HD, HF = D // 2, F // 2
    NS = KH // KS
    KV = UPB * R
    KHP = KH // 2
    GP = T + 8
    GJ = B * GP + 8
    pad = K // 2
    NC4 = D // 128

    def wcopy(src, dst, k):
        return pltpu.make_async_copy(src, dst, sem_w.at[k])

    c_wq, c_wk = wcopy(wq_hbm, wt0, 0), wcopy(wk_hbm, wt1, 1)
    def lead(ref):
        return ref.at[pl.ds(0, ref.shape[0] - 32), :]

    c_wb1 = wcopy(wb1_hbm, lead(wb_s), 3)
    c_dw, c_wp1, c_wp2 = wcopy(dw_hbm, dwb, 4), wcopy(wp1_hbm, lead(wp1_s), 5), wcopy(wp2_hbm, lead(wp2_s), 6)
    c_wa2, c_wb2 = wcopy(wa2_hbm, lead(wa_s), 7), wcopy(wb2_hbm, lead(wb_s), 8)

    def wa1_half(q):
        return [wcopy(wa1_hbm.at[:, pl.ds(c0, 512)], wa_s.at[pl.ds(0, D), pl.ds(c0, 512)], 11 + 2 * q + h)
                for h, c0 in enumerate((q * 512, F // 2 + q * 512))]

    c_wv, c_wo = wcopy(wv_hbm, wt0, 9), wcopy(wo_hbm, wt1, 10)

    NS_X = 8
    OFF = 1
    assert APOS == 3

    def slot_row(i):
        return (i % NS_X) * M if isinstance(i, int) else pl.multiple_of((i & (NS_X - 1)) * M, M)

    def x_copy(i):
        src = (i if i < NB else 0) if isinstance(i, int) else jnp.where(i < NB, i, 0)
        sem = sem_x.at[i % NS_X if isinstance(i, int) else i & (NS_X - 1)]
        return pltpu.make_async_copy(x_hbm.at[pl.ds(_mo(src * M, M), M), :],
                                     xs.at[pl.ds(slot_row(i), M), :], sem)

    def o_copy(j):
        dst = (j if j >= 0 else j + NS_X) if isinstance(j, int) else jnp.where(j >= 0, j, j + NS_X)
        sem = sem_o.at[j % NS_X if isinstance(j, int) else j & (NS_X - 1)]
        return pltpu.make_async_copy(xs.at[pl.ds(slot_row(j), M), :],
                                     out_hbm.at[pl.ds(_mo(dst * M, M), M), :], sem)

    x_copy(0).start()
    for c in wa1_half(0):
        c.start()

    zero[0] = 0
    for b in range(B):
        r0 = b * KHP + KV // 2
        kx[pl.ds(r0, KHP - KV // 2), :] = jnp.zeros((KHP - KV // 2, 7 * HD), U32)
        k7[pl.ds(r0, KHP - KV // 2), :] = jnp.zeros((KHP - KV // 2, 7 * HD), U32)
    for b in range(B + 1):
        g[:, pl.ds(b * GP, 8), :] = jnp.zeros((NC4, 8, 128), F32)
    g[:, pl.ds(8 + 2 * U, 8), :] = jnp.zeros((NC4, 8, 128), F32)

    def store7(t_ref, blocks, scale=None):
        hk = blocks[0].shape[0]
        for p, t in enumerate(_rhs7(*blocks)):
            t_ref[p * hk // 2:(p + 1) * hk // 2, :] = _pack(t if scale is None else t * scale)

    def prep_weight(w_ref, t_ref, scale, cw):
        kk, nn = w_ref.shape[0] - 32, w_ref.shape[1]
        hk, hn = kk // 2, nn // 2
        for c0 in range(0, hn, cw):
            blk = [w_ref[r0:r0 + hk, cc:cc + cw].astype(F32) * scale
                   for r0 in (0, hk) for cc in (c0, hn + c0)]
            for p, t in enumerate(_rhs7(*blk)):
                t_ref[p * hk // 2:(p + 1) * hk // 2, c0:c0 + cw] = _pack(t)

    def weight_pieces(w_ref, t_ref, scale, rows):
        kk, nn = w_ref.shape[0] - 32, w_ref.shape[1]
        hk, hn = kk // 2, nn // 2

        def piece(r0, c0, n, pinval):
            if pinval is not None:
                pin_to(w_ref, kk + 16 * (n & 1), pinval)
            blk = [w_ref[rr:rr + rows, cc:cc + 128].astype(F32) * scale
                   for rr in (r0, hk + r0) for cc in (c0, hn + c0)]
            for p, t in enumerate(_rhs7(*blk)):
                t_ref[(p * hk + r0) // 2:(p * hk + r0 + rows) // 2, c0:c0 + 128] = _pack(t)

        return [functools.partial(piece, r0, c0, r0 // rows + c0 // 128)
                for c0 in range(0, hn, 128) for r0 in range(0, hk, rows)]

    def mm7(ops, t_ref, cs=slice(None)):
        hk = t_ref.shape[0] // 7
        return [_dot(ops[p], _unpack(t_ref[p * hk:(p + 1) * hk, cs])) for p in range(7)]

    def load7(ref, r0, hp):
        return [_unpack(ref[pl.ds(r0 + p * hp, hp), :]) for p in range(7)]

    def store_lhs7(ref, r0, blocks, cs=slice(None)):
        hp = blocks[0].shape[0] // 2
        for p, t in enumerate(_lhs7(*blocks)):
            ref[pl.ds(r0 + p * hp, hp), cs] = _pack(t)

    SL = 256
    NSL = HF // SL

    def ffa_prep(xn):
        return [t.astype(BF) for t in _lhs7(*_quads(xn))]

    def ffa_slab(ops, ta, s, pieces=()):
        cs = slice(s * SL, (s + 1) * SL)
        ms = mm7(ops, ta, cs)
        for p in range(7):
            for piece in share(pieces, p, 7):
                piece(ms[p])
        act = [hx * jnp.tanh(hx) + hx for hx in _comb(ms)]
        store_lhs7(sbuf, 0, act, cs)

    def pin_to(ref, row, val):
        n = 16 if ref.dtype == BF else 8
        v = val[0:n, 0:128]
        ref[pl.ds(pl.multiple_of(row, n), n), 0:128] = (
            pltpu.bitcast(v, U32) if ref.dtype == U32 else v.astype(ref.dtype))

    def share(pieces, step, steps):
        return pieces[step * len(pieces) // steps:(step + 1) * len(pieces) // steps]

    def interleave(a, b):
        out, n = [], max(len(a), len(b))
        for t in range(n):
            out += share(a, t, n) + share(b, t, n)
        return out

    KB = 256

    def ffb(tb, pieces=()):
        ms = []
        nk = HF // KB
        for p in range(7):
            acc = None
            for kc in range(nk):
                part = _dot(_unpack(sbuf[p * UP:(p + 1) * UP, kc * KB:(kc + 1) * KB]),
                            _unpack(tb[(p * HF + kc * KB) // 2:(p * HF + (kc + 1) * KB) // 2, :]))
                acc = part if acc is None else acc + part
                for piece in share(pieces, p * nk + kc, 7 * nk):
                    piece(part)
            ms.append(acc)
        return _join(*_comb(ms))

    tokens = []
    PR = 16

    def lhs7_pieces(src, r, junk, fn, slot, packed):
        def piece(j, pinval):
            if pinval is not None:
                pin_to(src, junk, pinval)
            if packed:
                top = fn(_unpack(src[pl.ds(r + j * PR // 2, PR // 2), :]).astype(F32))
                bot = fn(_unpack(src[pl.ds(r + (U + j * PR) // 2, PR // 2), :]).astype(F32))
            else:
                top = fn(src[pl.ds(r + j * PR, PR), :].astype(F32))
                bot = fn(src[pl.ds(r + U + j * PR, PR), :].astype(F32))
            tokens.append(bot[8:16, 0:128])
            for p, t in enumerate(_lhs7(top[:, :HD], top[:, HD:], bot[:, :HD], bot[:, HD:])):
                ubuf[pl.ds(_mo(slot * 7 * UP + p * UP + j * (PR // 2), 8), PR // 2), :] = _pack(t)
        return [functools.partial(piece, j) for j in range(U // PR)]

    def a_prep(i, slot):
        return lhs7_pieces(xs, slot_row(i), NS_X * M + 16 * (slot & 1), _ln, slot, False)

    def a_second(i, pieces=()):
        y = ffb(tb1, pieces)
        r = _mo(i * M, M)
        x1v = xs[pl.ds(slot_row(i), M), :].astype(F32) + y
        x1[pl.ds(r, M), :] = x1v
        if pieces and TOK:
            tok = jnp.where(jnp.abs(tokens[-1]) > float(D), 1.0, 0.0)
            h = _ln_after(x1v, tok)
        else:
            h = _ln(x1v)
        for sub in range(2):
            un = 2 * i + sub
            b = _div(un, UPB)
            u = un - b * UPB
            rk = _mo(b * KHP + u * RP, 8)
            h11, h12, h21, h22 = _quads(h[sub * U:(sub + 1) * U])
            blocks = (h11 + h22, h11, h22, h12 - h22, h21 - h11, h11 + h12, h21 + h22)
            for n, t in enumerate(blocks):
                kx[pl.ds(rk, RP), n * HD:(n + 1) * HD] = _pack(t)

    L_OPS = (0, 6, 1, 2, 5, 4, 3)
    V_OPS = (0, 1, 3, 4, 2, 5, 6)

    def unit_row(un):
        b = _div(un, UPB)
        return _mo(b * KHP + (un - b * UPB) * RP, 8)

    def a_third(i, kmax):
        for sub in range(2):
            rk = unit_row(2 * i + sub)
            ops = [_unpack(kx[pl.ds(rk, RP), n * HD:(n + 1) * HD]) for n in L_OPS]
            k11, k12, k21, k22 = _comb(mm7(ops, tqk))
            for n, t in enumerate((k11 + k22, k11, k21 - k22, k12 - k11, k22, k11 + k21, k12 + k22)):
                k7[pl.ds(rk, RP), n * HD:(n + 1) * HD] = _pack(t)
            n2 = jnp.maximum(jnp.sum(k11 * k11 + k12 * k12, axis=-1, keepdims=True),
                             jnp.sum(k21 * k21 + k22 * k22, axis=-1, keepdims=True))
            kmax = jnp.maximum(kmax, jnp.max(n2.reshape(R // 8, 8, 1), axis=0))
        return kmax

    wp_a1 = weight_pieces(wa_s, ta1, 0.5, WR)
    nh = len(wp_a1) // 2
    with scope2('s0a'):
        x_copy(0).wait()
        for c in wa1_half(0):
            c.wait()
        for c in wa1_half(1):
            c.start()
        for c in (c_wq, c_wk, c_wb1):
            c.start()
        x_copy(1).start()
    with scope2('s0b'):
        ops = ffa_prep(_ln(xs[pl.ds(slot_row(0), M), :].astype(F32)))
        for piece in wp_a1[:nh]:
            piece(None)
        ffa_slab(ops, ta1, 0)
        ffa_slab(ops, ta1, 1)
    with scope2('s0c'):
        for c in wa1_half(1):
            c.wait()
        for piece in wp_a1[nh:]:
            piece(None)
        ffa_slab(ops, ta1, 2)
        ffa_slab(ops, ta1, 3)
    with scope2('s0d'):
        c_wq.wait()
        c_wk.wait()
        store7(tqk, _quads(_dot_nt(wt1[...], wt0[...])), LOG2E * float(D) ** -0.5)
    with scope2('s0e'):
        c_wb1.wait()
        for i in range(2, OFF + 4):
            x_copy(i).start()
        for c in (c_wv, c_wo, c_dw, c_wp1, c_wp2, c_wa2):
            c.start()
    with scope2('s0f'):
        for piece in weight_pieces(wb_s, tb1, 0.5, WR):
            piece(None)
        c_wb2.start()

    def a_step(i, slot, qmax):
        if APOS == 3:
            a_second(i - 1)
            ops = ffa_prep(_ln(xs[pl.ds(slot_row(i), M), :].astype(F32)))
            ffa_slab(ops, ta1, 0)
            ffa_slab(ops, ta1, 1)
            qmax = a_third(i - 1, qmax)
            ffa_slab(ops, ta1, 2)
            ffa_slab(ops, ta1, 3)
            return qmax
        ops = load7(ubuf, _mo(slot * 7 * UP, 8), UP)
        pcs = a_prep(i + 1, 1 - slot)
        a_second(i - 1, pcs if APOS == 0 else ())
        ffa_slab(ops, ta1, 0)
        ffa_slab(ops, ta1, 1, share(pcs, 0, 3) if APOS == 2 else ())
        qmax = a_third(i - 1, qmax)
        ffa_slab(ops, ta1, 2, share(pcs, 0, 2) if APOS == 1 else share(pcs, 1, 3) if APOS == 2 else ())
        ffa_slab(ops, ta1, 3, share(pcs, 1, 2) if APOS == 1 else share(pcs, 2, 3) if APOS == 2 else ())
        return qmax

    def a_body(k, qmax):
        for t in range(UA):
            x_copy(UA * k + OFF + t).wait()
        for t in range(UA):
            x_copy(UA * k + OFF + 4 + t).start()
        for t in range(UA):
            i = 1 + UA * k + t
            qmax = a_step(i, (1 + t) % 2 if UA % 2 == 0 else i & 1, qmax)
        return qmax

    assert (NB - 1) % UA == 0
    qmax = jnp.zeros((8, 1), F32)
    with scope('loopA'):
        qmax = lax.fori_loop(0, (NB - 1) // UA, a_body, qmax)
    with scope2('seg2'):
        for i in range(NB - 1 + OFF, NB + 3 + OFF):
            x_copy(i).wait()
        a_second(NB - 1)
        qmax = a_third(NB - 1, qmax)
        for c in (c_dw, c_wp1, c_wp2, c_wv, c_wo, c_wa2, c_wb2):
            c.wait()
        dwf[...] = dwb[...].astype(F32)
        store7(tvo, _quads(_dot(wt0[...], wt1[...])))

    def g_row(i):
        b = _div(i, UPB)
        return _mo(8 + b * GP + (i - b * UPB) * U, 8)

    for b in range(B):
        g[0, pl.ds(8 + b * GP, T), :] = jnp.zeros((T, 128), F32)

    def kv_ops(ref, b, r0, n, which):
        rk = _mo(b * KHP + r0, 8)
        return [_unpack(ref[pl.ds(rk, n), i * HD:(i + 1) * HD]) for i in which]

    def q_ops(un):
        rk = unit_row(un)
        return [_unpack(kx[pl.ds(rk, RP), n * HD:(n + 1) * HD]) for n in L_OPS]

    def s_blocks(qops, b, s):
        ko = kv_ops(k7, b, s * (KS // 2), KS // 2, range(7))
        return _comb([_dot_nt(qops[p], ko[p]) for p in range(7)])

    bound2 = jnp.max(qmax) * (float(D) * 1.05)

    @pl.when(jnp.logical_not(bound2 <= SAFE_BOUND * SAFE_BOUND))
    def _():
        def unit_body(i, carry):
            b = _div(i, UPB)
            qops = q_ops(i)

            def slab_body(s, m):
                c = s_blocks(qops, b, s)
                col = s * KS + lax.broadcasted_iota(jnp.int32, (R, KS), 1)
                c = [jnp.where(col < KV, t, -jnp.inf) for t in c]
                top = jnp.max(jnp.maximum(c[0], c[1]), axis=-1, keepdims=True)
                bot = jnp.max(jnp.maximum(c[2], c[3]), axis=-1, keepdims=True)
                return jnp.maximum(m[0], top), jnp.maximum(m[1], bot)

            ninf = jnp.full((R, 1), -jnp.inf, F32)
            mt, mb = lax.fori_loop(0, NS, slab_body, (ninf, ninf))
            r = g_row(i)
            g[0, pl.ds(r, R), :] = jnp.broadcast_to(mt, (R, 128))
            g[0, pl.ds(r + R, R), :] = jnp.broadcast_to(mb, (R, 128))
            return carry

        lax.fori_loop(0, NU, unit_body, 0)

    def pin(pin_i, val):
        g[0, pl.ds(pl.multiple_of(GJ + 8 * (pin_i & 1), 8), 8), :] = val

    def s_job(i, slot, pieces, pin_i):
        b = _div(i, UPB)
        r = g_row(i)
        qops = q_ops(i)
        m = [jnp.concatenate([g[0, pl.ds(r + h * R, R), :]] * (KS // 128), axis=1) for h in range(2)]
        l = [None, None]
        np_ = len(pieces)
        for s in range(NS):
            c = s_blocks(qops, b, s)
            pv = []
            for q in range(4):
                p = jnp.exp2(c[q] - m[q // 2])
                lo, hi = s * KS, (s + 1) * KS
                if hi > KV:
                    parts = []
                    for c0 in range(0, KS, 128):
                        nv = KV - (lo + c0)
                        if nv >= 128:
                            parts.append(p[:, c0:c0 + 128])
                        elif nv <= 0:
                            parts.append(jnp.zeros((R, 128), F32))
                        else:
                            lane = lax.broadcasted_iota(jnp.int32, (R, 128), 1)
                            parts.append(jnp.where(lane < nv, p[:, c0:c0 + 128], 0.0))
                    p = jnp.concatenate(parts, axis=1)
                pv.append(p)
                pbuf[slot * 4 + q, :, s * KS:(s + 1) * KS] = p
            for h in range(2):
                t = jnp.sum(pv[2 * h] + pv[2 * h + 1], axis=-1, keepdims=True)
                l[h] = t if l[h] is None else l[h] + t
            mine = share(pieces, s, NS)
            for t, piece in enumerate(mine):
                piece(pv[t % 4][(t * (R // 8)) // len(mine) * 8:, :])
        return l

    def pv_prep(slot, l, tick):
        inv = [1.0 / l[0], 1.0 / l[1]]

        def piece(j, c0, pinval):
            if pinval is not None:
                pbuf[8, pl.ds(pl.multiple_of(8 * zero[0], 8), 8), 0:128] = pinval[0:8, 0:128]
            rs, cs = slice(j * 16, (j + 1) * 16), slice(c0, c0 + PC)
            ops = _lhs7(*[pbuf[slot * 4 + q, rs, cs] * inv[q // 2][rs] for q in range(4)])
            for p in range(7):
                r0 = (slot * 7 + p) * RP + j * 8
                abuf[r0:r0 + 8, cs] = _pack(ops[p])
        return [functools.partial(piece, j, c0) for c0 in range(0, KH, PC) for j in range(R // 16)]

    def pv_job(i, slot, pieces):
        b = _div(i, UPB)
        NKG = KH // KG
        acc = [None] * 7
        for p in range(7):
            for kg in range(NKG):
                cs = slice(kg * KG, (kg + 1) * KG)
                vo, = kv_ops(kx, b, kg * (KG // 2), KG // 2, V_OPS[p:p + 1])
                part = _dot(_unpack(abuf[(slot * 7 + p) * RP:(slot * 7 + p + 1) * RP, cs]), vo)
                acc[p] = part if acc[p] is None else acc[p] + part
                mine = share(pieces, p * NKG + kg, NKG * 7)
                for t, piece in enumerate(mine):
                    j = (t * (R // 16)) // len(mine)
                    piece(part[j * 16:(j + 1) * 16, :])
        return _join(*_comb(acc))

    def post_1(k):
        attn = _join(*_comb(mm7(load7(obuf, 0, UP), tvo)))
        r = _mo(k * M, M)
        x2 = x1[pl.ds(r, M), :] + attn
        x1[pl.ds(r, M), :] = x2
        return ffa_prep(_ln(x2))

    def post_2(k, ops, pieces=()):
        ms = mm7(ops, tp1)
        for p in range(7):
            mine = share(pieces, p, 7)
            for t, piece in enumerate(mine):
                j = (t * (U // 8)) // len(mine)
                c0 = (t % 2) * HD
                piece(ms[p][j * 8:, c0:])
        a_top, g_top, a_bot, g_bot = _comb(ms)
        for a, bb, sub in ((a_top, g_top, 0), (a_bot, g_bot, 1)):
            gr = g_row(2 * k + sub)
            ha = a * 0.5
            gv = ha * jnp.tanh(bb * 0.5) + ha
            for c4 in range(NC4):
                g[c4, pl.ds(gr, U), :] = gv[:, c4 * 128:(c4 + 1) * 128]

    def conv_pieces(i):
        gr = g_row(i)
        r = _mo(i * (U // 2), 8)
        pieces = []
        G = CG * 8
        for c4 in range(NC4):
            cs = slice(c4 * 128, (c4 + 1) * 128)
            stt = {}

            def out_rows(k0, stt=stt, c4=c4, cs=cs):
                w = stt['w']
                if CMODE == 0:
                    acc = None
                    for j in range(K):
                        t = g[c4, pl.ds(gr + k0 - pad + j, 8), :] * w[j]
                        acc = t if acc is None else acc + t
                    return acc
                st = 2 if CMODE == 1 else 4

                def y(b, k):
                    if (b, k) not in stt:
                        acc = None
                        for j in range(b, K, st):
                            t = g[c4, pl.ds(gr + k - pad + j - b, 8), :] * w[j]
                            acc = t if acc is None else acc + t
                        stt[(b, k)] = acc
                    return stt[(b, k)]

                sub = lax.broadcasted_iota(jnp.int32, (8, 128), 0)
                acc = y(0, k0)
                for b in range(1, st):
                    lo = pltpu.roll(y(b, k0), 8 - b, 0)
                    hi = pltpu.roll(y(b, k0 + 8), 8 - b, 0)
                    acc = acc + jnp.where(sub < 8 - b, lo, hi)
                return acc

            for k in range(U // G):
                def piece(pinval, k=k, stt=stt, cs=cs, out_rows=out_rows):
                    if pinval is not None:
                        g[0, pl.ds(pl.multiple_of(GJ + 8 * (i & 1), 8), 8), :] = pinval[0:8, 0:128]
                    if k == 0:
                        stt['w'] = [dwf[pl.ds(j, 1), cs] for j in range(K)]
                    rows = []
                    for k0 in range(k * G, (k + 1) * G, 8):
                        acc = out_rows(k0)
                        rows.append(acc)
                        if k0 == 0:
                            stt['c'] = acc[0:1]
                        d = acc - stt['c']
                        stt['s1'] = d if k0 == 0 else stt['s1'] + d
                        stt['s2'] = d * d if k0 == 0 else stt['s2'] + d * d
                    dc[pl.ds(r + k * (G // 2), G // 2), cs] = _pack(jnp.concatenate(rows, axis=0))
                    if k == U // G - 1:
                        stat_c[pl.ds(_mo(i * 8, 8), 8), cs] = jnp.broadcast_to(stt['c'], (8, 128))
                        stat_1[pl.ds(_mo(i * 8, 8), 8), cs] = stt['s1']
                        stat_2[pl.ds(_mo(i * 8, 8), 8), cs] = stt['s2']
                pieces.append(piece)
        return pieces

    def conv(i):
        for p_ in conv_pieces(i):
            p_(None)

    def b_group(k, do_post, do_conv, fill=None):
        units = [2 * k, 2 * k + 1]
        if do_post:
            pops = post_1(k - 1)
        if do_conv:
            cp = conv_pieces(jnp.maximum(units[0] - 4, 0)) + conv_pieces(jnp.maximum(units[1] - 4, 1))
        else:
            cp = fill
        l0 = s_job(units[0], 0, [], k)
        prep0 = pv_prep(0, l0, k)
        n0 = len(prep0) * PSPLIT // 8 if do_post else 0
        if do_post:
            post_2(k - 1, pops, prep0[:n0])
        l1 = s_job(units[1], 1, prep0[n0:], k)
        prep1 = pv_prep(1, l1, k)
        nc = len(cp) * CSPLIT // 8
        os_ = [pv_job(units[0], 0, interleave(prep1, cp[:nc])), pv_job(units[1], 1, cp[nc:])]
        store_lhs7(obuf, 0, (os_[0][:, :HD], os_[0][:, HD:], os_[1][:, :HD], os_[1][:, HD:]))

    with scope2('proB'):
        wp = (weight_pieces(wp1_s, tp1, 1.0, WR) + weight_pieces(wp2_s, tp2, 1.0, WR)
              + weight_pieces(wa_s, ta2, 0.5, WR) + weight_pieces(wb_s, tb2, 0.5, WR))
        b_group(0, False, False, wp)

    def b_body(k, carry):
        b_group(k, True, True)
        return carry

    with scope('loopB'):
        lax.fori_loop(1, NB, b_body, 0)
    with scope2('tail1'):
        post_2(NB - 1, post_1(NB - 1), conv_pieces(NU - 4))
    with scope2('tail2'):
        for u in range(NU - 3, NU):
            conv(u)

    acc = None
    for u in range(NU):
        t = stat_1[u * 8:(u + 1) * 8, :] + float(U // 8) * stat_c[u * 8:(u + 1) * 8, :]
        acc = t if acc is None else acc + t
    mu = jnp.sum(acc, axis=0, keepdims=True) * (1.0 / N)
    acc = None
    for u in range(NU):
        e = mu - stat_c[u * 8:(u + 1) * 8, :]
        t = stat_2[u * 8:(u + 1) * 8, :] + e * (float(U // 8) * e - 2.0 * stat_1[u * 8:(u + 1) * 8, :])
        acc = t if acc is None else acc + t
    bn[pl.ds(0, 1), :] = mu
    bn[pl.ds(1, 1), :] = lax.rsqrt(jnp.sum(acc, axis=0, keepdims=True) * (1.0 / N) + EPS)

    def bn_silu(v):
        hx = (v - bn[pl.ds(0, 1), :]) * (bn[pl.ds(1, 1), :] * 0.5)
        return hx * jnp.tanh(hx) + hx

    def d_pre(j, slot):
        return lhs7_pieces(dc, _mo(j * U, 8), N // 2 + 8 * (slot & 1), bn_silu, slot, True)

    def d_first(j, slot):
        r = _mo(j * M, M)
        x3 = x1[pl.ds(r, M), :] + _join(*_comb(mm7(load7(ubuf, _mo(slot * 7 * UP, 8), UP), tp2)))
        x1[pl.ds(r, M), :] = x3
        return ffa_prep(_ln(x3))

    def d_last(j, y):
        r = _mo(j * M, M)
        xs[pl.ds(slot_row(j), M), :] = _ln(x1[pl.ds(r, M), :] + y).astype(BF)

    for j in range(-NS_X, -UD):
        o_copy(j).start()
    with scope2('proD'):
        for piece in d_pre(0, 0):
            piece(None)
        ops = d_first(0, 0)
        pcs = d_pre(1, 1)
        for s in range(NSL):
            ffa_slab(ops, ta2, s, share(pcs, s, NSL))

    def d_body(k, carry):
        for t in range(UD):
            o_copy(UD * k + t - NS_X).wait()
        for t in range(UD):
            o_copy(UD * k + t - UD).start()
        for t in range(UD):
            j = 1 + UD * k + t
            slot = (1 + t) % 2 if UD % 2 == 0 else j & 1
            ops = d_first(j, slot)
            y = ffb(tb2, d_pre(jnp.minimum(j + 1, NB - 1), 1 - slot))
            d_last(j - 1, y)
            for s in range(NSL):
                ffa_slab(ops, ta2, s)
        return carry

    assert (NB - 1) % UD == 0
    with scope('loopD'):
        lax.fori_loop(0, (NB - 1) // UD, d_body, 0)
    with scope2('end'):
        o_copy(NB - 1 - NS_X).wait()
        for j in range(NB - 1 - UD, NB - 1):
            o_copy(j).start()
        d_last(NB - 1, ffb(tb2))
        o_copy(NB - 1).start()
        for j in range(NB - NS_X, NB):
            o_copy(j).wait()


def conformer(x, w_ff1_a, w_ff1_b, w_q, w_k, w_v, w_o, w_pw1, dw, w_pw2, w_ff2_a, w_ff2_b,
              *, U=160, KS=512, UA=1, UB=2, UD=1, CG=2, CMODE=2, PINMODE=1, WR=32, APOS=3, KG=256, PC=256, CSPLIT=0, PSPLIT=6, TOK=0, interpret=False, vmem_mb=126, scopes=0):
    B, T, D = x.shape
    F = w_ff1_a.shape[1]
    K = dw.shape[0]
    N = B * T
    NU = N // U
    R = U // 2
    RP = R // 2
    KH = -(-(T // 2) // KS) * KS
    kern = functools.partial(_kernel, B=B, T=T, D=D, F=F, K=K, U=U, KH=KH, KS=KS, UA=UA, UB=UB, UD=UD,
                             CG=CG, CMODE=CMODE, PINMODE=PINMODE, WR=WR, APOS=APOS, KG=KG, PC=PC, CSPLIT=CSPLIT, PSPLIT=PSPLIT, TOK=TOK, scopes=scopes)
    hbm = pl.BlockSpec(memory_space=pl.ANY)
    V = pltpu.VMEM
    HD, HF = D // 2, F // 2
    scratch = [
        V((16 * U + 32, D), BF),
        V((N, D), F32),
        V((B * KH // 2, 7 * HD), U32),
        V((B * KH // 2, 7 * HD), U32),
        V((D // 128, B * (T + 8) + 8 + 16, 128), F32),
        V((N // 2 + 16, D), U32),
        V((7 * HD // 2, HF), U32), V((7 * HF // 2, HD), U32),
        V((7 * HD // 2, HF), U32), V((7 * HF // 2, HD), U32),
        V((D + 32, F), BF), V((F + 32, D), BF),
        V((D, D), BF), V((D, D), BF),
        V((D + 32, 2 * D), BF), V((D + 32, D), BF),
        V((7 * HD // 2, HD), U32), V((7 * HD // 2, HD), U32),
        V((7 * HD // 2, D), U32), V((7 * HD // 2, HD), U32),
        V((K, D), BF), V((K, D), F32),
        V((7 * U // 2, HF), U32),
        V((9, R, KH), F32),
        V((2 * 7 * RP, KH), U32),
        V((7 * U // 2, HD), U32),
        V((2 * 7 * U // 2, HD), U32),
        V((NU * 8, D), F32), V((NU * 8, D), F32), V((NU * 8, D), F32), V((8, D), F32),
        pltpu.SMEM((1,), jnp.int32),
        pltpu.SemaphoreType.DMA((19,)),
        pltpu.SemaphoreType.DMA((8,)),
        pltpu.SemaphoreType.DMA((8,)),
    ]
    out = pl.pallas_call(
        kern,
        out_shape=jax.ShapeDtypeStruct((N, D), x.dtype),
        in_specs=[hbm] * 12,
        out_specs=hbm,
        scratch_shapes=scratch,
        compiler_params=pltpu.CompilerParams(vmem_limit_bytes=vmem_mb * 1024 * 1024),
        interpret=interpret,
    )(x.reshape(N, D), w_ff1_a, w_ff1_b, w_q, w_k, w_v, w_o, w_pw1, dw, w_pw2, w_ff2_a, w_ff2_b)
    return out.reshape(B, T, D)


@jax.jit
def pallas_standalone__conformer_family_conformer__speech_kernel(
    x: jax.Array,
    w_ff1_a: jax.Array,
    w_ff1_b: jax.Array,
    w_q: jax.Array,
    w_k: jax.Array,
    w_v: jax.Array,
    w_o: jax.Array,
    w_pw1: jax.Array,
    dw: jax.Array,
    w_pw2: jax.Array,
    w_ff2_a: jax.Array,
    w_ff2_b: jax.Array,
):
    return conformer(x, w_ff1_a, w_ff1_b, w_q, w_k, w_v, w_o, w_pw1, dw, w_pw2, w_ff2_a, w_ff2_b)
```

```python
import contextlib
import functools

import numpy as np
import jax
import jax.numpy as jnp
from jax import lax
import jax.experimental.pallas as pl
import jax.experimental.pallas.tpu as pltpu

BF = jnp.bfloat16
F32 = jnp.float32
U32 = jnp.uint32
EPS = 1e-5
LOG2E = float(np.log2(np.e))
SAFE_BOUND = 60.0


def _div(i, n):
    return i // n if isinstance(i, int) else lax.div(i, jnp.int32(n))


def _mo(v, n):
    return v if isinstance(v, int) else pl.multiple_of(v, n)


def _ln(x):
    m = jnp.mean(x, axis=-1, keepdims=True)
    xc = x - m
    v = jnp.mean(xc * xc, axis=-1, keepdims=True)
    return xc * lax.rsqrt(v + EPS)


def _ln_after(x, token):
    n = x.shape[0]
    t = jnp.concatenate([token] * (n // 8), axis=0)
    s = t
    for c in range(0, x.shape[1], 128):
        s = s + x[:, c:c + 128]
    xc = x - jnp.sum(s, axis=-1, keepdims=True) * (1.0 / x.shape[1])
    v = jnp.mean(xc * xc, axis=-1, keepdims=True)
    return xc * lax.rsqrt(v + EPS)


def _pack(v):
    return pltpu.bitcast(v.astype(BF), U32)


def _unpack(v):
    return pltpu.bitcast(v, BF)


def _dot(a, b):
    return jnp.dot(a, b, preferred_element_type=F32)


def _dot_nt(a, b):
    return lax.dot_general(a, b, (((1,), (1,)), ((), ())), preferred_element_type=F32)


def _lhs7(a11, a12, a21, a22):
    return [a11 + a22, a21 + a22, a11, a22, a11 + a12, a21 - a11, a12 - a22]


def _rhs7(b11, b12, b21, b22):
    return [b11 + b22, b11, b12 - b22, b21 - b11, b22, b11 + b12, b21 + b22]


def _comb(m):
    return (m[0] + m[3] - m[4] + m[6], m[2] + m[4], m[1] + m[3], m[0] - m[1] + m[2] + m[5])


def _quads(x):
    r, h = x.shape[0] // 2, x.shape[1] // 2
    return x[:r, :h], x[:r, h:], x[r:, :h], x[r:, h:]


def _join(c11, c12, c21, c22):
    return jnp.concatenate([jnp.concatenate([c11, c12], 1), jnp.concatenate([c21, c22], 1)], 0)


def _kernel(x_hbm, wa1_hbm, wb1_hbm, wq_hbm, wk_hbm, wv_hbm, wo_hbm, wp1_hbm, dw_hbm, wp2_hbm,
            wa2_hbm, wb2_hbm, out_hbm,
            xs, x1, kx, k7, g, dc,
            ta1, tb1, ta2, tb2, wa_s, wb_s, wt0, wt1, wp1_s, wp2_s, tqk, tvo, tp1, tp2, dwb, dwf,
            sbuf, pbuf, abuf, obuf, ubuf, stat_c, stat_1, stat_2, bn,
            zero, sem_w, sem_x, sem_o,
            *, B, T, D, F, K, U, KH, KS, UA, UB, UD, CG, CMODE, PINMODE, WR, APOS, KG, PC, CSPLIT, PSPLIT, TOK, KB, SL, KPOS, DORD, scopes):
    def scope(n):
        return jax.named_scope(n) if scopes else contextlib.nullcontext()

    def scope2(n):
        return jax.named_scope(n) if scopes == 2 else contextlib.nullcontext()

    N = B * T
    NU = N // U
    UPB = T // U
    R = U // 2
    RP = R // 2
    M = 2 * U
    UP = U // 2
    NB = N // M
    HD, HF = D // 2, F // 2
    NS = KH // KS
    KV = UPB * R
    KHP = KH // 2
    GP = T + 8
    GJ = B * GP + 8
    pad = K // 2
    NC4 = D // 128

    def wcopy(src, dst, k):
        return pltpu.make_async_copy(src, dst, sem_w.at[k])

    c_wq, c_wk = wcopy(wq_hbm, wt0, 0), wcopy(wk_hbm, wt1, 1)
    def lead(ref):
        return ref.at[pl.ds(0, ref.shape[0] - 32), :]

    c_wb1 = wcopy(wb1_hbm, lead(wb_s), 3)
    c_dw, c_wp1, c_wp2 = wcopy(dw_hbm, dwb, 4), wcopy(wp1_hbm, lead(wp1_s), 5), wcopy(wp2_hbm, lead(wp2_s), 6)
    c_wa2, c_wb2 = wcopy(wa2_hbm, lead(wa_s), 7), wcopy(wb2_hbm, lead(wb_s), 8)

    def wa1_half(q):
        return [wcopy(wa1_hbm.at[:, pl.ds(c0, 512)], wa_s.at[pl.ds(0, D), pl.ds(c0, 512)], 11 + 2 * q + h)
                for h, c0 in enumerate((q * 512, F // 2 + q * 512))]

    c_wv, c_wo = wcopy(wv_hbm, wt0, 9), wcopy(wo_hbm, wt1, 10)

    NS_X = 8
    OFF = 1
    assert APOS == 3

    def slot_row(i):
        return (i % NS_X) * M if isinstance(i, int) else pl.multiple_of((i & (NS_X - 1)) * M, M)

    def x_copy(i):
        src = (i if i < NB else 0) if isinstance(i, int) else jnp.where(i < NB, i, 0)
        sem = sem_x.at[i % NS_X if isinstance(i, int) else i & (NS_X - 1)]
        return pltpu.make_async_copy(x_hbm.at[pl.ds(_mo(src * M, M), M), :],
                                     xs.at[pl.ds(slot_row(i), M), :], sem)

    def o_copy(j):
        dst = (j if j >= 0 else j + NS_X) if isinstance(j, int) else jnp.where(j >= 0, j, j + NS_X)
        sem = sem_o.at[j % NS_X if isinstance(j, int) else j & (NS_X - 1)]
        return pltpu.make_async_copy(xs.at[pl.ds(slot_row(j), M), :],
                                     out_hbm.at[pl.ds(_mo(dst * M, M), M), :], sem)

    x_copy(0).start()
    for c in wa1_half(0):
        c.start()

    zero[0] = 0
    for b in range(B):
        r0 = b * KHP + KV // 2
        kx[pl.ds(r0, KHP - KV // 2), :] = jnp.zeros((KHP - KV // 2, 7 * HD), U32)
        k7[pl.ds(r0, KHP - KV // 2), :] = jnp.zeros((KHP - KV // 2, 7 * HD), U32)
    for b in range(B + 1):
        g[:, pl.ds(b * GP, 8), :] = jnp.zeros((NC4, 8, 128), F32)
    g[0, pl.ds(0, GJ), :] = jnp.zeros((GJ, 128), F32)
    g[:, pl.ds(8 + 2 * U, 8), :] = jnp.zeros((NC4, 8, 128), F32)

    def store7(t_ref, blocks, scale=None):
        hk = blocks[0].shape[0]
        for p, t in enumerate(_rhs7(*blocks)):
            t_ref[p * hk // 2:(p + 1) * hk // 2, :] = _pack(t if scale is None else t * scale)

    def prep_weight(w_ref, t_ref, scale, cw):
        kk, nn = w_ref.shape[0] - 32, w_ref.shape[1]
        hk, hn = kk // 2, nn // 2
        for c0 in range(0, hn, cw):
            blk = [w_ref[r0:r0 + hk, cc:cc + cw].astype(F32) * scale
                   for r0 in (0, hk) for cc in (c0, hn + c0)]
            for p, t in enumerate(_rhs7(*blk)):
                t_ref[p * hk // 2:(p + 1) * hk // 2, c0:c0 + cw] = _pack(t)

    def weight_pieces(w_ref, t_ref, scale, rows):
        kk, nn = w_ref.shape[0] - 32, w_ref.shape[1]
        hk, hn = kk // 2, nn // 2

        def piece(r0, c0, n, pinval):
            if pinval is not None:
                pin_to(w_ref, kk + 16 * (n & 1), pinval)
            blk = [w_ref[rr:rr + rows, cc:cc + 128].astype(F32) * scale
                   for rr in (r0, hk + r0) for cc in (c0, hn + c0)]
            for p, t in enumerate(_rhs7(*blk)):
                t_ref[(p * hk + r0) // 2:(p * hk + r0 + rows) // 2, c0:c0 + 128] = _pack(t)

        return [functools.partial(piece, r0, c0, r0 // rows + c0 // 128)
                for c0 in range(0, hn, 128) for r0 in range(0, hk, rows)]

    def mm7(ops, t_ref, cs=slice(None)):
        hk = t_ref.shape[0] // 7
        return [_dot(ops[p], _unpack(t_ref[p * hk:(p + 1) * hk, cs])) for p in range(7)]

    def load7(ref, r0, hp):
        return [_unpack(ref[pl.ds(r0 + p * hp, hp), :]) for p in range(7)]

    def store_lhs7(ref, r0, blocks, cs=slice(None)):
        hp = blocks[0].shape[0] // 2
        for p, t in enumerate(_lhs7(*blocks)):
            ref[pl.ds(r0 + p * hp, hp), cs] = _pack(t)

    NSL = HF // SL

    def ffa_prep(xn):
        return [t.astype(BF) for t in _lhs7(*_quads(xn))]

    def ffa_slab(ops, ta, s, pieces=()):
        cs = slice(s * SL, (s + 1) * SL)
        ms = mm7(ops, ta, cs)
        for p in range(7):
            for piece in share(pieces, p, 7):
                piece(ms[p])
        act = [hx * jnp.tanh(hx) + hx for hx in _comb(ms)]
        store_lhs7(sbuf, 0, act, cs)

    def pin_to(ref, row, val):
        n = 16 if ref.dtype == BF else 8
        v = val[0:n, 0:128]
        ref[pl.ds(pl.multiple_of(row, n), n), 0:128] = (
            pltpu.bitcast(v, U32) if ref.dtype == U32 else v.astype(ref.dtype))

    def share(pieces, step, steps):
        return pieces[step * len(pieces) // steps:(step + 1) * len(pieces) // steps]

    def interleave(a, b):
        out, n = [], max(len(a), len(b))
        for t in range(n):
            out += share(a, t, n) + share(b, t, n)
        return out


    def ffb(tb, pieces=()):
        ms = []
        nk = HF // KB
        for p in range(7):
            acc = None
            for kc in range(nk):
                part = _dot(_unpack(sbuf[p * UP:(p + 1) * UP, kc * KB:(kc + 1) * KB]),
                            _unpack(tb[(p * HF + kc * KB) // 2:(p * HF + (kc + 1) * KB) // 2, :]))
                acc = part if acc is None else acc + part
                for piece in share(pieces, p * nk + kc, 7 * nk):
                    piece(part)
            ms.append(acc)
        return _join(*_comb(ms))

    tokens = []
    PR = 16

    def lhs7_pieces(src, r, junk, fn, slot, packed):
        def piece(j, pinval):
            if pinval is not None:
                pin_to(src, junk, pinval)
            if packed:
                top = fn(_unpack(src[pl.ds(r + j * PR // 2, PR // 2), :]).astype(F32))
                bot = fn(_unpack(src[pl.ds(r + (U + j * PR) // 2, PR // 2), :]).astype(F32))
            else:
                top = fn(src[pl.ds(r + j * PR, PR), :].astype(F32))
                bot = fn(src[pl.ds(r + U + j * PR, PR), :].astype(F32))
            tokens.append(bot[8:16, 0:128])
            for p, t in enumerate(_lhs7(top[:, :HD], top[:, HD:], bot[:, :HD], bot[:, HD:])):
                ubuf[pl.ds(_mo(slot * 7 * UP + p * UP + j * (PR // 2), 8), PR // 2), :] = _pack(t)
        return [functools.partial(piece, j) for j in range(U // PR)]

    def a_prep(i, slot):
        return lhs7_pieces(xs, slot_row(i), NS_X * M + 16 * (slot & 1), _ln, slot, False)

    def a_second(i, pieces=()):
        y = ffb(tb1, pieces)
        r = _mo(i * M, M)
        x1v = xs[pl.ds(slot_row(i), M), :].astype(F32) + y
        x1[pl.ds(r, M), :] = x1v
        if pieces and TOK:
            tok = jnp.where(jnp.abs(tokens[-1]) > float(D), 1.0, 0.0)
            h = _ln_after(x1v, tok)
        else:
            h = _ln(x1v)
        for sub in range(2):
            un = 2 * i + sub
            b = _div(un, UPB)
            u = un - b * UPB
            rk = _mo(b * KHP + u * RP, 8)
            h11, h12, h21, h22 = _quads(h[sub * U:(sub + 1) * U])
            blocks = (h11 + h22, h11, h22, h12 - h22, h21 - h11, h11 + h12, h21 + h22)
            for n, t in enumerate(blocks):
                kx[pl.ds(rk, RP), n * HD:(n + 1) * HD] = _pack(t)

    L_OPS = (0, 6, 1, 2, 5, 4, 3)
    V_OPS = (0, 1, 3, 4, 2, 5, 6)

    def unit_row(un):
        b = _div(un, UPB)
        return _mo(b * KHP + (un - b * UPB) * RP, 8)

    def a_third(i, kmax):
        for sub in range(2):
            rk = unit_row(2 * i + sub)
            ops = [_unpack(kx[pl.ds(rk, RP), n * HD:(n + 1) * HD]) for n in L_OPS]
            k11, k12, k21, k22 = _comb(mm7(ops, tqk))
            for n, t in enumerate((k11 + k22, k11, k21 - k22, k12 - k11, k22, k11 + k21, k12 + k22)):
                k7[pl.ds(rk, RP), n * HD:(n + 1) * HD] = _pack(t)
            n2 = jnp.maximum(jnp.sum(k11 * k11 + k12 * k12, axis=-1, keepdims=True),
                             jnp.sum(k21 * k21 + k22 * k22, axis=-1, keepdims=True))
            kmax = jnp.maximum(kmax, jnp.max(n2.reshape(R // 8, 8, 1), axis=0))
        return kmax

    wp_a1 = weight_pieces(wa_s, ta1, 0.5, WR)
    nh = len(wp_a1) // 2
    with scope2('s0a'):
        x_copy(0).wait()
        for c in wa1_half(0):
            c.wait()
        for c in wa1_half(1):
            c.start()
        for c in (c_wb1, c_wq, c_wk):
            c.start()
        x_copy(1).start()
    with scope2('s0b'):
        ops = ffa_prep(_ln(xs[pl.ds(slot_row(0), M), :].astype(F32)))
        for piece in wp_a1[:nh]:
            piece(None)
        for s in range(NSL // 2):
            ffa_slab(ops, ta1, s)
    with scope2('s0c'):
        for c in wa1_half(1):
            c.wait()
        for piece in wp_a1[nh:]:
            piece(None)
        for s in range(NSL // 2, NSL):
            ffa_slab(ops, ta1, s)
    with scope2('s0d'):
        c_wb1.wait()
        for piece in weight_pieces(wb_s, tb1, 0.5, WR):
            piece(None)
    with scope2('s0e'):
        c_wq.wait()
        c_wk.wait()
        for i in range(2, OFF + 4):
            x_copy(i).start()
        for c in (c_dw, c_wp1, c_wp2, c_wa2, c_wb2):
            c.start()
    with scope2('s0f'):
        store7(tqk, _quads(_dot_nt(wt1[...], wt0[...])), LOG2E * float(D) ** -0.5)
        c_wv.start()
        c_wo.start()

    def a_step(i, slot, qmax):
        if APOS == 3:
            a_second(i - 1)
            ops = ffa_prep(_ln(xs[pl.ds(slot_row(i), M), :].astype(F32)))
            for s in range(NSL):
                if s == KPOS:
                    qmax = a_third(i - 1, qmax)
                ffa_slab(ops, ta1, s)
            if KPOS >= NSL:
                qmax = a_third(i - 1, qmax)
            return qmax
        ops = load7(ubuf, _mo(slot * 7 * UP, 8), UP)
        pcs = a_prep(i + 1, 1 - slot)
        a_second(i - 1, pcs if APOS == 0 else ())
        ffa_slab(ops, ta1, 0)
        ffa_slab(ops, ta1, 1, share(pcs, 0, 3) if APOS == 2 else ())
        qmax = a_third(i - 1, qmax)
        ffa_slab(ops, ta1, 2, share(pcs, 0, 2) if APOS == 1 else share(pcs, 1, 3) if APOS == 2 else ())
        ffa_slab(ops, ta1, 3, share(pcs, 1, 2) if APOS == 1 else share(pcs, 2, 3) if APOS == 2 else ())
        return qmax

    def a_body(k, qmax):
        for t in range(UA):
            x_copy(UA * k + OFF + t).wait()
        for t in range(UA):
            x_copy(UA * k + OFF + 4 + t).start()
        for t in range(UA):
            i = 1 + UA * k + t
            qmax = a_step(i, (1 + t) % 2 if UA % 2 == 0 else i & 1, qmax)
        return qmax

    assert (NB - 1) % UA == 0
    qmax = jnp.zeros((8, 1), F32)
    with scope('loopA'):
        qmax = lax.fori_loop(0, (NB - 1) // UA, a_body, qmax)
    with scope2('seg2'):
        for i in range(NB - 1 + OFF, NB + 3 + OFF):
            x_copy(i).wait()
        a_second(NB - 1)
        qmax = a_third(NB - 1, qmax)
        for c in (c_dw, c_wp1, c_wp2, c_wv, c_wo, c_wa2, c_wb2):
            c.wait()
        dwf[...] = dwb[...].astype(F32)
        store7(tvo, _quads(_dot(wt0[...], wt1[...])))

    def g_row(i):
        b = _div(i, UPB)
        return _mo(8 + b * GP + (i - b * UPB) * U, 8)


    def kv_ops(ref, b, r0, n, which):
        rk = _mo(b * KHP + r0, 8)
        return [_unpack(ref[pl.ds(rk, n), i * HD:(i + 1) * HD]) for i in which]

    def q_ops(un):
        rk = unit_row(un)
        return [_unpack(kx[pl.ds(rk, RP), n * HD:(n + 1) * HD]) for n in L_OPS]

    def s_blocks(qops, b, s):
        ko = kv_ops(k7, b, s * (KS // 2), KS // 2, range(7))
        return _comb([_dot_nt(qops[p], ko[p]) for p in range(7)])

    bound2 = jnp.max(qmax) * (float(D) * 1.05)

    @pl.when(jnp.logical_not(bound2 <= SAFE_BOUND * SAFE_BOUND))
    def _():
        def unit_body(i, carry):
            b = _div(i, UPB)
            qops = q_ops(i)

            def slab_body(s, m):
                c = s_blocks(qops, b, s)
                col = s * KS + lax.broadcasted_iota(jnp.int32, (R, KS), 1)
                c = [jnp.where(col < KV, t, -jnp.inf) for t in c]
                top = jnp.max(jnp.maximum(c[0], c[1]), axis=-1, keepdims=True)
                bot = jnp.max(jnp.maximum(c[2], c[3]), axis=-1, keepdims=True)
                return jnp.maximum(m[0], top), jnp.maximum(m[1], bot)

            ninf = jnp.full((R, 1), -jnp.inf, F32)
            mt, mb = lax.fori_loop(0, NS, slab_body, (ninf, ninf))
            r = g_row(i)
            g[0, pl.ds(r, R), :] = jnp.broadcast_to(mt, (R, 128))
            g[0, pl.ds(r + R, R), :] = jnp.broadcast_to(mb, (R, 128))
            return carry

        lax.fori_loop(0, NU, unit_body, 0)

    def pin(pin_i, val):
        g[0, pl.ds(pl.multiple_of(GJ + 8 * (pin_i & 1), 8), 8), :] = val

    def s_job(i, slot, pieces, pin_i):
        b = _div(i, UPB)
        r = g_row(i)
        qops = q_ops(i)
        m = [jnp.concatenate([g[0, pl.ds(r + h * R, R), :]] * (KS // 128), axis=1) for h in range(2)]
        l = [None, None]
        np_ = len(pieces)
        for s in range(NS):
            c = s_blocks(qops, b, s)
            pv = []
            for q in range(4):
                p = jnp.exp2(c[q] - m[q // 2])
                lo, hi = s * KS, (s + 1) * KS
                if hi > KV:
                    parts = []
                    for c0 in range(0, KS, 128):
                        nv = KV - (lo + c0)
                        if nv >= 128:
                            parts.append(p[:, c0:c0 + 128])
                        elif nv <= 0:
                            parts.append(jnp.zeros((R, 128), F32))
                        else:
                            lane = lax.broadcasted_iota(jnp.int32, (R, 128), 1)
                            parts.append(jnp.where(lane < nv, p[:, c0:c0 + 128], 0.0))
                    p = jnp.concatenate(parts, axis=1)
                pv.append(p)
                pbuf[slot * 4 + q, :, s * KS:(s + 1) * KS] = p
            for h in range(2):
                t = jnp.sum(pv[2 * h] + pv[2 * h + 1], axis=-1, keepdims=True)
                l[h] = t if l[h] is None else l[h] + t
            mine = share(pieces, s, NS)
            for t, piece in enumerate(mine):
                piece(pv[t % 4][(t * (R // 8)) // len(mine) * 8:, :])
        return l

    def pv_prep(slot, l, tick):
        inv = [1.0 / l[0], 1.0 / l[1]]

        def piece(j, c0, pinval):
            if pinval is not None:
                pbuf[8, pl.ds(pl.multiple_of(8 * zero[0], 8), 8), 0:128] = pinval[0:8, 0:128]
            rs, cs = slice(j * 16, (j + 1) * 16), slice(c0, c0 + PC)
            ops = _lhs7(*[pbuf[slot * 4 + q, rs, cs] * inv[q // 2][rs] for q in range(4)])
            for p in range(7):
                r0 = (slot * 7 + p) * RP + j * 8
                abuf[r0:r0 + 8, cs] = _pack(ops[p])
        return [functools.partial(piece, j, c0) for c0 in range(0, KH, PC) for j in range(R // 16)]

    def pv_job(i, slot, pieces):
        b = _div(i, UPB)
        NKG = KH // KG
        acc = [None] * 7
        for p in range(7):
            for kg in range(NKG):
                cs = slice(kg * KG, (kg + 1) * KG)
                vo, = kv_ops(kx, b, kg * (KG // 2), KG // 2, V_OPS[p:p + 1])
                part = _dot(_unpack(abuf[(slot * 7 + p) * RP:(slot * 7 + p + 1) * RP, cs]), vo)
                acc[p] = part if acc[p] is None else acc[p] + part
                mine = share(pieces, p * NKG + kg, NKG * 7)
                for t, piece in enumerate(mine):
                    j = (t * (R // 16)) // len(mine)
                    piece(part[j * 16:(j + 1) * 16, :])
        return _join(*_comb(acc))

    def post_1(k):
        attn = _join(*_comb(mm7(load7(obuf, 0, UP), tvo)))
        r = _mo(k * M, M)
        x2 = x1[pl.ds(r, M), :] + attn
        x1[pl.ds(r, M), :] = x2
        return ffa_prep(_ln(x2))

    def post_2(k, ops, pieces=()):
        ms = mm7(ops, tp1)
        for p in range(7):
            mine = share(pieces, p, 7)
            for t, piece in enumerate(mine):
                j = (t * (U // 8)) // len(mine)
                c0 = (t % 2) * HD
                piece(ms[p][j * 8:, c0:])
        a_top, g_top, a_bot, g_bot = _comb(ms)
        for a, bb, sub in ((a_top, g_top, 0), (a_bot, g_bot, 1)):
            gr = g_row(2 * k + sub)
            ha = a * 0.5
            gv = ha * jnp.tanh(bb * 0.5) + ha
            for c4 in range(NC4):
                g[c4, pl.ds(gr, U), :] = gv[:, c4 * 128:(c4 + 1) * 128]

    def conv_pieces(i):
        gr = g_row(i)
        r = _mo(i * (U // 2), 8)
        pieces = []
        G = CG * 8
        for c4 in range(NC4):
            cs = slice(c4 * 128, (c4 + 1) * 128)
            stt = {}

            def out_rows(k0, stt=stt, c4=c4, cs=cs):
                w = stt['w']
                if CMODE == 0:
                    acc = None
                    for j in range(K):
                        t = g[c4, pl.ds(gr + k0 - pad + j, 8), :] * w[j]
                        acc = t if acc is None else acc + t
                    return acc
                st = 2 if CMODE == 1 else 4

                def y(b, k):
                    if (b, k) not in stt:
                        acc = None
                        for j in range(b, K, st):
                            t = g[c4, pl.ds(gr + k - pad + j - b, 8), :] * w[j]
                            acc = t if acc is None else acc + t
                        stt[(b, k)] = acc
                    return stt[(b, k)]

                sub = lax.broadcasted_iota(jnp.int32, (8, 128), 0)
                acc = y(0, k0)
                for b in range(1, st):
                    lo = pltpu.roll(y(b, k0), 8 - b, 0)
                    hi = pltpu.roll(y(b, k0 + 8), 8 - b, 0)
                    acc = acc + jnp.where(sub < 8 - b, lo, hi)
                return acc

            for k in range(U // G):
                def piece(pinval, k=k, stt=stt, cs=cs, out_rows=out_rows):
                    if pinval is not None:
                        g[0, pl.ds(pl.multiple_of(GJ + 8 * (i & 1), 8), 8), :] = pinval[0:8, 0:128]
                    if k == 0:
                        stt['w'] = [dwf[pl.ds(j, 1), cs] for j in range(K)]
                    rows = []
                    for k0 in range(k * G, (k + 1) * G, 8):
                        acc = out_rows(k0)
                        rows.append(acc)
                        if k0 == 0:
                            stt['c'] = acc[0:1]
                        d = acc - stt['c']
                        stt['s1'] = d if k0 == 0 else stt['s1'] + d
                        stt['s2'] = d * d if k0 == 0 else stt['s2'] + d * d
                    dc[pl.ds(r + k * (G // 2), G // 2), cs] = _pack(jnp.concatenate(rows, axis=0))
                    if k == U // G - 1:
                        stat_c[pl.ds(_mo(i * 8, 8), 8), cs] = jnp.broadcast_to(stt['c'], (8, 128))
                        stat_1[pl.ds(_mo(i * 8, 8), 8), cs] = stt['s1']
                        stat_2[pl.ds(_mo(i * 8, 8), 8), cs] = stt['s2']
                pieces.append(piece)
        return pieces

    def conv(i):
        for p_ in conv_pieces(i):
            p_(None)

    def b_group(k, do_post, do_conv, fill=None):
        units = [2 * k, 2 * k + 1]
        if do_post:
            pops = post_1(k - 1)
        if do_conv:
            cp = conv_pieces(jnp.maximum(units[0] - 4, 0)) + conv_pieces(jnp.maximum(units[1] - 4, 1))
        else:
            cp = fill
        l0 = s_job(units[0], 0, [], k)
        prep0 = pv_prep(0, l0, k)
        n0 = len(prep0) * PSPLIT // 8 if do_post else 0
        if do_post:
            post_2(k - 1, pops, prep0[:n0])
        l1 = s_job(units[1], 1, prep0[n0:], k)
        prep1 = pv_prep(1, l1, k)
        nc = len(cp) * CSPLIT // 8
        os_ = [pv_job(units[0], 0, interleave(prep1, cp[:nc])), pv_job(units[1], 1, cp[nc:])]
        store_lhs7(obuf, 0, (os_[0][:, :HD], os_[0][:, HD:], os_[1][:, :HD], os_[1][:, HD:]))

    with scope2('proB'):
        wp = (weight_pieces(wp1_s, tp1, 1.0, WR) + weight_pieces(wp2_s, tp2, 1.0, WR)
              + weight_pieces(wa_s, ta2, 0.5, WR) + weight_pieces(wb_s, tb2, 0.5, WR))
        b_group(0, False, False, wp)

    def b_body(k, carry):
        b_group(k, True, True)
        return carry

    with scope('loopB'):
        lax.fori_loop(1, NB, b_body, 0)
    with scope2('tail1'):
        post_2(NB - 1, post_1(NB - 1), conv_pieces(NU - 4))
    with scope2('tail2'):
        for u in range(NU - 3, NU):
            conv(u)

    acc = None
    for u in range(NU):
        t = stat_1[u * 8:(u + 1) * 8, :] + float(U // 8) * stat_c[u * 8:(u + 1) * 8, :]
        acc = t if acc is None else acc + t
    mu = jnp.sum(acc, axis=0, keepdims=True) * (1.0 / N)
    acc = None
    for u in range(NU):
        e = mu - stat_c[u * 8:(u + 1) * 8, :]
        t = stat_2[u * 8:(u + 1) * 8, :] + e * (float(U // 8) * e - 2.0 * stat_1[u * 8:(u + 1) * 8, :])
        acc = t if acc is None else acc + t
    bn[pl.ds(0, 1), :] = mu
    bn[pl.ds(1, 1), :] = lax.rsqrt(jnp.sum(acc, axis=0, keepdims=True) * (1.0 / N) + EPS)

    def bn_silu(v):
        hx = (v - bn[pl.ds(0, 1), :]) * (bn[pl.ds(1, 1), :] * 0.5)
        return hx * jnp.tanh(hx) + hx

    def d_pre(j, slot):
        return lhs7_pieces(dc, _mo(j * U, 8), N // 2 + 8 * (slot & 1), bn_silu, slot, True)

    def d_first(j, slot):
        r = _mo(j * M, M)
        x3 = x1[pl.ds(r, M), :] + _join(*_comb(mm7(load7(ubuf, _mo(slot * 7 * UP, 8), UP), tp2)))
        x1[pl.ds(r, M), :] = x3
        return ffa_prep(_ln(x3))

    def d_last(j, y):
        r = _mo(j * M, M)
        xs[pl.ds(slot_row(j), M), :] = _ln(x1[pl.ds(r, M), :] + y).astype(BF)

    for j in range(-NS_X, -UD):
        o_copy(j).start()
    with scope2('proD'):
        for piece in d_pre(0, 0):
            piece(None)
        ops = d_first(0, 0)
        pcs = d_pre(1, 1)
        for s in range(NSL):
            ffa_slab(ops, ta2, s, share(pcs, s, NSL))

    def d_body(k, carry):
        for t in range(UD):
            o_copy(UD * k + t - NS_X).wait()
        for t in range(UD):
            o_copy(UD * k + t - UD).start()
        for t in range(UD):
            j = 1 + UD * k + t
            slot = (1 + t) % 2 if UD % 2 == 0 else j & 1
            if DORD == 0:
                ops = d_first(j, slot)
            y = ffb(tb2, d_pre(jnp.minimum(j + 1, NB - 1), 1 - slot))
            if DORD == 1:
                ops = d_first(j, slot)
            d_last(j - 1, y)
            for s in range(NSL):
                ffa_slab(ops, ta2, s)
        return carry

    assert (NB - 1) % UD == 0
    with scope('loopD'):
        lax.fori_loop(0, (NB - 1) // UD, d_body, 0)
    with scope2('end'):
        o_copy(NB - 1 - NS_X).wait()
        for j in range(NB - 1 - UD, NB - 1):
            o_copy(j).start()
        d_last(NB - 1, ffb(tb2))
        o_copy(NB - 1).start()
        for j in range(NB - NS_X, NB):
            o_copy(j).wait()


def conformer(x, w_ff1_a, w_ff1_b, w_q, w_k, w_v, w_o, w_pw1, dw, w_pw2, w_ff2_a, w_ff2_b,
              *, U=160, KS=512, UA=1, UB=2, UD=1, CG=2, CMODE=2, PINMODE=1, WR=32, APOS=3, KG=256, PC=256, CSPLIT=0, PSPLIT=6, TOK=0, KB=256, SL=256, KPOS=2, DORD=0, interpret=False, vmem_mb=126, scopes=0):
    B, T, D = x.shape
    F = w_ff1_a.shape[1]
    K = dw.shape[0]
    N = B * T
    NU = N // U
    R = U // 2
    RP = R // 2
    KH = -(-(T // 2) // KS) * KS
    kern = functools.partial(_kernel, B=B, T=T, D=D, F=F, K=K, U=U, KH=KH, KS=KS, UA=UA, UB=UB, UD=UD,
                             CG=CG, CMODE=CMODE, PINMODE=PINMODE, WR=WR, APOS=APOS, KG=KG, PC=PC, CSPLIT=CSPLIT, PSPLIT=PSPLIT, TOK=TOK, KB=KB, SL=SL, KPOS=KPOS, DORD=DORD, scopes=scopes)
    hbm = pl.BlockSpec(memory_space=pl.ANY)
    V = pltpu.VMEM
    HD, HF = D // 2, F // 2
    scratch = [
        V((16 * U + 32, D), BF),
        V((N, D), F32),
        V((B * KH // 2, 7 * HD), U32),
        V((B * KH // 2, 7 * HD), U32),
        V((D // 128, B * (T + 8) + 8 + 16, 128), F32),
        V((N // 2 + 16, D), U32),
        V((7 * HD // 2, HF), U32), V((7 * HF // 2, HD), U32),
        V((7 * HD // 2, HF), U32), V((7 * HF // 2, HD), U32),
        V((D + 32, F), BF), V((F + 32, D), BF),
        V((D, D), BF), V((D, D), BF),
        V((D + 32, 2 * D), BF), V((D + 32, D), BF),
        V((7 * HD // 2, HD), U32), V((7 * HD // 2, HD), U32),
        V((7 * HD // 2, D), U32), V((7 * HD // 2, HD), U32),
        V((K, D), BF), V((K, D), F32),
        V((7 * U // 2, HF), U32),
        V((9, R, KH), F32),
        V((2 * 7 * RP, KH), U32),
        V((7 * U // 2, HD), U32),
        V((2 * 7 * U // 2, HD), U32),
        V((NU * 8, D), F32), V((NU * 8, D), F32), V((NU * 8, D), F32), V((8, D), F32),
        pltpu.SMEM((1,), jnp.int32),
        pltpu.SemaphoreType.DMA((19,)),
        pltpu.SemaphoreType.DMA((8,)),
        pltpu.SemaphoreType.DMA((8,)),
    ]
    out = pl.pallas_call(
        kern,
        out_shape=jax.ShapeDtypeStruct((N, D), x.dtype),
        in_specs=[hbm] * 12,
        out_specs=hbm,
        scratch_shapes=scratch,
        compiler_params=pltpu.CompilerParams(vmem_limit_bytes=vmem_mb * 1024 * 1024),
        interpret=interpret,
    )(x.reshape(N, D), w_ff1_a, w_ff1_b, w_q, w_k, w_v, w_o, w_pw1, dw, w_pw2, w_ff2_a, w_ff2_b)
    return out.reshape(B, T, D)


@jax.jit
def pallas_standalone__conformer_family_conformer__speech_kernel(
    x: jax.Array,
    w_ff1_a: jax.Array,
    w_ff1_b: jax.Array,
    w_q: jax.Array,
    w_k: jax.Array,
    w_v: jax.Array,
    w_o: jax.Array,
    w_pw1: jax.Array,
    dw: jax.Array,
    w_pw2: jax.Array,
    w_ff2_a: jax.Array,
    w_ff2_b: jax.Array,
):
    return conformer(x, w_ff1_a, w_ff1_b, w_q, w_k, w_v, w_o, w_pw1, dw, w_pw2, w_ff2_a, w_ff2_b)
```

```python
import functools

import numpy as np
import jax
import jax.numpy as jnp
from jax import lax
import jax.experimental.pallas as pl
import jax.experimental.pallas.tpu as pltpu

BF = jnp.bfloat16
F32 = jnp.float32
U32 = jnp.uint32
EPS = 1e-5
LOG2E = float(np.log2(np.e))
SAFE_BOUND = 60.0
UNIT = 160
KS = 512
KG = 256
PC = 256
KB = 128
SL = 256
WR = 32
CG = 2
PSPLIT = 6


def _div(i, n):
    return i // n if isinstance(i, int) else lax.div(i, jnp.int32(n))


def _mo(v, n):
    return v if isinstance(v, int) else pl.multiple_of(v, n)


def _ln(x):
    m = jnp.mean(x, axis=-1, keepdims=True)
    xc = x - m
    v = jnp.mean(xc * xc, axis=-1, keepdims=True)
    return xc * lax.rsqrt(v + EPS)


def _pack(v):
    return pltpu.bitcast(v.astype(BF), U32)


def _unpack(v):
    return pltpu.bitcast(v, BF)


def _dot(a, b):
    return jnp.dot(a, b, preferred_element_type=F32)


def _dot_nt(a, b):
    return lax.dot_general(a, b, (((1,), (1,)), ((), ())), preferred_element_type=F32)


def _lhs7(a11, a12, a21, a22):
    return [a11 + a22, a21 + a22, a11, a22, a11 + a12, a21 - a11, a12 - a22]


def _rhs7(b11, b12, b21, b22):
    return [b11 + b22, b11, b12 - b22, b21 - b11, b22, b11 + b12, b21 + b22]


def _comb(m):
    return (m[0] + m[3] - m[4] + m[6], m[2] + m[4], m[1] + m[3], m[0] - m[1] + m[2] + m[5])


def _quads(x):
    r, h = x.shape[0] // 2, x.shape[1] // 2
    return x[:r, :h], x[:r, h:], x[r:, :h], x[r:, h:]


def _join(c11, c12, c21, c22):
    return jnp.concatenate([jnp.concatenate([c11, c12], 1), jnp.concatenate([c21, c22], 1)], 0)


def _kernel(x_hbm, wa1_hbm, wb1_hbm, wq_hbm, wk_hbm, wv_hbm, wo_hbm, wp1_hbm, dw_hbm, wp2_hbm,
            wa2_hbm, wb2_hbm, out_hbm,
            xs, x1, kx, k7, g, dc,
            ta1, tb1, ta2, tb2, wa_s, wb_s, wt0, wt1, wp1_s, wp2_s, tqk, tvo, tp1, tp2, dwb, dwf,
            sbuf, pbuf, abuf, obuf, ubuf, stat_c, stat_1, stat_2, bn,
            zero, sem_w, sem_x, sem_o,
            *, B, T, D, F, K, KH):
    U = UNIT
    N = B * T
    NU = N // U
    UPB = T // U
    R = U // 2
    RP = R // 2
    M = 2 * U
    UP = U // 2
    NB = N // M
    HD, HF = D // 2, F // 2
    NS = KH // KS
    KV = UPB * R
    KHP = KH // 2
    GP = T + 8
    GJ = B * GP + 8
    pad = K // 2
    NC4 = D // 128

    def wcopy(src, dst, k):
        return pltpu.make_async_copy(src, dst, sem_w.at[k])

    c_wq, c_wk = wcopy(wq_hbm, wt0, 0), wcopy(wk_hbm, wt1, 1)

    def lead(ref):
        return ref.at[pl.ds(0, ref.shape[0] - 32), :]

    c_wb1 = wcopy(wb1_hbm, lead(wb_s), 3)
    c_dw, c_wp1, c_wp2 = wcopy(dw_hbm, dwb, 4), wcopy(wp1_hbm, lead(wp1_s), 5), wcopy(wp2_hbm, lead(wp2_s), 6)
    c_wa2, c_wb2 = wcopy(wa2_hbm, lead(wa_s), 7), wcopy(wb2_hbm, lead(wb_s), 8)

    def wa1_half(q):
        return [wcopy(wa1_hbm.at[:, pl.ds(c0, 512)], wa_s.at[pl.ds(0, D), pl.ds(c0, 512)], 11 + 2 * q + h)
                for h, c0 in enumerate((q * 512, F // 2 + q * 512))]

    c_wv, c_wo = wcopy(wv_hbm, wt0, 9), wcopy(wo_hbm, wt1, 10)

    NS_X = 8

    def slot_row(i):
        return (i % NS_X) * M if isinstance(i, int) else pl.multiple_of((i & (NS_X - 1)) * M, M)

    def x_copy(i):
        src = (i if i < NB else 0) if isinstance(i, int) else jnp.where(i < NB, i, 0)
        sem = sem_x.at[i % NS_X if isinstance(i, int) else i & (NS_X - 1)]
        return pltpu.make_async_copy(x_hbm.at[pl.ds(_mo(src * M, M), M), :],
                                     xs.at[pl.ds(slot_row(i), M), :], sem)

    def o_copy(j):
        dst = (j if j >= 0 else j + NS_X) if isinstance(j, int) else jnp.where(j >= 0, j, j + NS_X)
        sem = sem_o.at[j % NS_X if isinstance(j, int) else j & (NS_X - 1)]
        return pltpu.make_async_copy(xs.at[pl.ds(slot_row(j), M), :],
                                     out_hbm.at[pl.ds(_mo(dst * M, M), M), :], sem)

    x_copy(0).start()
    for c in wa1_half(0):
        c.start()

    zero[0] = 0
    for b in range(B):
        r0 = b * KHP + KV // 2
        kx[pl.ds(r0, KHP - KV // 2), :] = jnp.zeros((KHP - KV // 2, 7 * HD), U32)
        k7[pl.ds(r0, KHP - KV // 2), :] = jnp.zeros((KHP - KV // 2, 7 * HD), U32)
    for b in range(B + 1):
        g[:, pl.ds(b * GP, 8), :] = jnp.zeros((NC4, 8, 128), F32)
    g[0, pl.ds(0, GJ), :] = jnp.zeros((GJ, 128), F32)
    g[:, pl.ds(8 + 2 * U, 8), :] = jnp.zeros((NC4, 8, 128), F32)

    def store7(t_ref, blocks, scale=None):
        hk = blocks[0].shape[0]
        for p, t in enumerate(_rhs7(*blocks)):
            t_ref[p * hk // 2:(p + 1) * hk // 2, :] = _pack(t if scale is None else t * scale)

    def weight_pieces(w_ref, t_ref, scale, rows):
        kk, nn = w_ref.shape[0] - 32, w_ref.shape[1]
        hk, hn = kk // 2, nn // 2

        def piece(r0, c0, n, pinval):
            if pinval is not None:
                pin_to(w_ref, kk + 16 * (n & 1), pinval)
            blk = [w_ref[rr:rr + rows, cc:cc + 128].astype(F32) * scale
                   for rr in (r0, hk + r0) for cc in (c0, hn + c0)]
            for p, t in enumerate(_rhs7(*blk)):
                t_ref[(p * hk + r0) // 2:(p * hk + r0 + rows) // 2, c0:c0 + 128] = _pack(t)

        return [functools.partial(piece, r0, c0, r0 // rows + c0 // 128)
                for c0 in range(0, hn, 128) for r0 in range(0, hk, rows)]

    def mm7(ops, t_ref, cs=slice(None)):
        hk = t_ref.shape[0] // 7
        return [_dot(ops[p], _unpack(t_ref[p * hk:(p + 1) * hk, cs])) for p in range(7)]

    def load7(ref, r0, hp):
        return [_unpack(ref[pl.ds(r0 + p * hp, hp), :]) for p in range(7)]

    def store_lhs7(ref, r0, blocks, cs=slice(None)):
        hp = blocks[0].shape[0] // 2
        for p, t in enumerate(_lhs7(*blocks)):
            ref[pl.ds(r0 + p * hp, hp), cs] = _pack(t)

    NSL = HF // SL

    def ffa_prep(xn):
        return [t.astype(BF) for t in _lhs7(*_quads(xn))]

    def ffa_slab(ops, ta, s, pieces=()):
        cs = slice(s * SL, (s + 1) * SL)
        ms = mm7(ops, ta, cs)
        for p in range(7):
            for piece in share(pieces, p, 7):
                piece(ms[p])
        act = [hx * jnp.tanh(hx) + hx for hx in _comb(ms)]
        store_lhs7(sbuf, 0, act, cs)

    def pin_to(ref, row, val):
        n = 16 if ref.dtype == BF else 8
        v = val[0:n, 0:128]
        ref[pl.ds(pl.multiple_of(row, n), n), 0:128] = (
            pltpu.bitcast(v, U32) if ref.dtype == U32 else v.astype(ref.dtype))

    def share(pieces, step, steps):
        return pieces[step * len(pieces) // steps:(step + 1) * len(pieces) // steps]

    def ffb(tb, pieces=()):
        kb = KB if pieces else HF
        ms = []
        nk = HF // kb
        for p in range(7):
            acc = None
            for kc in range(nk):
                part = _dot(_unpack(sbuf[p * UP:(p + 1) * UP, kc * kb:(kc + 1) * kb]),
                            _unpack(tb[(p * HF + kc * kb) // 2:(p * HF + (kc + 1) * kb) // 2, :]))
                acc = part if acc is None else acc + part
                for piece in share(pieces, p * nk + kc, 7 * nk):
                    piece(part)
            ms.append(acc)
        return _join(*_comb(ms))

    PR = 16

    def lhs7_pieces(src, r, junk, fn, slot):
        def piece(j, pinval):
            if pinval is not None:
                pin_to(src, junk, pinval)
            top = fn(_unpack(src[pl.ds(r + j * PR // 2, PR // 2), :]).astype(F32))
            bot = fn(_unpack(src[pl.ds(r + (U + j * PR) // 2, PR // 2), :]).astype(F32))
            for p, t in enumerate(_lhs7(top[:, :HD], top[:, HD:], bot[:, :HD], bot[:, HD:])):
                ubuf[pl.ds(_mo(slot * 7 * UP + p * UP + j * (PR // 2), 8), PR // 2), :] = _pack(t)
        return [functools.partial(piece, j) for j in range(U // PR)]

    def a_second(i):
        y = ffb(tb1)
        r = _mo(i * M, M)
        x1v = xs[pl.ds(slot_row(i), M), :].astype(F32) + y
        x1[pl.ds(r, M), :] = x1v
        h = _ln(x1v)
        for sub in range(2):
            un = 2 * i + sub
            b = _div(un, UPB)
            u = un - b * UPB
            rk = _mo(b * KHP + u * RP, 8)
            h11, h12, h21, h22 = _quads(h[sub * U:(sub + 1) * U])
            blocks = (h11 + h22, h11, h22, h12 - h22, h21 - h11, h11 + h12, h21 + h22)
            for n, t in enumerate(blocks):
                kx[pl.ds(rk, RP), n * HD:(n + 1) * HD] = _pack(t)

    L_OPS = (0, 6, 1, 2, 5, 4, 3)
    V_OPS = (0, 1, 3, 4, 2, 5, 6)

    def unit_row(un):
        b = _div(un, UPB)
        return _mo(b * KHP + (un - b * UPB) * RP, 8)

    def a_third(i, kmax):
        for sub in range(2):
            rk = unit_row(2 * i + sub)
            ops = [_unpack(kx[pl.ds(rk, RP), n * HD:(n + 1) * HD]) for n in L_OPS]
            k11, k12, k21, k22 = _comb(mm7(ops, tqk))
            for n, t in enumerate((k11 + k22, k11, k21 - k22, k12 - k11, k22, k11 + k21, k12 + k22)):
                k7[pl.ds(rk, RP), n * HD:(n + 1) * HD] = _pack(t)
            n2 = jnp.maximum(jnp.sum(k11 * k11 + k12 * k12, axis=-1, keepdims=True),
                             jnp.sum(k21 * k21 + k22 * k22, axis=-1, keepdims=True))
            kmax = jnp.maximum(kmax, jnp.max(n2.reshape(R // 8, 8, 1), axis=0))
        return kmax

    wp_a1 = weight_pieces(wa_s, ta1, 0.5, WR)
    nh = len(wp_a1) // 2
    x_copy(0).wait()
    for c in wa1_half(0):
        c.wait()
    for c in wa1_half(1):
        c.start()
    for c in (c_wb1, c_wq, c_wk):
        c.start()
    x_copy(1).start()
    ops = ffa_prep(_ln(xs[pl.ds(slot_row(0), M), :].astype(F32)))
    for piece in wp_a1[:nh]:
        piece(None)
    for s in range(NSL // 2):
        ffa_slab(ops, ta1, s)
    for c in wa1_half(1):
        c.wait()
    for piece in wp_a1[nh:]:
        piece(None)
    for s in range(NSL // 2, NSL):
        ffa_slab(ops, ta1, s)
    c_wb1.wait()
    for piece in weight_pieces(wb_s, tb1, 0.5, WR):
        piece(None)
    c_wq.wait()
    c_wk.wait()
    for i in range(2, 5):
        x_copy(i).start()
    for c in (c_dw, c_wp1, c_wp2, c_wa2, c_wb2):
        c.start()
    store7(tqk, _quads(_dot_nt(wt1[...], wt0[...])), LOG2E * float(D) ** -0.5)
    c_wv.start()
    c_wo.start()

    def a_step(i, kmax):
        a_second(i - 1)
        ops = ffa_prep(_ln(xs[pl.ds(slot_row(i), M), :].astype(F32)))
        for s in range(NSL):
            if s == 2:
                kmax = a_third(i - 1, kmax)
            ffa_slab(ops, ta1, s)
        return kmax

    def a_body(i, kmax):
        x_copy(i).wait()
        x_copy(i + 4).start()
        return a_step(i, kmax)

    kmax = jnp.zeros((8, 1), F32)
    kmax = lax.fori_loop(1, NB, a_body, kmax)
    for i in range(NB, NB + 4):
        x_copy(i).wait()
    a_second(NB - 1)
    kmax = a_third(NB - 1, kmax)
    for c in (c_dw, c_wp1, c_wp2, c_wv, c_wo, c_wa2, c_wb2):
        c.wait()
    dwf[...] = dwb[...].astype(F32)
    store7(tvo, _quads(_dot(wt0[...], wt1[...])))

    def g_row(i):
        b = _div(i, UPB)
        return _mo(8 + b * GP + (i - b * UPB) * U, 8)

    def kv_ops(ref, b, r0, n, which):
        rk = _mo(b * KHP + r0, 8)
        return [_unpack(ref[pl.ds(rk, n), i * HD:(i + 1) * HD]) for i in which]

    def q_ops(un):
        rk = unit_row(un)
        return [_unpack(kx[pl.ds(rk, RP), n * HD:(n + 1) * HD]) for n in L_OPS]

    def s_blocks(qops, b, s):
        ko = kv_ops(k7, b, s * (KS // 2), KS // 2, range(7))
        return _comb([_dot_nt(qops[p], ko[p]) for p in range(7)])

    bound2 = jnp.max(kmax) * (float(D) * 1.05)

    @pl.when(jnp.logical_not(bound2 <= SAFE_BOUND * SAFE_BOUND))
    def _():
        def unit_body(i, carry):
            b = _div(i, UPB)
            qops = q_ops(i)

            def slab_body(s, m):
                c = s_blocks(qops, b, s)
                col = s * KS + lax.broadcasted_iota(jnp.int32, (R, KS), 1)
                c = [jnp.where(col < KV, t, -jnp.inf) for t in c]
                top = jnp.max(jnp.maximum(c[0], c[1]), axis=-1, keepdims=True)
                bot = jnp.max(jnp.maximum(c[2], c[3]), axis=-1, keepdims=True)
                return jnp.maximum(m[0], top), jnp.maximum(m[1], bot)

            ninf = jnp.full((R, 1), -jnp.inf, F32)
            mt, mb = lax.fori_loop(0, NS, slab_body, (ninf, ninf))
            r = g_row(i)
            g[0, pl.ds(r, R), :] = jnp.broadcast_to(mt, (R, 128))
            g[0, pl.ds(r + R, R), :] = jnp.broadcast_to(mb, (R, 128))
            return carry

        lax.fori_loop(0, NU, unit_body, 0)

    def s_job(i, slot, pieces):
        b = _div(i, UPB)
        r = g_row(i)
        qops = q_ops(i)
        m = [jnp.concatenate([g[0, pl.ds(r + h * R, R), :]] * (KS // 128), axis=1) for h in range(2)]
        l = [None, None]
        for s in range(NS):
            c = s_blocks(qops, b, s)
            pv = []
            for q in range(4):
                p = jnp.exp2(c[q] - m[q // 2])
                lo, hi = s * KS, (s + 1) * KS
                if hi > KV:
                    parts = []
                    for c0 in range(0, KS, 128):
                        nv = KV - (lo + c0)
                        if nv >= 128:
                            parts.append(p[:, c0:c0 + 128])
                        elif nv <= 0:
                            parts.append(jnp.zeros((R, 128), F32))
                        else:
                            lane = lax.broadcasted_iota(jnp.int32, (R, 128), 1)
                            parts.append(jnp.where(lane < nv, p[:, c0:c0 + 128], 0.0))
                    p = jnp.concatenate(parts, axis=1)
                pv.append(p)
                pbuf[slot * 4 + q, :, s * KS:(s + 1) * KS] = p
            for h in range(2):
                t = jnp.sum(pv[2 * h] + pv[2 * h + 1], axis=-1, keepdims=True)
                l[h] = t if l[h] is None else l[h] + t
            mine = share(pieces, s, NS)
            for t, piece in enumerate(mine):
                piece(pv[t % 4][(t * (R // 8)) // len(mine) * 8:, :])
        return l

    def pv_prep(slot, l):
        inv = [1.0 / l[0], 1.0 / l[1]]

        def piece(j, c0, pinval):
            if pinval is not None:
                pbuf[8, pl.ds(pl.multiple_of(8 * zero[0], 8), 8), 0:128] = pinval[0:8, 0:128]
            rs, cs = slice(j * 16, (j + 1) * 16), slice(c0, c0 + PC)
            ops = _lhs7(*[pbuf[slot * 4 + q, rs, cs] * inv[q // 2][rs] for q in range(4)])
            for p in range(7):
                r0 = (slot * 7 + p) * RP + j * 8
                abuf[r0:r0 + 8, cs] = _pack(ops[p])
        return [functools.partial(piece, j, c0) for c0 in range(0, KH, PC) for j in range(R // 16)]

    def pv_job(i, slot, pieces):
        b = _div(i, UPB)
        NKG = KH // KG
        acc = [None] * 7
        for p in range(7):
            for kg in range(NKG):
                cs = slice(kg * KG, (kg + 1) * KG)
                vo, = kv_ops(kx, b, kg * (KG // 2), KG // 2, V_OPS[p:p + 1])
                part = _dot(_unpack(abuf[(slot * 7 + p) * RP:(slot * 7 + p + 1) * RP, cs]), vo)
                acc[p] = part if acc[p] is None else acc[p] + part
                mine = share(pieces, p * NKG + kg, NKG * 7)
                for t, piece in enumerate(mine):
                    j = (t * (R // 16)) // len(mine)
                    piece(part[j * 16:(j + 1) * 16, :])
        return _join(*_comb(acc))

    def post_1(k):
        attn = _join(*_comb(mm7(load7(obuf, 0, UP), tvo)))
        r = _mo(k * M, M)
        x2 = x1[pl.ds(r, M), :] + attn
        x1[pl.ds(r, M), :] = x2
        return ffa_prep(_ln(x2))

    def post_2(k, ops, pieces=()):
        ms = mm7(ops, tp1)
        for p in range(7):
            mine = share(pieces, p, 7)
            for t, piece in enumerate(mine):
                j = (t * (U // 8)) // len(mine)
                c0 = (t % 2) * HD
                piece(ms[p][j * 8:, c0:])
        a_top, g_top, a_bot, g_bot = _comb(ms)
        for a, bb, sub in ((a_top, g_top, 0), (a_bot, g_bot, 1)):
            gr = g_row(2 * k + sub)
            ha = a * 0.5
            gv = ha * jnp.tanh(bb * 0.5) + ha
            for c4 in range(NC4):
                g[c4, pl.ds(gr, U), :] = gv[:, c4 * 128:(c4 + 1) * 128]

    def conv_pieces(i):
        gr = g_row(i)
        r = _mo(i * (U // 2), 8)
        pieces = []
        G = CG * 8
        for c4 in range(NC4):
            cs = slice(c4 * 128, (c4 + 1) * 128)
            stt = {}

            def out_rows(k0, stt=stt, c4=c4, cs=cs):
                w = stt['w']
                st = 4

                def y(b, k):
                    if (b, k) not in stt:
                        acc = None
                        for j in range(b, K, st):
                            t = g[c4, pl.ds(gr + k - pad + j - b, 8), :] * w[j]
                            acc = t if acc is None else acc + t
                        stt[(b, k)] = acc
                    return stt[(b, k)]

                sub = lax.broadcasted_iota(jnp.int32, (8, 128), 0)
                acc = y(0, k0)
                for b in range(1, st):
                    lo = pltpu.roll(y(b, k0), 8 - b, 0)
                    hi = pltpu.roll(y(b, k0 + 8), 8 - b, 0)
                    acc = acc + jnp.where(sub < 8 - b, lo, hi)
                return acc

            for k in range(U // G):
                def piece(pinval, k=k, stt=stt, cs=cs, out_rows=out_rows):
                    if pinval is not None:
                        g[0, pl.ds(pl.multiple_of(GJ + 8 * (i & 1), 8), 8), :] = pinval[0:8, 0:128]
                    if k == 0:
                        stt['w'] = [dwf[pl.ds(j, 1), cs] for j in range(K)]
                    rows = []
                    for k0 in range(k * G, (k + 1) * G, 8):
                        acc = out_rows(k0)
                        rows.append(acc)
                        if k0 == 0:
                            stt['c'] = acc[0:1]
                        d = acc - stt['c']
                        stt['s1'] = d if k0 == 0 else stt['s1'] + d
                        stt['s2'] = d * d if k0 == 0 else stt['s2'] + d * d
                    dc[pl.ds(r + k * (G // 2), G // 2), cs] = _pack(jnp.concatenate(rows, axis=0))
                    if k == U // G - 1:
                        stat_c[pl.ds(_mo(i * 8, 8), 8), cs] = jnp.broadcast_to(stt['c'], (8, 128))
                        stat_1[pl.ds(_mo(i * 8, 8), 8), cs] = stt['s1']
                        stat_2[pl.ds(_mo(i * 8, 8), 8), cs] = stt['s2']
                pieces.append(piece)
        return pieces

    def conv(i):
        for p_ in conv_pieces(i):
            p_(None)

    def b_group(k, do_post, do_conv, fill=None):
        units = [2 * k, 2 * k + 1]
        if do_post:
            pops = post_1(k - 1)
        if do_conv:
            cp = conv_pieces(jnp.maximum(units[0] - 4, 0)) + conv_pieces(jnp.maximum(units[1] - 4, 1))
        else:
            cp = fill
        l0 = s_job(units[0], 0, [])
        prep0 = pv_prep(0, l0)
        n0 = len(prep0) * PSPLIT // 8 if do_post else 0
        if do_post:
            post_2(k - 1, pops, prep0[:n0])
        l1 = s_job(units[1], 1, prep0[n0:])
        prep1 = pv_prep(1, l1)
        os_ = [pv_job(units[0], 0, prep1), pv_job(units[1], 1, cp)]
        store_lhs7(obuf, 0, (os_[0][:, :HD], os_[0][:, HD:], os_[1][:, :HD], os_[1][:, HD:]))

    wp = (weight_pieces(wp1_s, tp1, 1.0, WR) + weight_pieces(wp2_s, tp2, 1.0, WR)
          + weight_pieces(wa_s, ta2, 0.5, WR) + weight_pieces(wb_s, tb2, 0.5, WR))
    b_group(0, False, False, wp)

    def b_body(k, carry):
        b_group(k, True, True)
        return carry

    lax.fori_loop(1, NB, b_body, 0)
    post_2(NB - 1, post_1(NB - 1), conv_pieces(NU - 4))
    for u in range(NU - 3, NU):
        conv(u)

    acc = None
    for u in range(NU):
        t = stat_1[u * 8:(u + 1) * 8, :] + float(U // 8) * stat_c[u * 8:(u + 1) * 8, :]
        acc = t if acc is None else acc + t
    mu = jnp.sum(acc, axis=0, keepdims=True) * (1.0 / N)
    acc = None
    for u in range(NU):
        e = mu - stat_c[u * 8:(u + 1) * 8, :]
        t = stat_2[u * 8:(u + 1) * 8, :] + e * (float(U // 8) * e - 2.0 * stat_1[u * 8:(u + 1) * 8, :])
        acc = t if acc is None else acc + t
    bn[pl.ds(0, 1), :] = mu
    bn[pl.ds(1, 1), :] = lax.rsqrt(jnp.sum(acc, axis=0, keepdims=True) * (1.0 / N) + EPS)

    def bn_silu(v):
        hx = (v - bn[pl.ds(0, 1), :]) * (bn[pl.ds(1, 1), :] * 0.5)
        return hx * jnp.tanh(hx) + hx

    def d_pre(j, slot):
        return lhs7_pieces(dc, _mo(j * U, 8), N // 2 + 8 * (slot & 1), bn_silu, slot)

    def d_first(j, slot):
        r = _mo(j * M, M)
        x3 = x1[pl.ds(r, M), :] + _join(*_comb(mm7(load7(ubuf, _mo(slot * 7 * UP, 8), UP), tp2)))
        x1[pl.ds(r, M), :] = x3
        return ffa_prep(_ln(x3))

    def d_last(j, y):
        r = _mo(j * M, M)
        xs[pl.ds(slot_row(j), M), :] = _ln(x1[pl.ds(r, M), :] + y).astype(BF)

    for j in range(-NS_X, -1):
        o_copy(j).start()
    for piece in d_pre(0, 0):
        piece(None)
    ops = d_first(0, 0)
    pcs = d_pre(1, 1)
    for s in range(NSL):
        ffa_slab(ops, ta2, s, share(pcs, s, NSL))

    def d_body(j, carry):
        o_copy(j - 1 - NS_X).wait()
        o_copy(j - 2).start()
        slot = j & 1
        ops = d_first(j, slot)
        y = ffb(tb2, d_pre(jnp.minimum(j + 1, NB - 1), 1 - slot))
        d_last(j - 1, y)
        for s in range(NSL):
            ffa_slab(ops, ta2, s)
        return carry

    lax.fori_loop(1, NB, d_body, 0)
    o_copy(NB - 1 - NS_X).wait()
    o_copy(NB - 2).start()
    d_last(NB - 1, ffb(tb2))
    o_copy(NB - 1).start()
    for j in range(NB - NS_X, NB):
        o_copy(j).wait()


def conformer(x, w_ff1_a, w_ff1_b, w_q, w_k, w_v, w_o, w_pw1, dw, w_pw2, w_ff2_a, w_ff2_b):
    B, T, D = x.shape
    F = w_ff1_a.shape[1]
    K = dw.shape[0]
    N = B * T
    U = UNIT
    NU = N // U
    R = U // 2
    RP = R // 2
    KH = -(-(T // 2) // KS) * KS
    kern = functools.partial(_kernel, B=B, T=T, D=D, F=F, K=K, KH=KH)
    hbm = pl.BlockSpec(memory_space=pl.ANY)
    V = pltpu.VMEM
    HD, HF = D // 2, F // 2
    scratch = [
        V((16 * U + 32, D), BF),
        V((N, D), F32),
        V((B * KH // 2, 7 * HD), U32),
        V((B * KH // 2, 7 * HD), U32),
        V((D // 128, B * (T + 8) + 8 + 16, 128), F32),
        V((N // 2 + 16, D), U32),
        V((7 * HD // 2, HF), U32), V((7 * HF // 2, HD), U32),
        V((7 * HD // 2, HF), U32), V((7 * HF // 2, HD), U32),
        V((D + 32, F), BF), V((F + 32, D), BF),
        V((D, D), BF), V((D, D), BF),
        V((D + 32, 2 * D), BF), V((D + 32, D), BF),
        V((7 * HD // 2, HD), U32), V((7 * HD // 2, HD), U32),
        V((7 * HD // 2, D), U32), V((7 * HD // 2, HD), U32),
        V((K, D), BF), V((K, D), F32),
        V((7 * U // 2, HF), U32),
        V((9, R, KH), F32),
        V((2 * 7 * RP, KH), U32),
        V((7 * U // 2, HD), U32),
        V((2 * 7 * U // 2, HD), U32),
        V((NU * 8, D), F32), V((NU * 8, D), F32), V((NU * 8, D), F32), V((8, D), F32),
        pltpu.SMEM((1,), jnp.int32),
        pltpu.SemaphoreType.DMA((19,)),
        pltpu.SemaphoreType.DMA((8,)),
        pltpu.SemaphoreType.DMA((8,)),
    ]
    out = pl.pallas_call(
        kern,
        out_shape=jax.ShapeDtypeStruct((N, D), x.dtype),
        in_specs=[hbm] * 12,
        out_specs=hbm,
        scratch_shapes=scratch,
        compiler_params=pltpu.CompilerParams(
            vmem_limit_bytes=126 * 1024 * 1024,
            flags={'XLA_TPU_EVENLY_DISTRIBUTE_CRITICAL_NODES': True}),
    )(x.reshape(N, D), w_ff1_a, w_ff1_b, w_q, w_k, w_v, w_o, w_pw1, dw, w_pw2, w_ff2_a, w_ff2_b)
    return out.reshape(B, T, D)


@jax.jit
def pallas_standalone__conformer_family_conformer__speech_kernel(
    x: jax.Array,
    w_ff1_a: jax.Array,
    w_ff1_b: jax.Array,
    w_q: jax.Array,
    w_k: jax.Array,
    w_v: jax.Array,
    w_o: jax.Array,
    w_pw1: jax.Array,
    dw: jax.Array,
    w_pw2: jax.Array,
    w_ff2_a: jax.Array,
    w_ff2_b: jax.Array,
):
    return conformer(x, w_ff1_a, w_ff1_b, w_q, w_k, w_v, w_o, w_pw1, dw, w_pw2, w_ff2_a, w_ff2_b)
```

```python
import functools

import numpy as np
import jax
import jax.numpy as jnp
from jax import lax
import jax.experimental.pallas as pl
import jax.experimental.pallas.tpu as pltpu

BF = jnp.bfloat16
F32 = jnp.float32
U32 = jnp.uint32
EPS = 1e-5
LOG2E = float(np.log2(np.e))
SAFE_BOUND = 60.0
UNIT = 160
KS = 512
KG = 256
PC = 256
KB = 256
SL = 256
WR = 32
CG = 2
PSPLIT = 6


def _div(i, n):
    return i // n if isinstance(i, int) else lax.div(i, jnp.int32(n))


def _mo(v, n):
    return v if isinstance(v, int) else pl.multiple_of(v, n)


def _ln(x):
    m = jnp.mean(x, axis=-1, keepdims=True)
    xc = x - m
    v = jnp.mean(xc * xc, axis=-1, keepdims=True)
    return xc * lax.rsqrt(v + EPS)


def _pack(v):
    return pltpu.bitcast(v.astype(BF), U32)


def _unpack(v):
    return pltpu.bitcast(v, BF)


def _dot(a, b):
    return jnp.dot(a, b, preferred_element_type=F32)


def _dot_nt(a, b):
    return lax.dot_general(a, b, (((1,), (1,)), ((), ())), preferred_element_type=F32)


def _lhs7(a11, a12, a21, a22):
    return [a11 + a22, a21 + a22, a11, a22, a11 + a12, a21 - a11, a12 - a22]


def _rhs7(b11, b12, b21, b22):
    return [b11 + b22, b11, b12 - b22, b21 - b11, b22, b11 + b12, b21 + b22]


def _comb(m):
    return (m[0] + m[3] - m[4] + m[6], m[2] + m[4], m[1] + m[3], m[0] - m[1] + m[2] + m[5])


def _quads(x):
    r, h = x.shape[0] // 2, x.shape[1] // 2
    return x[:r, :h], x[:r, h:], x[r:, :h], x[r:, h:]


def _join(c11, c12, c21, c22):
    return jnp.concatenate([jnp.concatenate([c11, c12], 1), jnp.concatenate([c21, c22], 1)], 0)


def _kernel(x_hbm, wa1_hbm, wb1_hbm, wq_hbm, wk_hbm, wv_hbm, wo_hbm, wp1_hbm, dw_hbm, wp2_hbm,
            wa2_hbm, wb2_hbm, out_hbm,
            xs, x1, kx, k7, g, dc,
            ta1, tb1, wa_s, wb_s, wt0, wt1, wp1_s, wp2_s, tqk, tvo, tp1, tp2, dwb, dwf,
            sbuf, pbuf, abuf, obuf, ubuf, stat_c, stat_1, stat_2, bn,
            zero, sem_w, sem_x, sem_o,
            *, B, T, D, F, K, KH):
    ta2, tb2 = ta1, tb1
    U = UNIT
    N = B * T
    NU = N // U
    UPB = T // U
    R = U // 2
    RP = R // 2
    M = 2 * U
    UP = U // 2
    NB = N // M
    HD, HF = D // 2, F // 2
    NS = KH // KS
    KV = UPB * R
    KHP = KH // 2
    GP = T + 8
    GJ = B * GP + 8
    pad = K // 2
    NC4 = D // 128

    def wcopy(src, dst, k):
        return pltpu.make_async_copy(src, dst, sem_w.at[k])

    c_wq, c_wk = wcopy(wq_hbm, wt0, 0), wcopy(wk_hbm, wt1, 1)

    def lead(ref):
        return ref.at[pl.ds(0, ref.shape[0] - 32), :]

    c_wb1 = wcopy(wb1_hbm, lead(wb_s), 3)
    c_dw, c_wp1, c_wp2 = wcopy(dw_hbm, dwb, 4), wcopy(wp1_hbm, lead(wp1_s), 5), wcopy(wp2_hbm, lead(wp2_s), 6)
    c_wa2, c_wb2 = wcopy(wa2_hbm, lead(wa_s), 7), wcopy(wb2_hbm, lead(wb_s), 8)

    def wa1_half(q):
        return [wcopy(wa1_hbm.at[:, pl.ds(c0, 512)], wa_s.at[pl.ds(0, D), pl.ds(c0, 512)], 11 + 2 * q + h)
                for h, c0 in enumerate((q * 512, F // 2 + q * 512))]

    c_wv, c_wo = wcopy(wv_hbm, wt0, 9), wcopy(wo_hbm, wt1, 10)

    NS_X = 8

    def slot_row(i):
        return (i % NS_X) * M if isinstance(i, int) else pl.multiple_of((i & (NS_X - 1)) * M, M)

    def x_copy(i):
        src = (i if i < NB else 0) if isinstance(i, int) else jnp.where(i < NB, i, 0)
        sem = sem_x.at[i % NS_X if isinstance(i, int) else i & (NS_X - 1)]
        return pltpu.make_async_copy(x_hbm.at[pl.ds(_mo(src * M, M), M), :],
                                     xs.at[pl.ds(slot_row(i), M), :], sem)

    def o_copy(j):
        dst = (j if j >= 0 else j + NS_X) if isinstance(j, int) else jnp.where(j >= 0, j, j + NS_X)
        sem = sem_o.at[j % NS_X if isinstance(j, int) else j & (NS_X - 1)]
        return pltpu.make_async_copy(xs.at[pl.ds(slot_row(j), M), :],
                                     out_hbm.at[pl.ds(_mo(dst * M, M), M), :], sem)

    x_copy(0).start()
    for c in wa1_half(0):
        c.start()

    zero[0] = 0
    for b in range(B):
        r0 = b * KHP + KV // 2
        kx[pl.ds(r0, KHP - KV // 2), :] = jnp.zeros((KHP - KV // 2, 7 * HD), U32)
        k7[pl.ds(r0, KHP - KV // 2), :] = jnp.zeros((KHP - KV // 2, 7 * HD), U32)
    for b in range(B + 1):
        g[:, pl.ds(b * GP, 8), :] = jnp.zeros((NC4, 8, 128), F32)
    g[0, pl.ds(0, GJ), :] = jnp.zeros((GJ, 128), F32)
    g[:, pl.ds(8 + 2 * U, 8), :] = jnp.zeros((NC4, 8, 128), F32)

    def store7(t_ref, blocks, scale=None):
        hk = blocks[0].shape[0]
        for p, t in enumerate(_rhs7(*blocks)):
            t_ref[p * hk // 2:(p + 1) * hk // 2, :] = _pack(t if scale is None else t * scale)

    def weight_pieces(w_ref, t_ref, scale, rows):
        kk, nn = w_ref.shape[0] - 32, w_ref.shape[1]
        hk, hn = kk // 2, nn // 2

        def piece(r0, c0, n, pinval):
            if pinval is not None:
                pin_to(w_ref, kk + 16 * (n & 1), pinval)
            blk = [w_ref[rr:rr + rows, cc:cc + 128].astype(F32) * scale
                   for rr in (r0, hk + r0) for cc in (c0, hn + c0)]
            for p, t in enumerate(_rhs7(*blk)):
                t_ref[(p * hk + r0) // 2:(p * hk + r0 + rows) // 2, c0:c0 + 128] = _pack(t)

        return [functools.partial(piece, r0, c0, r0 // rows + c0 // 128)
                for c0 in range(0, hn, 128) for r0 in range(0, hk, rows)]

    def mm7(ops, t_ref, cs=slice(None)):
        hk = t_ref.shape[0] // 7
        return [_dot(ops[p], _unpack(t_ref[p * hk:(p + 1) * hk, cs])) for p in range(7)]

    def load7(ref, r0, hp):
        return [_unpack(ref[pl.ds(r0 + p * hp, hp), :]) for p in range(7)]

    def store_lhs7(ref, r0, blocks, cs=slice(None)):
        hp = blocks[0].shape[0] // 2
        for p, t in enumerate(_lhs7(*blocks)):
            ref[pl.ds(r0 + p * hp, hp), cs] = _pack(t)

    NSL = HF // SL

    def ffa_prep(xn):
        return [t.astype(BF) for t in _lhs7(*_quads(xn))]

    def ffa_slab(ops, ta, s, pieces=()):
        cs = slice(s * SL, (s + 1) * SL)
        ms = mm7(ops, ta, cs)
        for p in range(7):
            for piece in share(pieces, p, 7):
                piece(ms[p])
        act = [hx * jnp.tanh(hx) + hx for hx in _comb(ms)]
        store_lhs7(sbuf, 0, act, cs)

    def pin_to(ref, row, val):
        n = 16 if ref.dtype == BF else 8
        v = val[0:n, 0:128]
        ref[pl.ds(pl.multiple_of(row, n), n), 0:128] = (
            pltpu.bitcast(v, U32) if ref.dtype == U32 else v.astype(ref.dtype))

    def share(pieces, step, steps):
        return pieces[step * len(pieces) // steps:(step + 1) * len(pieces) // steps]

    def ffb(tb, pieces=()):
        kb = KB if pieces else HF
        ms = []
        nk = HF // kb
        for p in range(7):
            acc = None
            for kc in range(nk):
                part = _dot(_unpack(sbuf[p * UP:(p + 1) * UP, kc * kb:(kc + 1) * kb]),
                            _unpack(tb[(p * HF + kc * kb) // 2:(p * HF + (kc + 1) * kb) // 2, :]))
                acc = part if acc is None else acc + part
                for piece in share(pieces, p * nk + kc, 7 * nk):
                    piece(part)
            ms.append(acc)
        return _join(*_comb(ms))

    PR = 16

    def lhs7_pieces(src, r, junk, fn, slot):
        def piece(j, pinval):
            if pinval is not None:
                pin_to(src, junk, pinval)
            top = fn(_unpack(src[pl.ds(r + j * PR // 2, PR // 2), :]).astype(F32))
            bot = fn(_unpack(src[pl.ds(r + (U + j * PR) // 2, PR // 2), :]).astype(F32))
            for p, t in enumerate(_lhs7(top[:, :HD], top[:, HD:], bot[:, :HD], bot[:, HD:])):
                ubuf[pl.ds(_mo(slot * 7 * UP + p * UP + j * (PR // 2), 8), PR // 2), :] = _pack(t)
        return [functools.partial(piece, j) for j in range(U // PR)]

    def a_second(i):
        y = ffb(tb1)
        r = _mo(i * M, M)
        x1v = xs[pl.ds(slot_row(i), M), :].astype(F32) + y
        x1[pl.ds(r, M), :] = x1v
        h = _ln(x1v)
        for sub in range(2):
            un = 2 * i + sub
            b = _div(un, UPB)
            u = un - b * UPB
            rk = _mo(b * KHP + u * RP, 8)
            h11, h12, h21, h22 = _quads(h[sub * U:(sub + 1) * U])
            blocks = (h11 + h22, h11, h22, h12 - h22, h21 - h11, h11 + h12, h21 + h22)
            for n, t in enumerate(blocks):
                kx[pl.ds(rk, RP), n * HD:(n + 1) * HD] = _pack(t)

    L_OPS = (0, 6, 1, 2, 5, 4, 3)
    V_OPS = (0, 1, 3, 4, 2, 5, 6)

    def unit_row(un):
        b = _div(un, UPB)
        return _mo(b * KHP + (un - b * UPB) * RP, 8)

    def a_third(i, kmax):
        for sub in range(2):
            rk = unit_row(2 * i + sub)
            ops = [_unpack(kx[pl.ds(rk, RP), n * HD:(n + 1) * HD]) for n in L_OPS]
            k11, k12, k21, k22 = _comb(mm7(ops, tqk))
            for n, t in enumerate((k11 + k22, k11, k21 - k22, k12 - k11, k22, k11 + k21, k12 + k22)):
                k7[pl.ds(rk, RP), n * HD:(n + 1) * HD] = _pack(t)
            n2 = jnp.maximum(jnp.sum(k11 * k11 + k12 * k12, axis=-1, keepdims=True),
                             jnp.sum(k21 * k21 + k22 * k22, axis=-1, keepdims=True))
            kmax = jnp.maximum(kmax, jnp.max(n2.reshape(R // 8, 8, 1), axis=0))
        return kmax

    wp_a1 = weight_pieces(wa_s, ta1, 0.5, WR)
    nh = len(wp_a1) // 2
    x_copy(0).wait()
    for c in wa1_half(0):
        c.wait()
    for c in wa1_half(1):
        c.start()
    for c in (c_wb1, c_wq, c_wk):
        c.start()
    x_copy(1).start()
    ops = ffa_prep(_ln(xs[pl.ds(slot_row(0), M), :].astype(F32)))
    for piece in wp_a1[:nh]:
        piece(None)
    for s in range(NSL // 2):
        ffa_slab(ops, ta1, s)
    for c in wa1_half(1):
        c.wait()
    for piece in wp_a1[nh:]:
        piece(None)
    for s in range(NSL // 2, NSL):
        ffa_slab(ops, ta1, s)
    c_wb1.wait()
    for piece in weight_pieces(wb_s, tb1, 0.5, WR):
        piece(None)
    c_wq.wait()
    c_wk.wait()
    for i in range(2, 5):
        x_copy(i).start()
    for c in (c_dw, c_wp1, c_wp2, c_wa2, c_wb2):
        c.start()
    store7(tqk, _quads(_dot_nt(wt1[...], wt0[...])), LOG2E * float(D) ** -0.5)
    c_wv.start()
    c_wo.start()

    def a_step(i, kmax):
        a_second(i - 1)
        ops = ffa_prep(_ln(xs[pl.ds(slot_row(i), M), :].astype(F32)))
        for s in range(NSL):
            if s == 2:
                kmax = a_third(i - 1, kmax)
            ffa_slab(ops, ta1, s)
        return kmax

    def a_body(i, kmax):
        x_copy(i).wait()
        x_copy(i + 4).start()
        return a_step(i, kmax)

    kmax = jnp.zeros((8, 1), F32)
    kmax = lax.fori_loop(1, NB, a_body, kmax)
    for i in range(NB, NB + 4):
        x_copy(i).wait()
    a_second(NB - 1)
    kmax = a_third(NB - 1, kmax)
    for c in (c_dw, c_wp1, c_wp2, c_wv, c_wo, c_wa2, c_wb2):
        c.wait()
    dwf[...] = dwb[...].astype(F32)
    store7(tvo, _quads(_dot(wt0[...], wt1[...])))

    def g_row(i):
        b = _div(i, UPB)
        return _mo(8 + b * GP + (i - b * UPB) * U, 8)

    def kv_ops(ref, b, r0, n, which):
        rk = _mo(b * KHP + r0, 8)
        return [_unpack(ref[pl.ds(rk, n), i * HD:(i + 1) * HD]) for i in which]

    def q_ops(un):
        rk = unit_row(un)
        return [_unpack(kx[pl.ds(rk, RP), n * HD:(n + 1) * HD]) for n in L_OPS]

    def s_blocks(qops, b, s):
        ko = kv_ops(k7, b, s * (KS // 2), KS // 2, range(7))
        return _comb([_dot_nt(qops[p], ko[p]) for p in range(7)])

    bound2 = jnp.max(kmax) * (float(D) * 1.05)

    @pl.when(jnp.logical_not(bound2 <= SAFE_BOUND * SAFE_BOUND))
    def _():
        def unit_body(i, carry):
            b = _div(i, UPB)
            qops = q_ops(i)

            def slab_body(s, m):
                c = s_blocks(qops, b, s)
                col = s * KS + lax.broadcasted_iota(jnp.int32, (R, KS), 1)
                c = [jnp.where(col < KV, t, -jnp.inf) for t in c]
                top = jnp.max(jnp.maximum(c[0], c[1]), axis=-1, keepdims=True)
                bot = jnp.max(jnp.maximum(c[2], c[3]), axis=-1, keepdims=True)
                return jnp.maximum(m[0], top), jnp.maximum(m[1], bot)

            ninf = jnp.full((R, 1), -jnp.inf, F32)
            mt, mb = lax.fori_loop(0, NS, slab_body, (ninf, ninf))
            r = g_row(i)
            g[0, pl.ds(r, R), :] = jnp.broadcast_to(mt, (R, 128))
            g[0, pl.ds(r + R, R), :] = jnp.broadcast_to(mb, (R, 128))
            return carry

        lax.fori_loop(0, NU, unit_body, 0)

    def s_job(i, slot, pieces):
        b = _div(i, UPB)
        r = g_row(i)
        qops = q_ops(i)
        m = [jnp.concatenate([g[0, pl.ds(r + h * R, R), :]] * (KS // 128), axis=1) for h in range(2)]
        l = [None, None]
        for s in range(NS):
            c = s_blocks(qops, b, s)
            pv = []
            for q in range(4):
                p = jnp.exp2(c[q] - m[q // 2])
                lo, hi = s * KS, (s + 1) * KS
                if hi > KV:
                    parts = []
                    for c0 in range(0, KS, 128):
                        nv = KV - (lo + c0)
                        if nv >= 128:
                            parts.append(p[:, c0:c0 + 128])
                        elif nv <= 0:
                            parts.append(jnp.zeros((R, 128), F32))
                        else:
                            lane = lax.broadcasted_iota(jnp.int32, (R, 128), 1)
                            parts.append(jnp.where(lane < nv, p[:, c0:c0 + 128], 0.0))
                    p = jnp.concatenate(parts, axis=1)
                pv.append(p)
                pbuf[slot * 4 + q, :, s * KS:(s + 1) * KS] = p
            for h in range(2):
                t = jnp.sum(pv[2 * h] + pv[2 * h + 1], axis=-1, keepdims=True)
                l[h] = t if l[h] is None else l[h] + t
            mine = share(pieces, s, NS)
            for t, piece in enumerate(mine):
                piece(pv[t % 4][(t * (R // 8)) // len(mine) * 8:, :])
        return l

    def pv_prep(slot, l):
        inv = [1.0 / l[0], 1.0 / l[1]]

        def piece(j, c0, pinval):
            if pinval is not None:
                pbuf[8, pl.ds(pl.multiple_of(8 * zero[0], 8), 8), 0:128] = pinval[0:8, 0:128]
            rs, cs = slice(j * 16, (j + 1) * 16), slice(c0, c0 + PC)
            ops = _lhs7(*[pbuf[slot * 4 + q, rs, cs] * inv[q // 2][rs] for q in range(4)])
            for p in range(7):
                r0 = (slot * 7 + p) * RP + j * 8
                abuf[r0:r0 + 8, cs] = _pack(ops[p])
        return [functools.partial(piece, j, c0) for c0 in range(0, KH, PC) for j in range(R // 16)]

    def pv_job(i, slot, pieces):
        b = _div(i, UPB)
        NKG = KH // KG
        acc = [None] * 7
        for p in range(7):
            for kg in range(NKG):
                cs = slice(kg * KG, (kg + 1) * KG)
                vo, = kv_ops(kx, b, kg * (KG // 2), KG // 2, V_OPS[p:p + 1])
                part = _dot(_unpack(abuf[(slot * 7 + p) * RP:(slot * 7 + p + 1) * RP, cs]), vo)
                acc[p] = part if acc[p] is None else acc[p] + part
                mine = share(pieces, p * NKG + kg, NKG * 7)
                for t, piece in enumerate(mine):
                    j = (t * (R // 16)) // len(mine)
                    piece(part[j * 16:(j + 1) * 16, :])
        return _join(*_comb(acc))

    def post_1(k):
        attn = _join(*_comb(mm7(load7(obuf, 0, UP), tvo)))
        r = _mo(k * M, M)
        x2 = x1[pl.ds(r, M), :] + attn
        x1[pl.ds(r, M), :] = x2
        return ffa_prep(_ln(x2))

    def post_2(k, ops, pieces=()):
        ms = mm7(ops, tp1)
        for p in range(7):
            mine = share(pieces, p, 7)
            for t, piece in enumerate(mine):
                j = (t * (U // 8)) // len(mine)
                c0 = (t % 2) * HD
                piece(ms[p][j * 8:, c0:])
        a_top, g_top, a_bot, g_bot = _comb(ms)
        for a, bb, sub in ((a_top, g_top, 0), (a_bot, g_bot, 1)):
            gr = g_row(2 * k + sub)
            ha = a * 0.5
            gv = ha * jnp.tanh(bb * 0.5) + ha
            for c4 in range(NC4):
                g[c4, pl.ds(gr, U), :] = gv[:, c4 * 128:(c4 + 1) * 128]

    def conv_pieces(i):
        gr = g_row(i)
        r = _mo(i * (U // 2), 8)
        pieces = []
        G = CG * 8
        for c4 in range(NC4):
            cs = slice(c4 * 128, (c4 + 1) * 128)
            stt = {}

            def out_rows(k0, stt=stt, c4=c4, cs=cs):
                w = stt['w']
                st = 4

                def y(b, k):
                    if (b, k) not in stt:
                        acc = None
                        for j in range(b, K, st):
                            t = g[c4, pl.ds(gr + k - pad + j - b, 8), :] * w[j]
                            acc = t if acc is None else acc + t
                        stt[(b, k)] = acc
                    return stt[(b, k)]

                sub = lax.broadcasted_iota(jnp.int32, (8, 128), 0)
                acc = y(0, k0)
                for b in range(1, st):
                    lo = pltpu.roll(y(b, k0), 8 - b, 0)
                    hi = pltpu.roll(y(b, k0 + 8), 8 - b, 0)
                    acc = acc + jnp.where(sub < 8 - b, lo, hi)
                return acc

            for k in range(U // G):
                def piece(pinval, k=k, stt=stt, cs=cs, out_rows=out_rows):
                    if pinval is not None:
                        g[0, pl.ds(pl.multiple_of(GJ + 8 * (i & 1), 8), 8), :] = pinval[0:8, 0:128]
                    if k == 0:
                        stt['w'] = [dwf[pl.ds(j, 1), cs] for j in range(K)]
                    rows = []
                    for k0 in range(k * G, (k + 1) * G, 8):
                        acc = out_rows(k0)
                        rows.append(acc)
                        if k0 == 0:
                            stt['c'] = acc[0:1]
                        d = acc - stt['c']
                        stt['s1'] = d if k0 == 0 else stt['s1'] + d
                        stt['s2'] = d * d if k0 == 0 else stt['s2'] + d * d
                    dc[pl.ds(r + k * (G // 2), G // 2), cs] = _pack(jnp.concatenate(rows, axis=0))
                    if k == U // G - 1:
                        stat_c[pl.ds(_mo(i * 8, 8), 8), cs] = jnp.broadcast_to(stt['c'], (8, 128))
                        stat_1[pl.ds(_mo(i * 8, 8), 8), cs] = stt['s1']
                        stat_2[pl.ds(_mo(i * 8, 8), 8), cs] = stt['s2']
                pieces.append(piece)
        return pieces

    def conv(i):
        for p_ in conv_pieces(i):
            p_(None)

    def b_group(k, do_post, do_conv, fill=None):
        units = [2 * k, 2 * k + 1]
        if do_post:
            pops = post_1(k - 1)
        if do_conv:
            cp = conv_pieces(jnp.maximum(units[0] - 4, 0)) + conv_pieces(jnp.maximum(units[1] - 4, 1))
        else:
            cp = fill
        l0 = s_job(units[0], 0, [])
        prep0 = pv_prep(0, l0)
        n0 = len(prep0) * PSPLIT // 8 if do_post else 0
        if do_post:
            post_2(k - 1, pops, prep0[:n0])
        l1 = s_job(units[1], 1, prep0[n0:])
        prep1 = pv_prep(1, l1)
        os_ = [pv_job(units[0], 0, prep1), pv_job(units[1], 1, cp)]
        store_lhs7(obuf, 0, (os_[0][:, :HD], os_[0][:, HD:], os_[1][:, :HD], os_[1][:, HD:]))

    wp = (weight_pieces(wp1_s, tp1, 1.0, WR) + weight_pieces(wp2_s, tp2, 1.0, WR)
          + weight_pieces(wa_s, ta2, 0.5, WR) + weight_pieces(wb_s, tb2, 0.5, WR))
    b_group(0, False, False, wp)

    def b_body(k, carry):
        b_group(k, True, True)
        return carry

    lax.fori_loop(1, NB, b_body, 0)
    post_2(NB - 1, post_1(NB - 1), conv_pieces(NU - 4))
    for u in range(NU - 3, NU):
        conv(u)

    acc = None
    for u in range(NU):
        t = stat_1[u * 8:(u + 1) * 8, :] + float(U // 8) * stat_c[u * 8:(u + 1) * 8, :]
        acc = t if acc is None else acc + t
    mu = jnp.sum(acc, axis=0, keepdims=True) * (1.0 / N)
    acc = None
    for u in range(NU):
        e = mu - stat_c[u * 8:(u + 1) * 8, :]
        t = stat_2[u * 8:(u + 1) * 8, :] + e * (float(U // 8) * e - 2.0 * stat_1[u * 8:(u + 1) * 8, :])
        acc = t if acc is None else acc + t
    bn[pl.ds(0, 1), :] = mu
    bn[pl.ds(1, 1), :] = lax.rsqrt(jnp.sum(acc, axis=0, keepdims=True) * (1.0 / N) + EPS)

    def bn_silu(v):
        hx = (v - bn[pl.ds(0, 1), :]) * (bn[pl.ds(1, 1), :] * 0.5)
        return hx * jnp.tanh(hx) + hx

    def d_pre(j, slot):
        return lhs7_pieces(dc, _mo(j * U, 8), N // 2 + 8 * (slot & 1), bn_silu, slot)

    def d_first(j, slot):
        r = _mo(j * M, M)
        x3 = x1[pl.ds(r, M), :] + _join(*_comb(mm7(load7(ubuf, _mo(slot * 7 * UP, 8), UP), tp2)))
        x1[pl.ds(r, M), :] = x3
        return ffa_prep(_ln(x3))

    def d_last(j, y):
        r = _mo(j * M, M)
        xs[pl.ds(slot_row(j), M), :] = _ln(x1[pl.ds(r, M), :] + y).astype(BF)

    for j in range(-NS_X, -1):
        o_copy(j).start()
    for piece in d_pre(0, 0):
        piece(None)
    ops = d_first(0, 0)
    pcs = d_pre(1, 1)
    for s in range(NSL):
        ffa_slab(ops, ta2, s, share(pcs, s, NSL))

    def d_body(j, carry):
        o_copy(j - 1 - NS_X).wait()
        o_copy(j - 2).start()
        slot = j & 1
        ops = d_first(j, slot)
        y = ffb(tb2, d_pre(jnp.minimum(j + 1, NB - 1), 1 - slot))
        d_last(j - 1, y)
        for s in range(NSL):
            ffa_slab(ops, ta2, s)
        return carry

    lax.fori_loop(1, NB, d_body, 0)
    o_copy(NB - 1 - NS_X).wait()
    o_copy(NB - 2).start()
    d_last(NB - 1, ffb(tb2))
    o_copy(NB - 1).start()
    for j in range(NB - NS_X, NB):
        o_copy(j).wait()


def conformer(x, w_ff1_a, w_ff1_b, w_q, w_k, w_v, w_o, w_pw1, dw, w_pw2, w_ff2_a, w_ff2_b):
    B, T, D = x.shape
    F = w_ff1_a.shape[1]
    K = dw.shape[0]
    N = B * T
    U = UNIT
    NU = N // U
    R = U // 2
    RP = R // 2
    KH = -(-(T // 2) // KS) * KS
    kern = functools.partial(_kernel, B=B, T=T, D=D, F=F, K=K, KH=KH)
    hbm = pl.BlockSpec(memory_space=pl.ANY)
    V = pltpu.VMEM
    HD, HF = D // 2, F // 2
    scratch = [
        V((16 * U + 32, D), BF),
        V((N, D), F32),
        V((B * KH // 2, 7 * HD), U32),
        V((B * KH // 2, 7 * HD), U32),
        V((D // 128, B * (T + 8) + 8 + 16, 128), F32),
        V((N // 2 + 16, D), U32),
        V((7 * HD // 2, HF), U32), V((7 * HF // 2, HD), U32),
        V((D + 32, F), BF), V((F + 32, D), BF),
        V((D, D), BF), V((D, D), BF),
        V((D + 32, 2 * D), BF), V((D + 32, D), BF),
        V((7 * HD // 2, HD), U32), V((7 * HD // 2, HD), U32),
        V((7 * HD // 2, D), U32), V((7 * HD // 2, HD), U32),
        V((K, D), BF), V((K, D), F32),
        V((7 * U // 2, HF), U32),
        V((9, R, KH), F32),
        V((2 * 7 * RP, KH), U32),
        V((7 * U // 2, HD), U32),
        V((2 * 7 * U // 2, HD), U32),
        V((NU * 8, D), F32), V((NU * 8, D), F32), V((NU * 8, D), F32), V((8, D), F32),
        pltpu.SMEM((1,), jnp.int32),
        pltpu.SemaphoreType.DMA((19,)),
        pltpu.SemaphoreType.DMA((8,)),
        pltpu.SemaphoreType.DMA((8,)),
    ]
    out = pl.pallas_call(
        kern,
        out_shape=jax.ShapeDtypeStruct((N, D), x.dtype),
        in_specs=[hbm] * 12,
        out_specs=hbm,
        scratch_shapes=scratch,
        compiler_params=pltpu.CompilerParams(
            vmem_limit_bytes=120 * 1024 * 1024,
            flags={'XLA_TPU_EVENLY_DISTRIBUTE_CRITICAL_NODES': True}),
    )(x.reshape(N, D), w_ff1_a, w_ff1_b, w_q, w_k, w_v, w_o, w_pw1, dw, w_pw2, w_ff2_a, w_ff2_b)
    return out.reshape(B, T, D)


@jax.jit
def pallas_standalone__conformer_family_conformer__speech_kernel(
    x: jax.Array,
    w_ff1_a: jax.Array,
    w_ff1_b: jax.Array,
    w_q: jax.Array,
    w_k: jax.Array,
    w_v: jax.Array,
    w_o: jax.Array,
    w_pw1: jax.Array,
    dw: jax.Array,
    w_pw2: jax.Array,
    w_ff2_a: jax.Array,
    w_ff2_b: jax.Array,
):
    return conformer(x, w_ff1_a, w_ff1_b, w_q, w_k, w_v, w_o, w_pw1, dw, w_pw2, w_ff2_a, w_ff2_b)
```
